```python
import jax
import jax.numpy as jnp

def _softmax(x, axis=-1):
    return jax.nn.softmax(x, axis=axis)

def _gelu(x):
    return jax.nn.gelu(x, approximate=True)

def _silu(x):
    return jax.nn.silu(x)

def _sigmoid(x):
    return jax.nn.sigmoid(x)

def _layernorm(x, axis=-1, eps=1e-05):
    m = jnp.mean(x, axis=axis, keepdims=True)
    v = jnp.var(x, axis=axis, keepdims=True)
    return (x - m) / jnp.sqrt(v + eps)

def _scatter_add(tgt, idx, src, axis=0):
    return tgt.at[idx].add(src)

def _segment_sum(src, seg, n):
    return jax.ops.segment_sum(src, seg, n)

class _Rng:

    def __init__(self, key):
        self._k = key

    def _next(self):
        self._k, sub = jax.random.split(self._k)
        return sub

    def normal(self, shape):
        return jax.random.normal(self._next(), shape, dtype=jnp.bfloat16)

    def randint(self, lo, hi, shape):
        return jax.random.randint(self._next(), shape, lo, hi, dtype=jnp.int32)

    def uniform(self, shape, lo=0.0, hi=1.0):
        return jax.random.uniform(self._next(), shape, jnp.bfloat16, lo, hi)

    def permutation(self, n):
        return jax.random.permutation(self._next(), n)
kernel_name = 'standalone__conformer_family_branchformer__speech'

def setup_inputs():
    _rng = _Rng(jax.random.key(int.from_bytes(__import__("os").urandom(4), "little")))
    _w = lambda a: (lambda t: t.astype(jnp.bfloat16) if jnp.issubdtype(t.dtype, jnp.floating) else t)(jnp.asarray(a))
    B, T, D, K = (2, 4000, 512, 31)
    s = float(D) ** (-0.5)
    return {'x': _w((lambda *s: _rng.normal(s) * 0.05)(B, T, D)), 'w_q': _w((lambda *s: _rng.normal(s) * 0.05)(D, D) * s), 'w_k': _w((lambda *s: _rng.normal(s) * 0.05)(D, D) * s), 'w_v': _w((lambda *s: _rng.normal(s) * 0.05)(D, D) * s), 'w_ao': _w((lambda *s: _rng.normal(s) * 0.05)(D, D) * s), 'w_up': _w((lambda *s: _rng.normal(s) * 0.05)(D, 2 * D) * s), 'dw': _w((lambda *s: _rng.normal(s) * 0.05)(K, D) * (1.0 / K)), 'w_dn': _w((lambda *s: _rng.normal(s) * 0.05)(D, D) * s), 'w_merge': _w((lambda *s: _rng.normal(s) * 0.05)(2 * D, D) * s)}

def reference(x, w_q, w_k, w_v, w_ao, w_up, dw, w_dn, w_merge):
    B, T, D = x.shape
    K = dw.shape[0]
    xa = _layernorm(x, axis=-1)
    q = jnp.einsum('btd,de->bte', xa, w_q)
    k = jnp.einsum('btd,de->bte', xa, w_k)
    v = jnp.einsum('btd,de->bte', xa, w_v)
    logits = jnp.einsum('btd,bsd->bts', q, k) * float(D) ** (-0.5)
    attn = _softmax(logits, axis=-1)
    ya = jnp.einsum('bts,bsd->btd', attn, v)
    ya = jnp.einsum('btd,de->bte', ya, w_ao)
    xc = _layernorm(x, axis=-1)
    h = _gelu(jnp.einsum('btd,de->bte', xc, w_up))
    u = h[..., :D].copy()
    g = _layernorm(h[..., D:], axis=-1)
    pad = K // 2
    gp = jnp.pad(g, ((0, 0), (pad, pad), (0, 0)))
    conv = jnp.zeros_like(g)
    for i in range(K):
        conv = conv + gp[:, i:i + T, :] * dw[i][None, None, :]
    yc = jnp.einsum('btd,de->bte', u * conv, w_dn)
    merged = jnp.concatenate([ya, yc], axis=-1)
    out = jnp.einsum('btf,fd->btd', merged, w_merge)
    return x + out
```

```python
import math
import jax
import jax.numpy as jnp
from jax import lax
import jax.experimental.pallas as pl
import jax.experimental.pallas.tpu as pltpu

F32 = jnp.float32
BF16 = jnp.bfloat16
U32 = jnp.uint32
LANES = 128
HALO = 16
EPS = 1e-5


def _dot(a, b):
    return jnp.dot(a, b, preferred_element_type=F32)


def _dot_nt(a, b):
    return lax.dot_general(a, b, (((1,), (1,)), ((), ())), preferred_element_type=F32)


def _layernorm(x):
    m = jnp.mean(x, axis=-1, keepdims=True)
    d = x - m
    v = jnp.mean(d * d, axis=-1, keepdims=True)
    return d * lax.rsqrt(v + EPS)


def _gelu(x):
    c = math.sqrt(2.0 / math.pi)
    hx = 0.5 * x
    return hx + hx * jnp.tanh(x * (c + (c * 0.044715) * (x * x)))


def _lhs_combos(a11, a12, a21, a22):
    return [a11 + a22, a21 + a22, a11, a22, a11 + a12, a21 - a11, a12 - a22]


def _rhs_combos(b11, b12, b21, b22):
    return [b11 + b22, b11, b12 - b22, b21 - b11, b22, b11 + b12, b21 + b22]


def _even(n, w):
    tot = sum(w)
    cum = [sum(w[:k]) for k in range(len(w) + 1)]
    return [n * cum[k + 1] // tot - n * cum[k] // tot for k in range(len(w))]


def make(H=400, CV=5, NCH=1, CG=4, PACK=True, PR=80, UNR=1, porder=(3, 4, 1, 5, 6, 2, 7), flags=None,
         SR=16, GR=16,
         w_pc=(1, 1, 1, 1, 1, 1, 1), w_se=(1, 1, 1, 1, 1, 1, 1), w_cv=(1, 1, 1, 1, 1, 1, 1),
         w_cv0=(1, 1, 1, 1, 0, 1, 0), w_fin=(1, 1, 1, 0, 0, 0, 0), w_st=(0, 0, 0, 1, 1, 1, 0)):
    def kernel(x_hbm, wq_hbm, wk_hbm, wv_hbm, wao_hbm, wup_hbm, dw_hbm, wdn_hbm, wm_hbm,
               o_hbm,
               xin, wtmp, wm, wup, dwv, wr, dwb, ql, la, kr, vr, gs, us, uc, ss0, ss1, pbuf, acc,
               mrun, mold, lrun, mfin, linv, obuf,
               wsem, xsem, osem):
        B, T, D = xin.shape
        DH = D // 2
        KT = dwv.shape[0]
        BQ = 2 * H
        NQ = T // BQ
        NP = T // 2
        NC = ss0.shape[0]
        CK = DH
        NT = D // LANES
        RS = 2 if PACK else 1
        ss = (ss0, ss1)

        def al(i, m):
            return i if isinstance(i, int) else pl.multiple_of(i, m)

        def st(ref, idx, r0, val):
            n, w = val.shape
            rows = pl.ds(al(r0 // RS, 8), n // RS)
            if PACK:
                v = val.reshape(n // 16, 2, 8, w)
                p = pltpu.pack_elementwise([v[:, 0], v[:, 1]], packed_dtype=BF16)
                ref[(*idx, rows, slice(None))] = p.reshape(n // 2, w)
            else:
                ref[(*idx, rows, slice(None))] = val.astype(BF16)

        def st_nat(ref, idx, r0, val):
            n, w = val.shape
            rows = pl.ds(al(r0 // RS, 8), n // RS)
            v = val.astype(BF16)
            ref[(*idx, rows, slice(None))] = pltpu.bitcast(v, U32) if PACK else v

        def ld(ref, idx, r0, n):
            v = ref[(*idx, pl.ds(al(r0 // RS, 8), n // RS), slice(None))]
            return pltpu.bitcast(v, BF16) if PACK else v

        wcopies = [
            pltpu.make_async_copy(wq_hbm, wtmp.at[0], wsem.at[0]),
            pltpu.make_async_copy(wk_hbm, wtmp.at[1], wsem.at[1]),
            pltpu.make_async_copy(wv_hbm, wtmp.at[2], wsem.at[2]),
            pltpu.make_async_copy(wao_hbm, wtmp.at[3], wsem.at[3]),
            pltpu.make_async_copy(wm_hbm, wm, wsem.at[4]),
            pltpu.make_async_copy(wdn_hbm, wtmp.at[4], wsem.at[5]),
            pltpu.make_async_copy(wup_hbm, wup, wsem.at[6]),
            pltpu.make_async_copy(dw_hbm, dwv, wsem.at[7]),
        ]

        def xcopy(b, j):
            r0 = al(j * BQ, BQ)
            return pltpu.make_async_copy(x_hbm.at[b, pl.ds(r0, BQ)], xin.at[b, pl.ds(r0, BQ)], xsem.at[b * NQ + j])

        def ocopy(b, j):
            r0 = al(j * BQ, BQ)
            return pltpu.make_async_copy(obuf.at[b, pl.ds(r0, BQ)], o_hbm.at[b, pl.ds(r0, BQ)], osem.at[b * NQ + j])

        def st_rhs(ref, idx, r0, w):
            cs = _rhs_combos(w[:DH, :DH], w[:DH, DH:], w[DH:, :DH], w[DH:, DH:])
            for i, c in enumerate(cs):
                st_nat(ref, (*idx, i), r0, c)

        wcopies[0].start()
        wcopies[1].start()
        zdt = U32 if PACK else BF16
        kr[:, pl.ds(NP // RS, (NC * CK - NP) // RS), :] = jnp.zeros((7, (NC * CK - NP) // RS, DH), zdt)
        vr[:, pl.ds(NP // RS, (NC * CK - NP) // RS), :] = jnp.zeros((7, (NC * CK - NP) // RS, DH), zdt)
        gs[:, pl.ds(0, HALO), :] = jnp.zeros((NT, HALO, LANES), F32)
        gs[:, pl.ds(HALO + T, HALO), :] = jnp.zeros((NT, HALO, LANES), F32)
        wcopies[0].wait()
        wcopies[1].wait()
        wcopies[2].start()
        wcopies[3].start()
        wcopies[7].start()
        scale = float(D) ** -0.5 * math.log2(math.e)
        st_rhs(wr, (2,), 0, _dot_nt(wtmp[1], wtmp[0]) * scale)
        wcopies[2].wait()
        wcopies[3].wait()
        wcopies[4].start()
        wcopies[5].start()
        wva = _dot(wtmp[2], wtmp[3]).astype(BF16)
        wcopies[7].wait()
        dwf = dwv[...].astype(F32)
        for t in range(NT):
            for i in range(KT):
                dwb[t, i] = jnp.broadcast_to(dwf[i:i + 1, t * LANES:(t + 1) * LANES], (8, LANES))
        wcopies[4].wait()
        wcopies[5].wait()
        wcopies[6].start()
        xcopy(0, 0).start()
        st_rhs(wr, (3,), 0, _dot(wva, wm[pl.ds(0, D), :]))
        st_rhs(vr, (), NC * CK, _dot(wtmp[4], wm[pl.ds(D, D), :]))
        wcopies[6].wait()
        for b in range(B):
            for j in range(NQ):
                if b or j:
                    xcopy(b, j).start()
        st_rhs(wr, (0,), 0, wup[:, pl.ds(0, D)].astype(F32))
        st_rhs(wr, (1,), 0, wup[:, pl.ds(D, D)].astype(F32))

        def never(i):
            return lax.broadcasted_iota(jnp.int32, (8, LANES), 1) + i < 0

        def gate(x, tok):
            if tok is None:
                return x
            t, nv = tok
            n, w = x.shape
            reps = (n // 8, w // LANES)
            return jnp.where(jnp.tile(nv, reps), jnp.tile(t, reps), x)

        def stream(gen, steps, weights):
            next(gen)
            return gen, _even(steps, weights)

        def step(gen, tok):
            try:
                gen.send(tok)
            except StopIteration:
                pass

        def drain(gen):
            for _ in gen:
                pass

        def spread(streams, nv):
            def hook(k, v):
                todo = []
                for gen, counts in streams:
                    for n in range(counts[k]):
                        todo.append(((H // 8) * n // counts[k] * 8, gen))
                todo.sort(key=lambda p: p[0])
                for r, gen in todo:
                    step(gen, (v[r:r + 8, :LANES], nv))
            return hook

        def norm_rows(b, j, n):
            for r in range(0, H, n):
                tok = yield
                a1 = _layernorm(gate(xin[b, pl.ds(al(j * BQ + r, 16), n), :].astype(F32), tok))
                a2 = _layernorm(gate(xin[b, pl.ds(al(j * BQ + H + r, 16), n), :].astype(F32), tok))
                cs = _lhs_combos(a1[:, :DH], a1[:, DH:], a2[:, :DH], a2[:, DH:])
                for i, c in enumerate(cs):
                    st_nat(ql, (i,), j * H + r, c)

        def strassen(M, buf, fin, hook):
            v = M(4)
            buf[2] = v
            hook(0, v)
            v = M(1) + buf[2]
            buf[0] = v
            hook(1, v)
            v = M(3)
            buf[0] = buf[0] + v
            buf[1] = v
            hook(2, v)
            v = buf[2] + M(2)
            buf[2] = v
            fin(2, v)
            hook(3, v)
            v = (buf[0] - buf[2]) + M(6)
            fin(3, v)
            hook(4, v)
            v = buf[1] + M(5)
            buf[1] = v
            fin(1, v)
            hook(5, v)
            v = (buf[0] - buf[1]) + M(7)
            fin(0, v)
            hook(6, v)

        def post_rows(j, m, n):
            buf = ss0.at[m]
            for r in range(0, H, n):
                tok = yield
                rr = pl.ds(r, n)
                if m <= 1:
                    for h in range(2):
                        v = jnp.concatenate([buf[2 * h, rr, :], buf[2 * h + 1, rr, :]], axis=1)
                        v = _gelu(gate(v, tok))
                        if m == 1:
                            v = _layernorm(v)
                        dst = gs if m == 1 else us
                        off = j * BQ + h * H + r + (HALO if m == 1 else 0)
                        for t in range(NT):
                            dst[t, pl.ds(al(off, 8), n), :] = v[:, t * LANES:(t + 1) * LANES]
                else:
                    q = [gate(buf[k, rr, :], tok) for k in range(4)]
                    cs = _rhs_combos(q[0], q[2], q[1], q[3]) if m == 2 else _rhs_combos(*q)
                    for i, c in enumerate(cs):
                        st(kr if m == 2 else vr, (i,), j * H + r, c)

        def proj_block(b, j, do_next):
            nv = never(b)
            for i in range(7):
                la[i] = ql[i, pl.ds(al(j * H // RS, 8), H // RS), :]
            ones = (1,) * 7
            fill = {
                2: [],
                1: [stream(post_rows(j, 2, GR), H // GR, ones)],
                0: [stream(post_rows(j, 1, GR), H // GR, ones)],
                3: [stream(post_rows(j, 0, GR), H // GR, ones)],
            }
            if do_next:
                fill[1].append(stream(norm_rows(b, j + 1, GR), H // GR, ones))
            for m in (2, 1, 0, 3):
                buf = ss0.at[m]

                def fin(q, v, buf=buf):
                    if q in (0, 3):
                        buf[q] = v
                strassen(lambda i: _dot(ld(la, (i - 1,), 0, H), ld(wr, (m, i - 1), 0, DH)), buf, fin,
                         spread(fill[m], nv))
            drain(post_rows(j, 3, GR))

        col = lax.broadcasted_iota(jnp.int32, (8, LANES), 1)

        def qk_unit(j, c, slot, valid, hook):
            buf = ss[slot].at[c]

            def fin(q, v):
                v = jnp.concatenate(
                    [v[:, :LANES], jnp.where(jnp.tile(valid, (H // 8, 1)), v[:, LANES:], -jnp.inf)], axis=1)
                if q in (0, 3):
                    buf[q] = v
                mrun[q // 2] = jnp.maximum(mrun[q // 2], jnp.maximum(v[:, :LANES], v[:, LANES:]))
            strassen(lambda i: _dot_nt(ld(ql, (i - 1,), j * H, H), ld(kr, (i - 1,), c * CK, CK)), buf, fin, hook)

        def sumexp(c, slot, valid, n):
            vn = jnp.tile(valid, (n // 8, 1))
            for h in (1, 0):
                for r in range(0, H, n):
                    tok = yield
                    rr = pl.ds(r, n)
                    m = gate(mrun[h, rr, :], tok)
                    l = lrun[h, rr, :] * jnp.exp2(mold[h, rr, :] - m)
                    for q in (2 * h, 2 * h + 1):
                        l = l + jnp.exp2(ss[slot][c, q, rr, pl.ds(0, LANES)] - m)
                        e = jnp.exp2(ss[slot][c, q, rr, pl.ds(LANES, LANES)] - m)
                        l = l + (e if q in (0, 3) else jnp.where(vn, e, 0.0))
                    lrun[h, rr, :] = l
                    mold[h, rr, :] = m

        def finish_stats(n):
            for h in range(2):
                for r in range(0, H, n):
                    tok = yield
                    rr = pl.ds(r, n)
                    ml = gate(mrun[h, rr, :], tok)
                    m = jnp.max(ml, axis=-1, keepdims=True)
                    l = jnp.sum(lrun[h, rr, :] * jnp.exp2(ml - m), axis=-1, keepdims=True)
                    mfin[h, rr, :] = jnp.broadcast_to(m, (n, LANES))
                    linv[h, rr, :] = jnp.broadcast_to(1.0 / l, (n, LANES))
                    mrun[h, rr, :] = jnp.full((n, LANES), -jnp.inf, F32)
                    mold[h, rr, :] = jnp.full((n, LANES), -jnp.inf, F32)
                    lrun[h, rr, :] = jnp.zeros((n, LANES), F32)

        def p_combos(c, slot, valid, n):
            vn = jnp.tile(valid, (n // 8, 1))
            for r in range(0, H, n):
                tok = yield
                rr = pl.ds(r, n)
                a = []
                for h in range(2):
                    m = gate(mfin[h, rr, :], tok)
                    il = linv[h, rr, :]
                    for q in (2 * h, 2 * h + 1):
                        p0 = jnp.exp2(ss[slot][c, q, rr, pl.ds(0, LANES)] - m) * il
                        p1 = jnp.exp2(ss[slot][c, q, rr, pl.ds(LANES, LANES)] - m) * il
                        if q in (1, 2):
                            p1 = jnp.where(vn, p1, 0.0)
                        a.append(jnp.concatenate([p0, p1], axis=1))
                for i, v in enumerate(_lhs_combos(*a)):
                    st(pbuf, (i,), r, v)

        def u_combos():
            for r in range(0, H, PR):
                a = []
                for q in range(4):
                    rr = pl.ds((q // 2) * H + r, PR)
                    a.append(jnp.concatenate([uc[2 * (q % 2), rr, :], uc[2 * (q % 2) + 1, rr, :]], axis=1))
                for i, v in enumerate(_lhs_combos(*a)):
                    st(pbuf, (i,), r, v)

        def pv_product(c, i, first):
            v = _dot(ld(pbuf, (i - 1,), 0, H), ld(vr, (i - 1,), c * CK, CK))
            for n in range(2):
                w = v[:, n * LANES:(n + 1) * LANES]
                acc[i - 1, n] = w if first else acc[i - 1, n] + w
            return v

        def conv(j, c):
            t = c // 2
            base = (c % 2) * H
            for a in range(0, H // 8, CV):
                n = CV
                o = [None] * NCH
                for i in range(KT):
                    w = dwb[t, i]
                    if i % CG == 0:
                        tok = yield
                        w = gate(w, tok)
                    g = gs[t, pl.ds(j * BQ + base + 8 * a + i + 1, 8 * n), :].reshape(n, 8, LANES)
                    term = (g * w[None]).reshape(8 * n, LANES)
                    k = i % NCH
                    o[k] = term if o[k] is None else o[k] + term
                tot = o[0]
                for k in range(1, NCH):
                    tot = tot + o[k]
                rows_in = pl.ds(al(j * BQ + base + 8 * a, 8), 8 * n)
                rows_out = pl.ds(al(base + 8 * a, 8), 8 * n)
                uc[t, rows_out, :] = us[t, rows_in, :] * tot

        def final(b, j, n):
            for r in range(0, H, n):
                tok = yield

                def A(i):
                    cols = []
                    for k in range(2):
                        if PACK:
                            lo = acc[i - 1, k, pl.ds(r, n // 2, stride=2), :].reshape(n // 16, 1, 8, LANES)
                            hi = acc[i - 1, k, pl.ds(r + 1, n // 2, stride=2), :].reshape(n // 16, 1, 8, LANES)
                            cols.append(jnp.concatenate([lo, hi], axis=1).reshape(n, LANES))
                        else:
                            cols.append(acc[i - 1, k, pl.ds(r, n), :])
                    return jnp.concatenate(cols, axis=1)
                m1, m3, m4 = A(1), gate(A(3), tok), gate(A(4), tok)
                c12 = m3 + A(5)
                c21 = A(2) + m4
                u = m1 + m4 + m3
                c11 = (u - c12) + A(7)
                c22 = (u - c21) + A(6)
                for h, v in enumerate((jnp.concatenate([c11, c12], axis=1), jnp.concatenate([c21, c22], axis=1))):
                    rows = pl.ds(al(j * BQ + h * H + r, 16), n)
                    obuf[b, rows, :] = (xin[b, rows, :].astype(F32) + v).astype(BF16)

        def unit(j, c, slot, do_qk, do_pv):
            nv = never(c)
            valid = col < NP - LANES - c * CK
            ncv = (H // 8 // CV) * (-(-KT // CG))
            if do_qk and do_pv:
                qk_unit(j + 1, c, 1 - slot, valid, spread([stream(p_combos(c, slot, valid, SR), H // SR, w_pc)], nv))
                hook = spread([stream(sumexp(c, 1 - slot, valid, SR), 2 * H // SR, w_se),
                               stream(conv(j + 1, c), ncv, w_cv)], nv)
            elif do_qk:
                qk_unit(j + 1, c, 1 - slot, valid, spread([stream(conv(j + 1, c), ncv, w_cv0)], nv))
                drain(sumexp(c, 1 - slot, valid, SR))
            else:
                drain(p_combos(c, slot, valid, SR))
                hook = spread([], nv)
            if do_pv:
                for k, i in enumerate(porder):
                    hook(k, pv_product(c, i, False))

        def chunks(f):
            def body(c, _):
                for k in range(UNR):
                    f(c * UNR + k)
                return 0
            lax.fori_loop(0, NC // UNR, body, 0)

        def start_block(b):
            u_combos()
            hook = spread([stream(finish_stats(SR), 2 * H // SR, w_st)], never(b))
            for k, i in enumerate(porder):
                hook(k, pv_product(NC, i, True))

        mrun[...] = jnp.full(mrun.shape, -jnp.inf, F32)
        mold[...] = jnp.full(mold.shape, -jnp.inf, F32)
        lrun[...] = jnp.zeros(lrun.shape, F32)

        def batch(b, _):
            xcopy(b, 0).wait()
            drain(norm_rows(b, 0, PR))

            def pbody(j, _):
                xcopy(b, j + 1).wait()
                proj_block(b, j, True)
                return 0
            lax.fori_loop(0, NQ - 1, pbody, 0)
            proj_block(b, NQ - 1, False)

            chunks(lambda c: unit(-1, c, 1, True, False))
            start_block(b)

            def qblock(jj, _):
                for slot in range(2):
                    j = 2 * jj + slot
                    chunks(lambda c: unit(j, c, slot, True, True))
                    drain(final(b, j, PR))
                    start_block(b)
                    ocopy(b, j).start()
                return 0
            lax.fori_loop(0, (NQ - 1) // 2, qblock, 0)
            chunks(lambda c: unit(NQ - 1, c, (NQ - 1) % 2, False, True))
            drain(final(b, NQ - 1, PR))
            ocopy(b, NQ - 1).start()
            return 0
        lax.fori_loop(0, B, batch, 0)
        for b in range(B):
            for j in range(NQ):
                ocopy(b, j).wait()

    def run(x, w_q, w_k, w_v, w_ao, w_up, dw, w_dn, w_merge):
        B, T, D = x.shape
        KT = dw.shape[0]
        DH = D // 2
        NT = D // LANES
        NP = T // 2
        NC = -(-NP // DH)
        NQ = T // (2 * H)
        assert NQ % 2 == 1
        RS = 2 if PACK else 1
        PT = U32 if PACK else BF16
        anyspec = pl.BlockSpec(memory_space=pl.ANY)
        return pl.pallas_call(
            kernel,
            out_shape=jax.ShapeDtypeStruct(x.shape, x.dtype),
            in_specs=[anyspec] * 9,
            out_specs=anyspec,
            scratch_shapes=[
                pltpu.VMEM((B, T, D), BF16),
                pltpu.VMEM((5, D, D), BF16),
                pltpu.VMEM((2 * D, D), BF16),
                pltpu.VMEM((D, 2 * D), BF16),
                pltpu.VMEM((KT, D), BF16),
                pltpu.VMEM((4, 7, DH // RS, DH), PT),
                pltpu.VMEM((NT, KT, 8, LANES), F32),
                pltpu.VMEM((7, NP // RS, DH), PT),
                pltpu.VMEM((7, H // RS, DH), PT),
                pltpu.VMEM((7, NC * DH // RS, DH), PT),
                pltpu.VMEM((7, (NC + 1) * DH // RS, DH), PT),
                pltpu.VMEM((NT, T + 2 * HALO, LANES), F32),
                pltpu.VMEM((NT, T, LANES), F32),
                pltpu.VMEM((NT, 2 * H, LANES), F32),
                pltpu.VMEM((NC, 4, H, DH), F32),
                pltpu.VMEM((NC, 4, H, DH), F32),
                pltpu.VMEM((7, H // RS, DH), PT),
                pltpu.VMEM((7, 2, H, LANES), F32),
                pltpu.VMEM((2, H, LANES), F32),
                pltpu.VMEM((2, H, LANES), F32),
                pltpu.VMEM((2, H, LANES), F32),
                pltpu.VMEM((2, H, LANES), F32),
                pltpu.VMEM((2, H, LANES), F32),
                pltpu.VMEM((B, T, D), BF16),
                pltpu.SemaphoreType.DMA((8,)),
                pltpu.SemaphoreType.DMA((B * NQ,)),
                pltpu.SemaphoreType.DMA((B * NQ,)),
            ],
            compiler_params=pltpu.CompilerParams(vmem_limit_bytes=124 * 1024 * 1024, flags=flags),
        )(x, w_q, w_k, w_v, w_ao, w_up, dw, w_dn, w_merge)
    return jax.jit(run)


@jax.jit
def pallas_standalone__conformer_family_branchformer__speech_kernel(x, w_q, w_k, w_v, w_ao, w_up, dw, w_dn, w_merge):
    return make()(x, w_q, w_k, w_v, w_ao, w_up, dw, w_dn, w_merge)
```

```python
import contextlib
import math
import jax
import jax.numpy as jnp
from jax import lax
import jax.experimental.pallas as pl
import jax.experimental.pallas.tpu as pltpu

F32 = jnp.float32
BF16 = jnp.bfloat16
U32 = jnp.uint32
LANES = 128
HALO = 16
EPS = 1e-5


def _dot(a, b):
    return jnp.dot(a, b, preferred_element_type=F32)


def _dot_nt(a, b):
    return lax.dot_general(a, b, (((1,), (1,)), ((), ())), preferred_element_type=F32)


def _layernorm(x):
    m = jnp.mean(x, axis=-1, keepdims=True)
    d = x - m
    v = jnp.mean(d * d, axis=-1, keepdims=True)
    return d * lax.rsqrt(v + EPS)


def _gelu(x):
    c = math.sqrt(2.0 / math.pi)
    hx = 0.5 * x
    return hx + hx * jnp.tanh(x * (c + (c * 0.044715) * (x * x)))


def _lhs_combos(a11, a12, a21, a22):
    return [a11 + a22, a21 + a22, a11, a22, a11 + a12, a21 - a11, a12 - a22]


def _lhs_combo(i, quad):
    a, b, sign = ((0, 3, 1), (2, 3, 1), (0, None, 0), (3, None, 0), (0, 1, 1), (2, 0, -1), (1, 3, -1))[i]
    if b is None:
        return quad(a)
    return quad(a) + quad(b) if sign > 0 else quad(a) - quad(b)


def _rhs_combos(b11, b12, b21, b22):
    return [b11 + b22, b11, b12 - b22, b21 - b11, b22, b11 + b12, b21 + b22]


def _even(n, w):
    tot = sum(w)
    cum = [sum(w[:k]) for k in range(len(w) + 1)]
    return [n * cum[k + 1] // tot - n * cum[k] // tot for k in range(len(w))]


ONES = (1, 1, 1, 1, 1, 1, 1)


def make(H=400, CV=10, CG=3, PACK=True, PR=80, US=4, UQ=1, UL=1, porder=(3, 4, 1, 5, 6, 2, 7), flags=None,
         SC=False, DM=1, SR=16, GR=8,
         w_pc=(1, 1, 1, 0, 0, 0, 0), w_se=(1, 1, 1, 0, 0, 0, 0), w_cv=(1, 1, 1, 3, 3, 3, 3), w_cv0=(0, 0, 1, 1, 1, 1, 1),
         w_fin=(1, 1, 1, 1, 0, 0, 0), w_st=(1, 1, 1, 1, 1, 0, 0),
         a_fill=(("k", 7, (1,) * 5), ("s", 1, (1,) * 6), ("g", 12, (1,) * 10), ("u", 19, (1,) * 8), ("n", 7, (1,) * 10))):
    def kernel(x_hbm, wq_hbm, wk_hbm, wv_hbm, wao_hbm, wup_hbm, dw_hbm, wdn_hbm, wm_hbm,
               o_hbm,
               xin, wtmp, wup, dwv, wr, dwb, ql, la, lnext, kr, vr, gs, us, uc, ss, tq, pbuf, acc,
               mrun, mold, lrun, mfin, linv, xst, obuf,
               wsem, xsem, osem):
        B, T, D = xin.shape
        DH = D // 2
        KT = dwv.shape[0]
        BQ = 2 * H
        NQ = T // BQ
        NP = T // 2
        NC = ss.shape[0]
        CK = DH
        NT = D // LANES
        RS = 2 if PACK else 1
        scope = jax.named_scope if SC else (lambda n: contextlib.nullcontext())

        def al(i, m):
            return i if isinstance(i, int) else pl.multiple_of(i, m)

        def st(ref, idx, r0, val):
            n, w = val.shape
            rows = pl.ds(al(r0 // RS, 8), n // RS)
            if PACK:
                v = val.reshape(n // 16, 2, 8, w)
                p = pltpu.pack_elementwise([v[:, 0], v[:, 1]], packed_dtype=BF16)
                ref[(*idx, rows, slice(None))] = p.reshape(n // 2, w)
            else:
                ref[(*idx, rows, slice(None))] = val.astype(BF16)

        def st_nat(ref, idx, r0, val):
            n, w = val.shape
            rows = pl.ds(al(r0 // RS, 8), n // RS)
            v = val.astype(BF16)
            ref[(*idx, rows, slice(None))] = pltpu.bitcast(v, U32) if PACK else v

        def un(v):
            return pltpu.bitcast(v, BF16) if PACK else v

        def ld(ref, idx, r0, n):
            return un(ref[(*idx, pl.ds(al(r0 // RS, 8), n // RS), slice(None))])

        def never(i):
            return lax.broadcasted_iota(jnp.int32, (8, LANES), 1) + i < 0

        def gate(x, tok):
            if tok is None:
                return x
            t, nv = tok
            n, w = x.shape
            reps = (n // 8, w // LANES)
            return jnp.where(jnp.tile(nv, reps), jnp.tile(t, reps), x)

        def stream(gen, steps, weights):
            next(gen)
            return gen, _even(steps, weights)

        def step(gen, tok):
            try:
                gen.send(tok)
            except StopIteration:
                pass

        def drain(gen):
            for _ in gen:
                pass

        def spread(streams, nv, first=0):
            def hook(k, v):
                todo = []
                for gen, counts in streams:
                    cnt = counts[first + k]
                    for n in range(cnt):
                        todo.append(((v.shape[0] // 8) * n // cnt * 8, gen))
                todo.sort(key=lambda p: p[0])
                for r, gen in todo:
                    step(gen, (v[r:r + 8, :LANES], nv))
            return hook

        def x_words(b, j, h, r, cols, n=16):
            w = pltpu.bitcast(xin[b, pl.ds(al(j * BQ + h * H + r, 16), n), cols], U32)
            return [pltpu.unpack_elementwise(w, index=k, packed_dtype=BF16, unpacked_dtype=F32) for k in range(2)]

        def norm_stats(b, j, n=16):
            for r in range(0, H, n):
                for h in range(2):
                    tok = yield
                    v = jnp.concatenate(x_words(b, j, h, r, slice(None), n), axis=0)
                    v = jnp.concatenate([gate(v[:, :LANES], tok), v[:, LANES:]], axis=1)
                    m = jnp.mean(v, axis=-1, keepdims=True)
                    d = v - m
                    rs = lax.rsqrt(jnp.mean(d * d, axis=-1, keepdims=True) + EPS)
                    for k in range(2):
                        rows = slice(k * n // 2, (k + 1) * n // 2)
                        xst[0, h, k, pl.ds(r // 2, n // 2), :] = jnp.broadcast_to(m[rows], (n // 2, LANES))
                        xst[1, h, k, pl.ds(r // 2, n // 2), :] = jnp.broadcast_to(rs[rows], (n // 2, LANES))

        def norm_apply(b, j):
            for r in range(0, H, 16):
                for t in range(DH // LANES):
                    tok = yield
                    q = {}
                    for h in range(2):
                        for k in range(2):
                            q[h, k] = (gate(xst[0, h, k, pl.ds(r // 2, 8), :], tok), xst[1, h, k, pl.ds(r // 2, 8), :])
                    a = [[None] * 4, [None] * 4]
                    for h in range(2):
                        for e in range(2):
                            for k, v in enumerate(x_words(b, j, h, r, pl.ds(e * DH + t * LANES, LANES))):
                                a[k][2 * h + e] = (v - q[h, k][0]) * q[h, k][1]
                    for i, pair in enumerate(zip(_lhs_combos(*a[0]), _lhs_combos(*a[1]))):
                        lnext[i, pl.ds(r // 2, 8), pl.ds(t * LANES, LANES)] = pltpu.pack_elementwise(
                            list(pair), packed_dtype=BF16)

        w_src = (wq_hbm, wk_hbm, wv_hbm, wao_hbm, wdn_hbm, wm_hbm.at[pl.ds(D, D)], wm_hbm.at[pl.ds(0, D)])
        wcopies = [pltpu.make_async_copy(s, wtmp.at[i], wsem.at[i]) for i, s in enumerate(w_src)]
        wup_copy = pltpu.make_async_copy(wup_hbm, wup, wsem.at[7])
        dw_copy = pltpu.make_async_copy(dw_hbm, dwv, wsem.at[8])

        def xcopy(b, j):
            r0 = al(j * BQ, BQ)
            return pltpu.make_async_copy(x_hbm.at[b, pl.ds(r0, BQ)], xin.at[b, pl.ds(r0, BQ)], xsem.at[b * NQ + j])

        def ocopy(b, j):
            r0 = al(j * BQ, BQ)
            return pltpu.make_async_copy(obuf.at[b, pl.ds(r0, BQ)], o_hbm.at[b, pl.ds(r0, BQ)], osem.at[b * NQ + j])

        def even_odd(w):
            u = pltpu.bitcast(w, U32)
            return [pltpu.unpack_elementwise(u, index=k, packed_dtype=BF16, unpacked_dtype=F32) for k in range(2)]

        def st_rhs(ref, r0, idx, halves):
            n = DH // 2
            cs = [_rhs_combos(w[:n, :DH], w[:n, DH:], w[n:, :DH], w[n:, DH:]) for w in halves]
            for i, pair in enumerate(zip(*cs)):
                ref[(*idx, i, pl.ds(r0 // 2, n), slice(None))] = pltpu.pack_elementwise(list(pair), packed_dtype=BF16)

        def product(dot, a, b):
            v = dot(jnp.concatenate(even_odd(a), axis=0).astype(BF16), b)
            return [v[:D // 2], v[D // 2:]]

        for c in (wcopies[0], wcopies[1], wcopies[2], wcopies[3], dw_copy, xcopy(0, 0), wcopies[6], wup_copy):
            c.start()
        zdt = U32 if PACK else BF16
        kr[:, pl.ds(NP // RS, (NC * CK - NP) // RS), :] = jnp.zeros((7, (NC * CK - NP) // RS, DH), zdt)
        vr[:, pl.ds(NP // RS, (NC * CK - NP) // RS), :] = jnp.zeros((7, (NC * CK - NP) // RS, DH), zdt)
        gs[:, pl.ds(0, HALO), :] = jnp.zeros((NT, HALO, LANES), F32)
        gs[:, pl.ds(HALO + T, HALO), :] = jnp.zeros((NT, HALO, LANES), F32)
        mrun[...] = jnp.full(mrun.shape, -jnp.inf, F32)
        mold[...] = jnp.full(mold.shape, -jnp.inf, F32)
        lrun[...] = jnp.zeros(lrun.shape, F32)
        acc[...] = jnp.zeros(acc.shape, F32)
        with scope("w01"):
            wcopies[0].wait()
            wcopies[1].wait()
        scale = float(D) ** -0.5 * math.log2(math.e)
        st_rhs(wr, 0, (2,), [v * scale for v in product(_dot_nt, wtmp[1], wtmp[0])])
        with scope("w23"):
            wcopies[2].wait()
            wcopies[3].wait()
            dw_copy.wait()
        wva = _dot(wtmp[2], wtmp[3]).astype(BF16)
        dwf = dwv[...].astype(F32)
        for t in range(NT):
            for i in range(KT):
                dwb[t, i] = jnp.broadcast_to(dwf[i:i + 1, t * LANES:(t + 1) * LANES], (8, LANES))
        with scope("w45"):
            xcopy(0, 0).wait()
            wcopies[6].wait()
        st_rhs(wr, 0, (3,), product(_dot, wva, wtmp[6]))
        drain(norm_stats(0, 0, PR))
        drain(norm_apply(0, 0))
        with scope("w6"):
            wup_copy.wait()
        wcopies[4].start()
        wcopies[5].start()
        for b in range(B):
            for j in range(NQ):
                if b or j:
                    xcopy(b, j).start()
        st_rhs(wr, 0, (0,), even_odd(wup[:, pl.ds(0, D)]))
        st_rhs(wr, 0, (1,), even_odd(wup[:, pl.ds(D, D)]))

        def strassen(M, tmp, out, fin, hook):
            v = M(4)
            tmp[2] = v
            hook(0, v)
            v = M(1) + tmp[2]
            tmp[0] = v
            hook(1, v)
            v = M(3)
            tmp[0] = tmp[0] + v
            tmp[1] = v
            hook(2, v)
            v = tmp[2] + M(2)
            fin(2, v)
            hook(3, v)
            v = (tmp[0] - out[2]) + M(6)
            fin(3, v)
            hook(4, v)
            v = tmp[1] + M(5)
            fin(1, v)
            hook(5, v)
            v = (tmp[0] - out[1]) + M(7)
            fin(0, v)
            hook(6, v)

        def post_act(j, m):
            buf = ss.at[m]
            dst = gs if m == 1 else us
            for h in (1, 0):
                for r in range(0, H, GR):
                    tok = yield
                    rr = pl.ds(r, GR)
                    v = _gelu(gate(jnp.concatenate([buf[2 * h, rr, :], buf[2 * h + 1, rr, :]], axis=1), tok))
                    if m == 1:
                        v = _layernorm(v)
                    off = j * BQ + h * H + r + (HALO if m == 1 else 0)
                    for t in range(NT):
                        dst[t, pl.ds(al(off, 8), GR), :] = v[:, t * LANES:(t + 1) * LANES]

        def post_kv(j, m):
            buf = ss.at[m]
            dst = kr if m == 2 else vr
            for r in range(0, H, 16):
                for t in range(DH // LANES):
                    tok = yield
                    cols = pl.ds(t * LANES, LANES)
                    q = [gate(buf[k, pl.ds(r, 16), cols], tok) for k in range(4)]
                    cs = _rhs_combos(q[0], q[2], q[1], q[3]) if m == 2 else _rhs_combos(*q)
                    for i, c in enumerate(cs):
                        dst[i, pl.ds(al((j * H + r) // 2, 8), 8), cols] = pltpu.pack_elementwise(
                            [c[:8], c[8:]], packed_dtype=BF16)

        def proj_block(j, nb, nj):
            nv = never(j)
            gens = {"k": (post_kv(j, 2), H // 8), "g": (post_act(j, 1), 2 * H // GR), "u": (post_act(j, 0), 2 * H // GR),
                    "s": (norm_stats(nb, nj), H // 8), "n": (norm_apply(nb, nj), H // 8)}
            streams = [stream(*gens[name], (0,) * pos + tuple(w) + (0,) * (28 - pos - len(w)))
                       for name, pos, w in a_fill]
            for pos, m in enumerate((2, 1, 0, 3)):
                buf = ss.at[m]

                def fin(q, v):
                    buf[q] = v

                def M(i):
                    if pos == 0:
                        v = lnext[i - 1]
                        la[i - 1] = v
                        ql[i - 1, pl.ds(al(j * H // RS, 8), H // RS), :] = v
                    else:
                        v = la[i - 1]
                    return _dot(un(v), ld(wr, (m, i - 1), 0, DH))
                strassen(M, buf, buf, fin, spread(streams, nv, 7 * pos))
            drain(post_kv(j, 3))

        col = lax.broadcasted_iota(jnp.int32, (8, LANES), 1)

        def qk_unit(j, c, valid, hook):
            buf = ss.at[c]

            def fin(q, v):
                buf[q] = v
                hi = jnp.where(jnp.tile(valid, (H // 8, 1)), v[:, LANES:], -jnp.inf)
                mrun[q // 2] = jnp.maximum(mrun[q // 2], jnp.maximum(v[:, :LANES], hi))
            strassen(lambda i: _dot_nt(ld(ql, (i - 1,), j * H, H), ld(kr, (i - 1,), c * CK, CK)),
                     tq, buf, fin, hook)

        def sumexp(c, valid, n):
            vn = jnp.tile(valid, (n // 8, 1))
            for h in (1, 0):
                for r in range(0, H, n):
                    tok = yield
                    rr = pl.ds(r, n)
                    m = gate(mrun[h, rr, :], tok)
                    lo = [jnp.exp2(ss[c, q, rr, pl.ds(0, LANES)] - m) for q in (2 * h, 2 * h + 1)]
                    hi = [jnp.exp2(ss[c, q, rr, pl.ds(LANES, LANES)] - m) for q in (2 * h, 2 * h + 1)]
                    l = lrun[h, rr, :] * jnp.exp2(mold[h, rr, :] - m)
                    lrun[h, rr, :] = (l + (lo[0] + lo[1])) + jnp.where(vn, hi[0] + hi[1], 0.0)
                    mold[h, rr, :] = m

        def finish_stats(n):
            for h in range(2):
                for r in range(0, H, n):
                    tok = yield
                    rr = pl.ds(r, n)
                    m = jnp.max(gate(mrun[h, rr, :], tok), axis=-1, keepdims=True)
                    mfin[h, rr, :] = jnp.broadcast_to(m, (n, LANES))
            for h in range(2):
                for r in range(0, H, n):
                    tok = yield
                    rr = pl.ds(r, n)
                    e = jnp.exp2(gate(mrun[h, rr, :], tok) - mfin[h, rr, :])
                    l = jnp.sum(lrun[h, rr, :] * e, axis=-1, keepdims=True)
                    linv[h, rr, :] = jnp.broadcast_to(1.0 / l, (n, LANES))
                    mrun[h, rr, :] = jnp.full((n, LANES), -jnp.inf, F32)
                    mold[h, rr, :] = jnp.full((n, LANES), -jnp.inf, F32)
                    lrun[h, rr, :] = jnp.zeros((n, LANES), F32)

        def p_combos(c, valid, n):
            vn = jnp.tile(valid, (n // 8, 1))
            for r in range(0, H, n):
                tok = yield
                rr = pl.ds(r, n)
                a = []
                for h in range(2):
                    m = gate(mfin[h, rr, :], tok)
                    mh = jnp.where(vn, m, jnp.inf)
                    il = linv[h, rr, :]
                    for q in (2 * h, 2 * h + 1):
                        p0 = jnp.exp2(ss[c, q, rr, pl.ds(0, LANES)] - m) * il
                        p1 = jnp.exp2(ss[c, q, rr, pl.ds(LANES, LANES)] - mh) * il
                        a.append(jnp.concatenate([p0, p1], axis=1))
                for i, v in enumerate(_lhs_combos(*a)):
                    st(pbuf, (i,), r, v)

        def pv_product(c, i):
            v = _dot(ld(pbuf, (i - 1,), 0, H), ld(vr, (i - 1,), c * CK, CK))
            for n in range(2):
                acc[i - 1, n] = acc[i - 1, n] + v[:, n * LANES:(n + 1) * LANES]
            return v

        def conv(j, c):
            t = c // 2
            base = (c % 2) * H
            r0 = j * BQ + base
            for a in range(0, H // 8, CV):
                n = min(CV, H // 8 - a)
                o = None
                cnt = 0
                win = gs[t, pl.ds(al(r0 + 8 * a, 8), 8 * (n + 4)), :]
                for r in range(8):
                    taps = [i for i in range(KT) if (i + 1) % 8 == r]
                    lo, hi = (taps[0] + 1) // 8, (taps[-1] + 1) // 8
                    g = win[8 * lo + r:8 * lo + r + 8 * (n + hi - lo)].reshape(n + hi - lo, 8, LANES)
                    for i in taps:
                        w = dwb[t, i]
                        if cnt % CG == 0:
                            tok = yield
                            w = gate(w, tok)
                        cnt += 1
                        k = (i + 1) // 8 - lo
                        term = g[k:k + n] * w[None]
                        o = term if o is None else o + term
                rows_in = pl.ds(al(r0 + 8 * a, 8), 8 * n)
                rows_out = pl.ds(al(base + 8 * a, 8), 8 * n)
                uc[t, rows_out, :] = us[t, rows_in, :] * o.reshape(8 * n, LANES)

        def finish_block(b, j):
            def quad(q):
                rr = pl.ds((q // 2) * H, H)
                return jnp.concatenate([uc[2 * (q % 2), rr, :], uc[2 * (q % 2) + 1, rr, :]], axis=1)

            def M(i):
                lhs = _lhs_combo(i - 1, quad).astype(BF16)
                cols = []
                for k in range(2):
                    if PACK:
                        lo = acc[i - 1, k, pl.ds(0, H // 2, stride=2), :].reshape(H // 16, 1, 8, LANES)
                        hi = acc[i - 1, k, pl.ds(1, H // 2, stride=2), :].reshape(H // 16, 1, 8, LANES)
                        cols.append(jnp.concatenate([lo, hi], axis=1).reshape(H, LANES))
                    else:
                        cols.append(acc[i - 1, k])
                    acc[i - 1, k] = jnp.zeros((H, LANES), F32)
                return jnp.concatenate(cols, axis=1) + _dot(lhs, ld(vr, (i - 1,), NC * CK, CK))

            def fin(q, v):
                if q in (1, 2):
                    tq[q] = v
                rows = pl.ds(al(j * BQ + (q // 2) * H, 16), H)
                cols = pl.ds((q % 2) * DH, DH)
                obuf[b, rows, cols] = (xin[b, rows, cols].astype(F32) + v).astype(BF16)
            strassen(M, tq, tq, fin, spread([stream(finish_stats(SR), 4 * H // SR, w_st)], never(j)))

        def unit(j, c, do_qk, do_pv):
            nv = never(c)
            valid = col < NP - LANES - c * CK
            ncv = (-(-(H // 8) // CV)) * (-(-KT // CG))
            if do_qk and do_pv:
                qk_unit(j + 1, c, valid, spread([stream(p_combos(c, valid, SR), H // SR, w_pc)], nv))
                hook = spread([stream(sumexp(c, valid, SR), 2 * H // SR, w_se),
                               stream(conv(j, c), ncv, w_cv)], nv)
            elif do_qk:
                qk_unit(j + 1, c, valid, spread([], nv))
                drain(sumexp(c, valid, SR))
            else:
                drain(p_combos(c, valid, SR))
                hook = spread([stream(conv(j, c), ncv, w_cv0)], nv)
            if do_pv:
                for k, i in enumerate(porder):
                    hook(k, pv_product(c, i))

        def chunks(f, unroll):
            def body(c, _):
                for k in range(unroll):
                    f(c * unroll + k)
                return 0
            lax.fori_loop(0, NC // unroll, body, 0)

        def batch(b, _):
            def pbody(j, _):
                f = b * NQ + j + 1
                nxt = jnp.minimum(f, B * NQ - 1)
                nb, nj = nxt // NQ, nxt % NQ

                @pl.when(f < B * NQ)
                def _():
                    xcopy(nb, nj).wait()
                proj_block(j, nb, nj)
                return 0
            with scope("pA"):
                lax.fori_loop(0, NQ, pbody, 0)
            with scope("Q0"):
                chunks(lambda c: unit(-1, c, True, False), UQ)
            with scope("st0"):
                @pl.when(b == 0)
                def _():
                    wcopies[4].wait()
                    wcopies[5].wait()
                    st_rhs(vr, NC * CK, (), product(_dot, wtmp[4], wtmp[5]))
                    drain(finish_stats(PR))

                @pl.when(b > 0)
                def _():
                    drain(finish_stats(PR))

            def qblock(j, _):
                @pl.when(j < NQ - 1)
                def _():
                    with scope("steady"):
                        chunks(lambda c: unit(j, c, True, True), US)

                @pl.when(j == NQ - 1)
                def _():
                    with scope("last"):
                        chunks(lambda c: unit(j, c, False, True), UL)
                with scope("sb"):
                    finish_block(b, j)
                ocopy(b, j).start()
                return 0
            lax.fori_loop(0, NQ, qblock, 0)
            return 0
        lax.fori_loop(0, B, batch, 0)
        with scope("owait"):
            for b in range(B):
                for j in range(NQ):
                    ocopy(b, j).wait()

    def run(x, w_q, w_k, w_v, w_ao, w_up, dw, w_dn, w_merge):
        B, T, D = x.shape
        KT = dw.shape[0]
        DH = D // 2
        NT = D // LANES
        NP = T // 2
        NC = -(-NP // DH)
        NQ = T // (2 * H)
        RS = 2 if PACK else 1
        PT = U32 if PACK else BF16
        anyspec = pl.BlockSpec(memory_space=pl.ANY)
        return pl.pallas_call(
            kernel,
            out_shape=jax.ShapeDtypeStruct(x.shape, x.dtype),
            in_specs=[anyspec] * 9,
            out_specs=anyspec,
            scratch_shapes=[
                pltpu.VMEM((B, T, D), BF16),
                pltpu.VMEM((7, D, D), BF16),
                pltpu.VMEM((D, 2 * D), BF16),
                pltpu.VMEM((KT, D), BF16),
                pltpu.VMEM((4, 7, DH // RS, DH), PT),
                pltpu.VMEM((NT, KT, 8, LANES), F32),
                pltpu.VMEM((7, NP // RS, DH), PT),
                pltpu.VMEM((7, H // RS, DH), PT),
                pltpu.VMEM((7, H // RS, DH), PT),
                pltpu.VMEM((7, NC * DH // RS, DH), PT),
                pltpu.VMEM((7, (NC + 1) * DH // RS, DH), PT),
                pltpu.VMEM((NT, T + 2 * HALO, LANES), F32),
                pltpu.VMEM((NT, T, LANES), F32),
                pltpu.VMEM((NT, 2 * H, LANES), F32),
                pltpu.VMEM((NC, 4, H, DH), F32),
                pltpu.VMEM((3, H, DH), F32),
                pltpu.VMEM((7, H // RS, DH), PT),
                pltpu.VMEM((7, 2, H, LANES), F32),
                pltpu.VMEM((2, H, LANES), F32),
                pltpu.VMEM((2, H, LANES), F32),
                pltpu.VMEM((2, H, LANES), F32),
                pltpu.VMEM((2, H, LANES), F32),
                pltpu.VMEM((2, H, LANES), F32),
                pltpu.VMEM((2, 2, 2, H // 2, LANES), F32),
                pltpu.VMEM((B, T, D), BF16),
                pltpu.SemaphoreType.DMA((9,)),
                pltpu.SemaphoreType.DMA((B * NQ,)),
                pltpu.SemaphoreType.DMA((B * NQ,)),
            ],
            compiler_params=pltpu.CompilerParams(vmem_limit_bytes=124 * 1024 * 1024, flags=flags),
        )(x, w_q, w_k, w_v, w_ao, w_up, dw, w_dn, w_merge)
    return jax.jit(run)


@jax.jit
def pallas_standalone__conformer_family_branchformer__speech_kernel(x, w_q, w_k, w_v, w_ao, w_up, dw, w_dn, w_merge):
    return make()(x, w_q, w_k, w_v, w_ao, w_up, dw, w_dn, w_merge)
```

```python
import contextlib
import math
import jax
import jax.numpy as jnp
from jax import lax
import jax.experimental.pallas as pl
import jax.experimental.pallas.tpu as pltpu

F32 = jnp.float32
BF16 = jnp.bfloat16
U32 = jnp.uint32
LANES = 128
HALO = 16
EPS = 1e-5


def _dot(a, b):
    return jnp.dot(a, b, preferred_element_type=F32)


def _dot_nt(a, b):
    return lax.dot_general(a, b, (((1,), (1,)), ((), ())), preferred_element_type=F32)


def _layernorm(x):
    m = jnp.mean(x, axis=-1, keepdims=True)
    d = x - m
    v = jnp.mean(d * d, axis=-1, keepdims=True)
    return d * lax.rsqrt(v + EPS)


def _gelu(x):
    c = math.sqrt(2.0 / math.pi)
    hx = 0.5 * x
    return hx + hx * jnp.tanh(x * (c + (c * 0.044715) * (x * x)))


def _lhs_combos(a11, a12, a21, a22):
    return [a11 + a22, a21 + a22, a11, a22, a11 + a12, a21 - a11, a12 - a22]


def _lhs_combo(i, quad):
    a, b, sign = ((0, 3, 1), (2, 3, 1), (0, None, 0), (3, None, 0), (0, 1, 1), (2, 0, -1), (1, 3, -1))[i]
    if b is None:
        return quad(a)
    return quad(a) + quad(b) if sign > 0 else quad(a) - quad(b)


def _rhs_combo(i, quad):
    a, b, sign = ((0, 3, 1), (0, None, 0), (1, 3, -1), (2, 0, -1), (3, None, 0), (0, 1, 1), (2, 3, 1))[i]
    if b is None:
        return quad(a)
    return quad(a) + quad(b) if sign > 0 else quad(a) - quad(b)


def _rhs_combos(b11, b12, b21, b22):
    return [b11 + b22, b11, b12 - b22, b21 - b11, b22, b11 + b12, b21 + b22]


def _even(n, w):
    tot = sum(w)
    cum = [sum(w[:k]) for k in range(len(w) + 1)]
    return [n * cum[k + 1] // tot - n * cum[k] // tot for k in range(len(w))]


ONES = (1, 1, 1, 1, 1, 1, 1)


def make(H=400, CV=10, CG=3, PACK=True, PR=80, flags=None, SC=False, SR=16, GR=8, CU=4,
         w_se=30, w_cv=(3, 1, 2), w_cv0=(1, 1, 1, 1, 0, 1, 0),
         w_fin=(1, 1, 1, 0, 0, 0, 0), w_st=(0, 0, 0, 1, 1, 1, 1), a_order=(2, 1, 3, 0),
         a_fill=(("k", 7, (1,) * 5), ("s", 1, (1,) * 6), ("g", 14, (1,) * 8), ("v", 21, (1,) * 7), ("n", 7, (1,) * 7))):
    def kernel(x_hbm, wq_hbm, wk_hbm, wv_hbm, wao_hbm, wup_hbm, dw_hbm, wdn_hbm, wm_hbm,
               o_hbm,
               xin, wtmp, wup, dwv, wr, dwb, ql, la, lnext, kr, vr, gs, us, uc, ss, sx, tq, pbuf, acc,
               mrun, mold, lrun, mfin, linv, xst, obuf,
               wsem, xsem, osem):
        B, T, D = xin.shape
        DH = D // 2
        KT = dwv.shape[0]
        BQ = 2 * H
        NQ = T // BQ
        NP = T // 2
        NC = ss.shape[0]
        Q = H // 2
        NW = T // 4
        WP = NC * LANES
        CU = pbuf.shape[-1] // LANES
        NT = D // LANES
        RS = 2 if PACK else 1
        scope = jax.named_scope if SC else (lambda n: contextlib.nullcontext())

        def al(i, m):
            return i if isinstance(i, int) else pl.multiple_of(i, m)

        def st(ref, idx, r0, val):
            n, w = val.shape
            rows = pl.ds(al(r0 // RS, 8), n // RS)
            if PACK:
                v = val.reshape(n // 16, 2, 8, w)
                p = pltpu.pack_elementwise([v[:, 0], v[:, 1]], packed_dtype=BF16)
                ref[(*idx, rows, slice(None))] = p.reshape(n // 2, w)
            else:
                ref[(*idx, rows, slice(None))] = val.astype(BF16)

        def st_nat(ref, idx, r0, val):
            n, w = val.shape
            rows = pl.ds(al(r0 // RS, 8), n // RS)
            v = val.astype(BF16)
            ref[(*idx, rows, slice(None))] = pltpu.bitcast(v, U32) if PACK else v

        def un(v):
            return pltpu.bitcast(v, BF16) if PACK else v

        def ld(ref, idx, r0, n):
            return un(ref[(*idx, pl.ds(al(r0 // RS, 8), n // RS), slice(None))])

        def never(i):
            return lax.broadcasted_iota(jnp.int32, (8, LANES), 1) + i < 0

        def gate(x, tok):
            if tok is None:
                return x
            t, nv = tok
            n, w = x.shape
            reps = (n // 8, w // LANES)
            return jnp.where(jnp.tile(nv, reps), jnp.tile(t, reps), x)

        def stream(gen, steps, weights):
            next(gen)
            return gen, _even(steps, weights)

        def step(gen, tok):
            try:
                gen.send(tok)
            except StopIteration:
                pass

        def drain(gen):
            for _ in gen:
                pass

        def spread(streams, nv, first=0):
            def hook(k, v):
                todo = []
                for gen, counts in streams:
                    cnt = counts[first + k]
                    for n in range(cnt):
                        todo.append(((v.shape[0] // 8) * n // cnt * 8, gen))
                todo.sort(key=lambda p: p[0])
                for r, gen in todo:
                    step(gen, (v[r:r + 8, :LANES], nv))
            return hook

        def x_words(b, j, h, r, cols, n=16):
            w = pltpu.bitcast(xin[b, pl.ds(al(j * BQ + h * H + r, 16), n), cols], U32)
            return [pltpu.unpack_elementwise(w, index=k, packed_dtype=BF16, unpacked_dtype=F32) for k in range(2)]

        def norm_stats(b, j, n=16):
            for r in range(0, H, n):
                for h in range(2):
                    tok = yield
                    v = jnp.concatenate(x_words(b, j, h, r, slice(None), n), axis=0)
                    v = jnp.concatenate([gate(v[:, :LANES], tok), v[:, LANES:]], axis=1)
                    m = jnp.mean(v, axis=-1, keepdims=True)
                    d = v - m
                    rs = lax.rsqrt(jnp.mean(d * d, axis=-1, keepdims=True) + EPS)
                    for k in range(2):
                        rows = slice(k * n // 2, (k + 1) * n // 2)
                        xst[0, h, k, pl.ds(r // 2, n // 2), :] = jnp.broadcast_to(m[rows], (n // 2, LANES))
                        xst[1, h, k, pl.ds(r // 2, n // 2), :] = jnp.broadcast_to(rs[rows], (n // 2, LANES))

        def norm_apply(b, j):
            for r in range(0, H, 16):
                for t in range(DH // LANES):
                    tok = yield
                    q = {}
                    for h in range(2):
                        for k in range(2):
                            q[h, k] = (gate(xst[0, h, k, pl.ds(r // 2, 8), :], tok), xst[1, h, k, pl.ds(r // 2, 8), :])
                    a = [[None] * 4, [None] * 4]
                    for h in range(2):
                        for e in range(2):
                            for k, v in enumerate(x_words(b, j, h, r, pl.ds(e * DH + t * LANES, LANES))):
                                a[k][2 * h + e] = (v - q[h, k][0]) * q[h, k][1]
                    for i, pair in enumerate(zip(_lhs_combos(*a[0]), _lhs_combos(*a[1]))):
                        lnext[i, pl.ds(r // 2, 8), pl.ds(t * LANES, LANES)] = pltpu.pack_elementwise(
                            list(pair), packed_dtype=BF16)

        w_src = (wq_hbm, wk_hbm, wv_hbm, wao_hbm, wdn_hbm, wm_hbm.at[pl.ds(D, D)], wm_hbm.at[pl.ds(0, D)])
        wcopies = [pltpu.make_async_copy(s, wtmp.at[i], wsem.at[i]) for i, s in enumerate(w_src)]
        wup_copy = pltpu.make_async_copy(wup_hbm, wup, wsem.at[7])
        dw_copy = pltpu.make_async_copy(dw_hbm, dwv, wsem.at[8])

        def xcopy(b, j):
            r0 = al(j * BQ, BQ)
            return pltpu.make_async_copy(x_hbm.at[b, pl.ds(r0, BQ)], xin.at[b, pl.ds(r0, BQ)], xsem.at[b * NQ + j])

        def ocopy(b, j):
            r0 = al(j * BQ, BQ)
            return pltpu.make_async_copy(obuf.at[b, pl.ds(r0, BQ)], o_hbm.at[b, pl.ds(r0, BQ)], osem.at[b * NQ + j])

        def even_odd(w):
            u = pltpu.bitcast(w, U32)
            return [pltpu.unpack_elementwise(u, index=k, packed_dtype=BF16, unpacked_dtype=F32) for k in range(2)]

        def st_rhs(ref, r0, idx, halves):
            n = DH // 2
            cs = [_rhs_combos(w[:n, :DH], w[:n, DH:], w[n:, :DH], w[n:, DH:]) for w in halves]
            for i, pair in enumerate(zip(*cs)):
                ref[(*idx, i, pl.ds(r0 // 2, n), slice(None))] = pltpu.pack_elementwise(list(pair), packed_dtype=BF16)

        def product(dot, a, b):
            v = dot(jnp.concatenate(even_odd(a), axis=0).astype(BF16), b)
            return [v[:D // 2], v[D // 2:]]

        for c in (wcopies[0], wcopies[1], wcopies[2], wcopies[3], dw_copy, xcopy(0, 0), wcopies[6], wup_copy):
            c.start()
        kr[:, :, pl.ds(NW, WP - NW), :] = jnp.zeros((7, 2, WP - NW, DH), BF16)
        vr[:, pl.ds(NW, WP - NW), :] = jnp.zeros((49, WP - NW, LANES), BF16)
        gs[:, pl.ds(0, HALO), :] = jnp.zeros((NT, HALO, LANES), F32)
        gs[:, pl.ds(HALO + T, HALO), :] = jnp.zeros((NT, HALO, LANES), F32)
        mrun[...] = jnp.full(mrun.shape, -jnp.inf, F32)
        mold[...] = jnp.full(mold.shape, -jnp.inf, F32)
        lrun[...] = jnp.zeros(lrun.shape, F32)
        with scope("w01"):
            wcopies[0].wait()
            wcopies[1].wait()
        scale = float(D) ** -0.5 * math.log2(math.e)
        st_rhs(wr, 0, (2,), [v * scale for v in product(_dot_nt, wtmp[1], wtmp[0])])
        with scope("w23"):
            wcopies[2].wait()
            wcopies[3].wait()
            dw_copy.wait()
        wva = _dot(wtmp[2], wtmp[3]).astype(BF16)
        dwf = dwv[...].astype(F32)
        for t in range(NT):
            for i in range(KT):
                dwb[t, i] = jnp.broadcast_to(dwf[i:i + 1, t * LANES:(t + 1) * LANES], (8, LANES))
        with scope("w45"):
            xcopy(0, 0).wait()
            wcopies[6].wait()
        st_rhs(wr, 0, (3,), product(_dot, wva, wtmp[6]))
        drain(norm_stats(0, 0, PR))
        drain(norm_apply(0, 0))
        with scope("w6"):
            wup_copy.wait()
        wcopies[4].start()
        wcopies[5].start()
        for b in range(B):
            for j in range(NQ):
                if b or j:
                    xcopy(b, j).start()
        st_rhs(wr, 0, (0,), even_odd(wup[:, pl.ds(0, D)]))
        st_rhs(wr, 0, (1,), even_odd(wup[:, pl.ds(D, D)]))

        def strassen(M, tmp, out, fin, hook):
            v = M(4)
            tmp[2] = v
            hook(0, v)
            v = M(1) + tmp[2]
            tmp[0] = v
            hook(1, v)
            v = M(3)
            tmp[0] = tmp[0] + v
            tmp[1] = v
            hook(2, v)
            v = tmp[2] + M(2)
            fin(2, v)
            hook(3, v)
            v = (tmp[0] - out[2]) + M(6)
            fin(3, v)
            hook(4, v)
            v = tmp[1] + M(5)
            fin(1, v)
            hook(5, v)
            v = (tmp[0] - out[1]) + M(7)
            fin(0, v)
            hook(6, v)

        def post_act(j, m):
            buf = ss.at[m]
            dst = gs if m == 1 else us
            for h in (1, 0):
                for r in range(0, H, GR):
                    tok = yield
                    rr = pl.ds(r, GR)
                    v = _gelu(gate(jnp.concatenate([buf[2 * h, rr, :], buf[2 * h + 1, rr, :]], axis=1), tok))
                    if m == 1:
                        v = _layernorm(v)
                    off = j * BQ + h * H + r + (HALO if m == 1 else 0)
                    for t in range(NT):
                        dst[t, pl.ds(al(off, 8), GR), :] = v[:, t * LANES:(t + 1) * LANES]

        def post_k(j):
            buf = ss.at[2]
            for r in range(0, H, 8):
                tok = yield
                q = [buf[k, pl.ds(r, 8), :] for k in range(4)]
                q[0], q[3] = gate(q[0], tok), gate(q[3], tok)
                for i, c in enumerate(_rhs_combos(q[0], q[2], q[1], q[3])):
                    kr[i, r // Q, pl.ds(al(j * Q + r % Q, 8), 8), :] = c.astype(BF16)

        def post_v(j):
            buf = ss.at[3]
            for r in range(0, Q, 8):
                for o in range(7):
                    tok = yield

                    def tile(kq, et):
                        return _rhs_combo(o, lambda q: buf[q, pl.ds(kq * Q + r, 8), pl.ds(et * LANES, LANES)])
                    t = [gate(tile(0, 0), tok), tile(0, 1), tile(1, 0), gate(tile(1, 1), tok)]
                    for i, c in enumerate(_rhs_combos(*t)):
                        vr[7 * o + i, pl.ds(al(j * Q + r, 8), 8), :] = c.astype(BF16)

        def proj_block(j, nb, nj):
            nv = never(j)
            gens = {"k": (post_k(j), H // 8), "v": (post_v(j), 7 * Q // 8),
                    "g": (post_act(j, 1), 2 * H // GR), "u": (post_act(j, 0), 2 * H // GR),
                    "s": (norm_stats(nb, nj), H // 8), "n": (norm_apply(nb, nj), H // 8)}
            streams = [stream(*gens[name], (0,) * pos + tuple(w) + (0,) * (28 - pos - len(w)))
                       for name, pos, w in a_fill]
            for pos, m in enumerate(a_order):
                buf = ss.at[m]

                def fin(q, v):
                    buf[q] = v

                def M(i):
                    if pos == 0:
                        v = lnext[i - 1]
                        la[i - 1] = v
                        ql[i - 1, pl.ds(al(j * H // 2, 8), H // 2), :] = v
                    else:
                        v = la[i - 1]
                    return _dot(un(v), ld(wr, (m, i - 1), 0, DH))
                strassen(M, buf, buf, fin, spread(streams, nv, 7 * pos))
            drain(gens["ugkv"[a_order[-1]]][0])

        col = lax.broadcasted_iota(jnp.int32, (8, LANES), 1)

        def valid_keys(c):
            return col < NW - c * LANES

        def qk_unit(j, c, buf, hook):
            valid = jnp.tile(valid_keys(c), (H // 8, 1))
            keys = pl.ds(al(c * LANES, LANES), LANES)

            def fin(q, v):
                buf[q] = v
                m = jnp.where(valid, jnp.maximum(v[:, :LANES], v[:, LANES:]), -jnp.inf)
                mrun[q // 2] = jnp.maximum(mrun[q // 2], m)

            def M(i):
                rhs = jnp.concatenate([kr[i - 1, 0, keys, :], kr[i - 1, 1, keys, :]], axis=0)
                return _dot_nt(ld(ql, (i - 1,), j * H, H), rhs)
            strassen(M, tq, buf, fin, hook)

        def sumexp(c, buf, n, copy_to=None):
            vn = jnp.tile(valid_keys(c), (n // 8, 1))
            for h in (1, 0):
                for r in range(0, H, n):
                    tok = yield
                    rr = pl.ds(r, n)
                    m = gate(mrun[h, rr, :], tok)
                    e = []
                    for q in (2 * h, 2 * h + 1):
                        for t in range(2):
                            v = buf[q, rr, pl.ds(t * LANES, LANES)]
                            if copy_to is not None:
                                copy_to[q, rr, pl.ds(t * LANES, LANES)] = v
                            e.append(jnp.exp2(v - m))
                    l = lrun[h, rr, :] * jnp.exp2(mold[h, rr, :] - m)
                    lrun[h, rr, :] = l + jnp.where(vn, (e[0] + e[1]) + (e[2] + e[3]), 0.0)
                    mold[h, rr, :] = m

        def finish_stats(n):
            for h in range(2):
                for r in range(0, H, n):
                    tok = yield
                    rr = pl.ds(r, n)
                    m = jnp.max(gate(mrun[h, rr, :], tok), axis=-1, keepdims=True)
                    mfin[h, rr, :] = jnp.broadcast_to(m, (n, LANES))
            for h in range(2):
                for r in range(0, H, n):
                    tok = yield
                    rr = pl.ds(r, n)
                    e = jnp.exp2(gate(mrun[h, rr, :], tok) - mfin[h, rr, :])
                    l = jnp.sum(lrun[h, rr, :] * e, axis=-1, keepdims=True)
                    linv[h, rr, :] = jnp.broadcast_to(1.0 / l, (n, LANES))
                    mrun[h, rr, :] = jnp.full((n, LANES), -jnp.inf, F32)
                    mold[h, rr, :] = jnp.full((n, LANES), -jnp.inf, F32)
                    lrun[h, rr, :] = jnp.zeros((n, LANES), F32)

        def p_combos(c, buf, k, r0=0, r1=Q):
            valid = valid_keys(c)
            for r in range(r0, r1, 8):
                for rq in range(2):
                    tok = yield
                    rr = pl.ds(rq * Q + r, 8)
                    m = [jnp.where(valid, gate(mfin[h, rr, :], tok), jnp.inf) for h in range(2)]
                    il = [linv[h, rr, :] for h in range(2)]
                    for kq in range(2):
                        p = [jnp.exp2(buf[q, rr, pl.ds(kq * LANES, LANES)] - m[q // 2]) * il[q // 2]
                             for q in range(4)]
                        for o, v in enumerate(_lhs_combos(*p)):
                            pbuf[o, 2 * rq + kq, pl.ds(r, 8), pl.ds(k * LANES, LANES)] = v

        def pv_unit(u, hook, r0=0, r1=Q):
            rows = pl.ds(r0, r1 - r0)
            keys = pl.ds(al(u * CU * LANES, LANES), CU * LANES)
            for o in range(7):
                for i in range(7):
                    lhs = _lhs_combo(i, lambda t: pbuf[o, t, rows, :])
                    v = _dot(lhs, vr[7 * o + i, keys, :])
                    acc[7 * o + i, rows, :] = jnp.where(u > 0, acc[7 * o + i, rows, :], 0.0) + v
                    hook(7 * o + i, v)

        def conv(j, c, slot):
            t = c // 2
            base = (c % 2) * H
            r0 = j * BQ + base
            for a in range(0, H // 8, CV):
                n = min(CV, H // 8 - a)
                o = None
                cnt = 0
                win = gs[t, pl.ds(al(r0 + 8 * a, 8), 8 * (n + 4)), :]
                for r in range(8):
                    taps = [i for i in range(KT) if (i + 1) % 8 == r]
                    lo, hi = (taps[0] + 1) // 8, (taps[-1] + 1) // 8
                    g = win[8 * lo + r:8 * lo + r + 8 * (n + hi - lo)].reshape(n + hi - lo, 8, LANES)
                    for i in taps:
                        w = dwb[t, i]
                        if cnt % CG == 0:
                            tok = yield
                            w = gate(w, tok)
                        cnt += 1
                        k = (i + 1) // 8 - lo
                        term = g[k:k + n] * w[None]
                        o = term if o is None else o + term
                rows_in = pl.ds(al(r0 + 8 * a, 8), 8 * n)
                rows_out = pl.ds(al(base + 8 * a, 8), 8 * n)
                uc[slot, t, rows_out, :] = us[t, rows_in, :] * o.reshape(8 * n, LANES)

        def out_combos(m):
            c12 = m[2] + m[4]
            c21 = m[1] + m[3]
            u = m[0] + m[3] + m[2]
            return [(u - c12) + m[6], c12, c21, (u - c21) + m[5]]

        def attn_rows():
            for r in range(0, Q, 8):
                tok = yield
                rr = pl.ds(r, 8)
                inner = []
                for o in range(7):
                    m = [acc[7 * o + i, rr, :] for i in range(7)]
                    m[2], m[3] = gate(m[2], tok), gate(m[3], tok)
                    inner.append(out_combos(m))
                for t in range(4):
                    for q, v in enumerate(out_combos([inner[o][t] for o in range(7)])):
                        sx[q, pl.ds((t // 2) * Q + r, 8), pl.ds((t % 2) * LANES, LANES)] = v

        def finish_block(b, j, slot):
            def quad(q):
                rr = pl.ds((q // 2) * H, H)
                return jnp.concatenate([uc[slot, 2 * (q % 2), rr, :], uc[slot, 2 * (q % 2) + 1, rr, :]], axis=1)

            def M(i):
                return _dot(_lhs_combo(i - 1, quad).astype(BF16), ld(wr, (4, i - 1), 0, DH))

            def fin(q, v):
                if q in (1, 2):
                    tq[q] = v
                rows = pl.ds(al(j * BQ + (q // 2) * H, 16), H)
                cols = pl.ds((q % 2) * DH, DH)
                obuf[b, rows, cols] = (xin[b, rows, cols].astype(F32) + (sx[q] + v)).astype(BF16)
            strassen(M, tq, tq, fin, spread([stream(attn_rows(), Q // 8, w_fin),
                                             stream(finish_stats(SR), 4 * H // SR, w_st)], never(j)))

        def chain(gens):
            for g in gens:
                yield from g

        NCV = (-(-(H // 8) // CV)) * (-(-KT // CG))

        def steady(j, u):
            nv = never(u)
            sv = ss.at[pl.ds(u * CU, CU)]
            order = list(range(1, CU)) + [0]
            nq = 7 * CU
            pc = stream(chain([p_combos(u * CU + k, sv.at[k], k) for k in order]), CU * Q // 4, (1,) * nq + (0,) * 49)
            cv = stream(chain([conv(j, u * CU + k, 0) for k in range(CU)]), CU * NCV,
                        (w_cv[0],) * nq + (w_cv[1],) * w_se + (w_cv[2],) * (49 - w_se))
            se = stream(chain([sumexp(u * CU + k, sv.at[k] if k else sx, SR, None if k else sv.at[0])
                               for k in range(CU)]), CU * 2 * H // SR, (0,) * nq + (1,) * w_se + (0,) * (49 - w_se))
            for k in range(CU):
                qk_unit(j + 1, u * CU + k, sv.at[k] if k else sx, spread([pc, cv], nv, 7 * k))
            pv_unit(u, spread([se, cv], nv, nq))

        def first(c):
            qk_unit(0, c, ss.at[c], spread([stream(conv(NQ - 1, c, 1), NCV, w_cv0)], never(c)))
            drain(sumexp(c, ss.at[c], SR))

        QS = Q // 16 * 8

        def last_rows(u, r0, r1):
            return chain([p_combos(u * CU + k, ss.at[u * CU + k], k, r0, r1) for k in range(CU)])

        def last(u):
            nv = never(u)
            pv_unit(u, spread([stream(last_rows(u, QS, Q), CU * (Q - QS) // 4, (1,) * 49)], nv), 0, QS)
            nu = jnp.minimum(u + 1, NC // CU - 1)
            pv_unit(u, spread([stream(last_rows(nu, 0, QS), CU * QS // 4, (1,) * 49)], nv), QS, Q)

        def loop(n, f):
            def body(i, _):
                f(i)
                return 0
            lax.fori_loop(0, n, body, 0)

        def batch(b):
            def pbody(j):
                f = b * NQ + j + 1
                nxt = jnp.minimum(f, B * NQ - 1)
                nb, nj = nxt // NQ, nxt % NQ

                @pl.when(f < B * NQ)
                def _():
                    xcopy(nb, nj).wait()
                proj_block(j, nb, nj)
            with scope("pA"):
                loop(NQ, pbody)
            with scope("Q0"):
                loop(NC, first)
            with scope("st0"):
                @pl.when(b == 0)
                def _():
                    wcopies[4].wait()
                    wcopies[5].wait()
                    st_rhs(wr, 0, (4,), product(_dot, wtmp[4], wtmp[5]))
                    drain(finish_stats(PR))

                @pl.when(b > 0)
                def _():
                    drain(finish_stats(PR))

            def qblock(j):
                @pl.when(j < NQ - 1)
                def _():
                    with scope("steady"):
                        loop(NC // CU, lambda u: steady(j, u))

                @pl.when(j == NQ - 1)
                def _():
                    with scope("last"):
                        drain(last_rows(0, 0, QS))
                        loop(NC // CU, last)
                with scope("sb"):
                    finish_block(b, j, j // (NQ - 1))
                ocopy(b, j).start()
            loop(NQ, qblock)
        loop(B, batch)
        with scope("owait"):
            for b in range(B):
                for j in range(NQ):
                    ocopy(b, j).wait()

    def run(x, w_q, w_k, w_v, w_ao, w_up, dw, w_dn, w_merge):
        B, T, D = x.shape
        KT = dw.shape[0]
        DH = D // 2
        NT = D // LANES
        NP = T // 2
        NC = -(-NP // DH)
        NQ = T // (2 * H)
        RS = 2 if PACK else 1
        PT = U32 if PACK else BF16
        anyspec = pl.BlockSpec(memory_space=pl.ANY)
        return pl.pallas_call(
            kernel,
            out_shape=jax.ShapeDtypeStruct(x.shape, x.dtype),
            in_specs=[anyspec] * 9,
            out_specs=anyspec,
            scratch_shapes=[
                pltpu.VMEM((B, T, D), BF16),
                pltpu.VMEM((7, D, D), BF16),
                pltpu.VMEM((D, 2 * D), BF16),
                pltpu.VMEM((KT, D), BF16),
                pltpu.VMEM((5, 7, DH // RS, DH), PT),
                pltpu.VMEM((NT, KT, 8, LANES), F32),
                pltpu.VMEM((7, NP // RS, DH), PT),
                pltpu.VMEM((7, H // RS, DH), PT),
                pltpu.VMEM((7, H // RS, DH), PT),
                pltpu.VMEM((7, 2, NC * LANES, DH), BF16),
                pltpu.VMEM((49, NC * LANES, LANES), BF16),
                pltpu.VMEM((NT, T + 2 * HALO, LANES), F32),
                pltpu.VMEM((NT, T, LANES), F32),
                pltpu.VMEM((2, NT, 2 * H, LANES), F32),
                pltpu.VMEM((NC, 4, H, DH), F32),
                pltpu.VMEM((4, H, DH), F32),
                pltpu.VMEM((3, H, DH), F32),
                pltpu.VMEM((7, 4, H // 2, CU * LANES), F32),
                pltpu.VMEM((49, H // 2, LANES), F32),
                pltpu.VMEM((2, H, LANES), F32),
                pltpu.VMEM((2, H, LANES), F32),
                pltpu.VMEM((2, H, LANES), F32),
                pltpu.VMEM((2, H, LANES), F32),
                pltpu.VMEM((2, H, LANES), F32),
                pltpu.VMEM((2, 2, 2, H // 2, LANES), F32),
                pltpu.VMEM((B, T, D), BF16),
                pltpu.SemaphoreType.DMA((9,)),
                pltpu.SemaphoreType.DMA((B * NQ,)),
                pltpu.SemaphoreType.DMA((B * NQ,)),
            ],
            compiler_params=pltpu.CompilerParams(vmem_limit_bytes=124 * 1024 * 1024, flags=flags),
        )(x, w_q, w_k, w_v, w_ao, w_up, dw, w_dn, w_merge)
    return jax.jit(run)


@jax.jit
def pallas_standalone__conformer_family_branchformer__speech_kernel(x, w_q, w_k, w_v, w_ao, w_up, dw, w_dn, w_merge):
    return make()(x, w_q, w_k, w_v, w_ao, w_up, dw, w_dn, w_merge)
```

```python
import contextlib
import math
import jax
import numpy as np
import jax.numpy as jnp
from jax import lax
import jax.experimental.pallas as pl
import jax.experimental.pallas.tpu as pltpu

F32 = jnp.float32
BF16 = jnp.bfloat16
U32 = jnp.uint32
LANES = 128
HALO = 16
EPS = 1e-5
LOWEST = float(np.finfo(np.float32).min)


def _dot(a, b):
    return jnp.dot(a, b, preferred_element_type=F32)


def _dot_nt(a, b):
    return lax.dot_general(a, b, (((1,), (1,)), ((), ())), preferred_element_type=F32)


def _layernorm(x):
    m = jnp.mean(x, axis=-1, keepdims=True)
    d = x - m
    v = jnp.mean(d * d, axis=-1, keepdims=True)
    return d * lax.rsqrt(v + EPS)


def _gelu(x):
    c = math.sqrt(2.0 / math.pi)
    hx = 0.5 * x
    return hx + hx * jnp.tanh(x * (c + (c * 0.044715) * (x * x)))


def _lhs_combos(a11, a12, a21, a22):
    return [a11 + a22, a21 + a22, a11, a22, a11 + a12, a21 - a11, a12 - a22]


def _lhs_combo(i, quad):
    a, b, sign = ((0, 3, 1), (2, 3, 1), (0, None, 0), (3, None, 0), (0, 1, 1), (2, 0, -1), (1, 3, -1))[i]
    if b is None:
        return quad(a)
    return quad(a) + quad(b) if sign > 0 else quad(a) - quad(b)


def _rhs_combo(i, quad):
    a, b, sign = ((0, 3, 1), (0, None, 0), (1, 3, -1), (2, 0, -1), (3, None, 0), (0, 1, 1), (2, 3, 1))[i]
    if b is None:
        return quad(a)
    return quad(a) + quad(b) if sign > 0 else quad(a) - quad(b)


def _rhs_combos(b11, b12, b21, b22):
    return [b11 + b22, b11, b12 - b22, b21 - b11, b22, b11 + b12, b21 + b22]


def _even(n, w):
    tot = sum(w)
    cum = [sum(w[:k]) for k in range(len(w) + 1)]
    return [n * cum[k + 1] // tot - n * cum[k] // tot for k in range(len(w))]


ONES = (1, 1, 1, 1, 1, 1, 1)


def make(H=400, CV=5, CG=3, PACK=True, PR=80, flags=None, SC=False, SR=16, GR=8, CU=4,
         CM=1, SKIP=(), w_se=40, w_cv=(0, 1, 1), w_sq=(4, 3) * 3 + (0,) * 8, se_early=(),
         w_pc=(6, 5, 6, 5, 2, 2) + (3,) * 8, w_s0=(4, 3) * 3 + (0,) * 8, w_cv0=(1,) * 8 + (0, 0, 1, 1, 0, 0),
         w_fin=(1, 1, 1, 0, 0, 0, 0), w_st=(0, 0, 0, 1, 1, 1, 1), a_order=(1, 2, 3, 0),
         a_fill=(("s", 0, (1,) * 4), ("n", 4, (1,) * 4), ("g", 8, (1,) * 8), ("k", 14, (1,) * 8),
                 ("p", 9, (1,) * 12), ("v", 21, (1,) * 7))):
    def kernel(x_hbm, wq_hbm, wk_hbm, wv_hbm, wao_hbm, wup_hbm, dw_hbm, wdn_hbm, wm_hbm,
               o_hbm,
               xin, wtmp, wup, dwv, wr, dwb, ql, la, lnext, kr, vr, gs, us, uc, ss, sx, tq, ti, to, pbuf, acc,
               mrun, lrun, mfin, linv, xst, obuf,
               wsem, xsem, osem):
        B, T, D = xin.shape
        DH = D // 2
        KT = dwv.shape[0]
        BQ = 2 * H
        NQ = T // BQ
        NP = T // 2
        NC = ss.shape[0]
        Q = H // 2
        NW = T // 4
        WP = NC * LANES
        CU = pbuf.shape[-1] // LANES
        NT = D // LANES
        RS = 2 if PACK else 1
        scope = jax.named_scope if SC else (lambda n: contextlib.nullcontext())

        def al(i, m):
            return i if isinstance(i, int) else pl.multiple_of(i, m)

        def st(ref, idx, r0, val):
            n, w = val.shape
            rows = pl.ds(al(r0 // RS, 8), n // RS)
            if PACK:
                v = val.reshape(n // 16, 2, 8, w)
                p = pltpu.pack_elementwise([v[:, 0], v[:, 1]], packed_dtype=BF16)
                ref[(*idx, rows, slice(None))] = p.reshape(n // 2, w)
            else:
                ref[(*idx, rows, slice(None))] = val.astype(BF16)

        def st_nat(ref, idx, r0, val):
            n, w = val.shape
            rows = pl.ds(al(r0 // RS, 8), n // RS)
            v = val.astype(BF16)
            ref[(*idx, rows, slice(None))] = pltpu.bitcast(v, U32) if PACK else v

        def un(v):
            return pltpu.bitcast(v, BF16) if PACK else v

        def ld(ref, idx, r0, n):
            return un(ref[(*idx, pl.ds(al(r0 // RS, 8), n // RS), slice(None))])

        def never(i):
            return lax.broadcasted_iota(jnp.int32, (8, LANES), 1) + i < 0

        def gate(x, tok):
            if tok is None:
                return x
            t, nv = tok
            n, w = x.shape
            reps = (n // 8, w // LANES)
            return jnp.where(jnp.tile(nv, reps), jnp.tile(t, reps), x)

        def stream(gen, steps, weights):
            next(gen)
            return gen, _even(steps, weights)

        def step(gen, tok):
            try:
                gen.send(tok)
            except StopIteration:
                pass

        def drain(gen):
            for _ in gen:
                pass

        def spread(streams, nv, first=0):
            def hook(k, v):
                todo = []
                for gen, counts in streams:
                    cnt = counts[first + k]
                    for n in range(cnt):
                        todo.append(((v.shape[0] // 8) * n // cnt * 8, gen))
                todo.sort(key=lambda p: p[0])
                for r, gen in todo:
                    step(gen, (v[r:r + 8, :LANES], nv))
            return hook

        def x_words(b, j, h, r, cols, n=16):
            w = pltpu.bitcast(xin[b, pl.ds(al(j * BQ + h * H + r, 16), n), cols], U32)
            return [pltpu.unpack_elementwise(w, index=k, packed_dtype=BF16, unpacked_dtype=F32) for k in range(2)]

        def norm_stats(b, j, n=16):
            for r in range(0, H, n):
                for h in range(2):
                    tok = yield
                    v = jnp.concatenate(x_words(b, j, h, r, slice(None), n), axis=0)
                    v = jnp.concatenate([gate(v[:, :LANES], tok), v[:, LANES:]], axis=1)
                    m = jnp.mean(v, axis=-1, keepdims=True)
                    d = v - m
                    rs = lax.rsqrt(jnp.mean(d * d, axis=-1, keepdims=True) + EPS)
                    for k in range(2):
                        rows = slice(k * n // 2, (k + 1) * n // 2)
                        xst[0, h, k, pl.ds(r // 2, n // 2), :] = jnp.broadcast_to(m[rows], (n // 2, LANES))
                        xst[1, h, k, pl.ds(r // 2, n // 2), :] = jnp.broadcast_to(rs[rows], (n // 2, LANES))

        def qslot(b, j):
            return (b * NQ + j) % (NQ + 1)

        def norm_apply(b, j):
            for r in range(0, H, 16):
                for t in range(DH // LANES):
                    tok = yield
                    q = {}
                    for h in range(2):
                        for k in range(2):
                            q[h, k] = (gate(xst[0, h, k, pl.ds(r // 2, 8), :], tok), xst[1, h, k, pl.ds(r // 2, 8), :])
                    a = [[None] * 4, [None] * 4]
                    for h in range(2):
                        for e in range(2):
                            for k, v in enumerate(x_words(b, j, h, r, pl.ds(e * DH + t * LANES, LANES))):
                                a[k][2 * h + e] = (v - q[h, k][0]) * q[h, k][1]
                    for k in range(2):
                        for i, v in enumerate(_lhs_combos(*a[k])):
                            ql[qslot(b, j), i, t, pl.ds(r + 8 * k, 8), :] = v

        def norm_pack(b, j):
            for r in range(0, H, 16):
                tok = yield
                for i in range(7):
                    for t in range(DH // LANES):
                        pair = [ql[qslot(b, j), i, t, pl.ds(r + 8 * k, 8), :] for k in range(2)]
                        if t == 0:
                            pair[0] = gate(pair[0], tok)
                        lnext[i, pl.ds(r // 2, 8), pl.ds(t * LANES, LANES)] = pltpu.pack_elementwise(
                            pair, packed_dtype=BF16)

        w_src = (wq_hbm, wk_hbm, wv_hbm, wao_hbm, wdn_hbm, wm_hbm.at[pl.ds(D, D)], wm_hbm.at[pl.ds(0, D)])
        wcopies = [pltpu.make_async_copy(s, wtmp.at[i], wsem.at[i]) for i, s in enumerate(w_src)]
        wup_copy = pltpu.make_async_copy(wup_hbm, wup, wsem.at[7])
        dw_copy = pltpu.make_async_copy(dw_hbm, dwv, wsem.at[8])

        def xcopy(b, j):
            r0 = al(j * BQ, BQ)
            return pltpu.make_async_copy(x_hbm.at[b, pl.ds(r0, BQ)], xin.at[b, pl.ds(r0, BQ)], xsem.at[b * NQ + j])

        def ocopy(b, j):
            r0 = al(j * BQ, BQ)
            slot = (b * NQ + j) % 2
            return pltpu.make_async_copy(obuf.at[slot], o_hbm.at[b, pl.ds(r0, BQ)], osem.at[slot])

        def even_odd(w):
            u = pltpu.bitcast(w, U32)
            return [pltpu.unpack_elementwise(u, index=k, packed_dtype=BF16, unpacked_dtype=F32) for k in range(2)]

        def st_rhs(ref, r0, idx, halves):
            n = DH // 2
            cs = [_rhs_combos(w[:n, :DH], w[:n, DH:], w[n:, :DH], w[n:, DH:]) for w in halves]
            for i, pair in enumerate(zip(*cs)):
                ref[(*idx, i, pl.ds(r0 // 2, n), slice(None))] = pltpu.pack_elementwise(list(pair), packed_dtype=BF16)

        def product(dot, a, b):
            v = dot(jnp.concatenate(even_odd(a), axis=0).astype(BF16), b)
            return [v[:D // 2], v[D // 2:]]

        for c in (wcopies[0], wcopies[1], wcopies[2], wcopies[3], dw_copy, xcopy(0, 0), wcopies[6], wup_copy):
            c.start()
        kr[:, pl.ds(NW, WP - NW), :] = jnp.zeros((49, WP - NW, LANES), BF16)
        vr[:, pl.ds(NW, WP - NW), :] = jnp.zeros((49, WP - NW, LANES), BF16)
        gs[:, pl.ds(0, HALO), :] = jnp.zeros((NT, HALO, LANES), F32)
        gs[:, pl.ds(HALO + T, HALO), :] = jnp.zeros((NT, HALO, LANES), F32)
        mrun[...] = jnp.full(mrun.shape, LOWEST, F32)
        lrun[...] = jnp.zeros(lrun.shape, F32)
        with scope("w01"):
            wcopies[0].wait()
            wcopies[1].wait()
        scale = float(D) ** -0.5 * math.log2(math.e)
        st_rhs(wr, 0, (2,), [v * scale for v in product(_dot_nt, wtmp[1], wtmp[0])])
        with scope("w23"):
            wcopies[2].wait()
            wcopies[3].wait()
            dw_copy.wait()
        wva = _dot(wtmp[2], wtmp[3]).astype(BF16)
        dwf = dwv[...].astype(F32)
        for t in range(NT):
            for i in range(KT):
                dwb[t, i] = jnp.broadcast_to(dwf[i:i + 1, t * LANES:(t + 1) * LANES], (8, LANES))
        with scope("w45"):
            xcopy(0, 0).wait()
            wcopies[6].wait()
        st_rhs(wr, 0, (3,), product(_dot, wva, wtmp[6]))
        drain(norm_stats(0, 0, PR))
        drain(norm_apply(0, 0))
        drain(norm_pack(0, 0))
        with scope("w6"):
            wup_copy.wait()
        wcopies[4].start()
        wcopies[5].start()
        for b in range(B):
            for j in range(NQ):
                if b or j:
                    xcopy(b, j).start()
        st_rhs(wr, 0, (0,), even_odd(wup[:, pl.ds(0, D)]))
        st_rhs(wr, 0, (1,), even_odd(wup[:, pl.ds(D, D)]))

        def strassen(M, tmp, out, fin, hook):
            v = M(4)
            tmp[2] = v
            hook(0, v)
            v = M(1) + tmp[2]
            tmp[0] = v
            hook(1, v)
            v = M(3)
            tmp[0] = tmp[0] + v
            tmp[1] = v
            hook(2, v)
            v = tmp[2] + M(2)
            fin(2, v)
            hook(3, v)
            v = (tmp[0] - out[2]) + M(6)
            fin(3, v)
            hook(4, v)
            v = tmp[1] + M(5)
            fin(1, v)
            hook(5, v)
            v = (tmp[0] - out[1]) + M(7)
            fin(0, v)
            hook(6, v)

        def post_act(j, m):
            buf = ss.at[m]
            dst = gs if m == 1 else us
            for h in (1, 0):
                for r in range(0, H, GR):
                    tok = yield
                    rr = pl.ds(r, GR)
                    v = _gelu(gate(jnp.concatenate([buf[2 * h, rr, :], buf[2 * h + 1, rr, :]], axis=1), tok))
                    if m == 1:
                        v = _layernorm(v)
                    off = j * BQ + h * H + r + (HALO if m == 1 else 0)
                    for t in range(NT):
                        dst[t, pl.ds(al(off, 8), GR), :] = v[:, t * LANES:(t + 1) * LANES]

        def post_kv(j, m):
            buf = ss.at[m]
            dst = kr if m == 2 else vr
            perm = (0, 2, 1, 3) if m == 2 else (0, 1, 2, 3)
            for r in range(0, Q, 8):
                for o in range(7):
                    tok = yield

                    def tile(t):
                        rows, cols = pl.ds((t // 2) * Q + r, 8), pl.ds((t % 2) * LANES, LANES)
                        return _rhs_combo(o, lambda q: buf[perm[q], rows, cols])
                    t = [gate(tile(0), tok), tile(perm[1]), tile(perm[2]), gate(tile(3), tok)]
                    for i, c in enumerate(_rhs_combos(*t)):
                        dst[7 * o + i, pl.ds(al(j * Q + r, 8), 8), :] = c.astype(BF16)

        def proj_block(j, nb, nj):
            nv = never(j)
            gens = {"k": (post_kv(j, 2), 7 * Q // 8), "v": (post_kv(j, 3), 7 * Q // 8),
                    "g": (post_act(j, 1), 2 * H // GR), "u": (post_act(j, 0), 2 * H // GR),
                    "s": (norm_stats(nb, nj), H // 8), "n": (norm_apply(nb, nj), H // 8),
                    "p": (norm_pack(nb, nj), H // 16)}
            streams = [stream(*gens[name], (0,) * pos + tuple(w) + (0,) * (28 - pos - len(w)))
                       for name, pos, w in a_fill]
            for pos, m in enumerate(a_order):
                buf = ss.at[m]

                def fin(q, v):
                    buf[q] = v

                def M(i):
                    if pos == 0:
                        v = lnext[i - 1]
                        la[i - 1] = v
                    else:
                        v = la[i - 1]
                    return _dot(un(v), ld(wr, (m, i - 1), 0, DH))
                strassen(M, buf, buf, fin, spread(streams, nv, 7 * pos))
            drain(gens["ugkv"[a_order[-1]]][0])

        col = lax.broadcasted_iota(jnp.int32, (8, LANES), 1)

        def valid_keys(c):
            return col < NW - c * LANES

        def qk_unit(slot, c, buf, hook):
            keys = pl.ds(al(c * LANES, LANES), LANES)
            for n, o in enumerate((4, 1, 3, 2, 6, 5, 7)):
                def M(i):
                    return _dot_nt(_lhs_combo(i - 1, lambda t: ql[slot, o - 1, t % 2, pl.ds((t // 2) * Q, Q), :]),
                                   kr[7 * (o - 1) + i - 1, keys, :])

                def emit(t, v):
                    rows, cols = pl.ds((t // 2) * Q, Q), pl.ds((t % 2) * LANES, LANES)

                    def fin(q, w):
                        buf[q, rows, cols] = w
                    if o == 4:
                        to[t, 2] = v
                    elif o == 1:
                        to[t, 0] = to[t, 2] + v
                    elif o == 3:
                        to[t, 0] = to[t, 0] + v
                        to[t, 1] = v
                    elif o == 2:
                        fin(2, to[t, 2] + v)
                    elif o == 6:
                        fin(3, (to[t, 0] - buf[2, rows, cols]) + v)
                    elif o == 5:
                        fin(1, to[t, 1] + v)
                    else:
                        fin(0, (to[t, 0] - buf[1, rows, cols]) + v)
                m3, m5, m2, m4 = M(3), M(5), M(2), M(4)
                ti[0] = m4 - m5
                ti[1] = m3 - m2
                c12 = m3 + m5
                emit(1, c12)
                emit(2, m2 + m4)
                hook(2 * n, c12)
                m1, m6, m7 = M(1), M(6), M(7)
                c22 = (m1 + ti[1]) + m6
                emit(3, c22)
                emit(0, (m1 + ti[0]) + m7)
                hook(2 * n + 1, c22)

        def sumexp(c, buf, n, copy_to=None):
            vn = jnp.tile(valid_keys(c), (n // 8, 1))
            for h in (1, 0):
                for r in range(0, H, n):
                    tok = yield
                    rr = pl.ds(r, n)
                    old = gate(mrun[h, rr, :], tok)
                    v = []
                    for q in (2 * h, 2 * h + 1):
                        for t in range(2):
                            v.append(buf[q, rr, pl.ds(t * LANES, LANES)])
                            if copy_to is not None:
                                copy_to[q, rr, pl.ds(t * LANES, LANES)] = v[-1]
                    top = jnp.maximum(jnp.maximum(v[0], v[1]), jnp.maximum(v[2], v[3]))
                    m = jnp.maximum(old, jnp.where(vn, top, LOWEST))
                    e = [jnp.exp2(x - m) for x in v]
                    l = lrun[h, rr, :] * jnp.exp2(old - m)
                    lrun[h, rr, :] = l + jnp.where(vn, (e[0] + e[1]) + (e[2] + e[3]), 0.0)
                    mrun[h, rr, :] = m

        def finish_stats(n):
            for h in range(2):
                for r in range(0, H, n):
                    tok = yield
                    rr = pl.ds(r, n)
                    m = jnp.max(gate(mrun[h, rr, :], tok), axis=-1, keepdims=True)
                    mfin[h, rr, :] = jnp.broadcast_to(m, (n, LANES))
            for h in range(2):
                for r in range(0, H, n):
                    tok = yield
                    rr = pl.ds(r, n)
                    e = jnp.exp2(gate(mrun[h, rr, :], tok) - mfin[h, rr, :])
                    l = jnp.sum(lrun[h, rr, :] * e, axis=-1, keepdims=True)
                    linv[h, rr, :] = jnp.broadcast_to(1.0 / l, (n, LANES))
                    mrun[h, rr, :] = jnp.full((n, LANES), LOWEST, F32)
                    lrun[h, rr, :] = jnp.zeros((n, LANES), F32)

        def p_combos(c, buf, k, r0=0, r1=Q):
            valid = valid_keys(c)
            for r in range(r0, r1, 8):
                for rq in range(2):
                    tok = yield
                    rr = pl.ds(rq * Q + r, 8)
                    m = [jnp.where(valid, gate(mfin[h, rr, :], tok), jnp.inf) for h in range(2)]
                    il = [linv[h, rr, :] for h in range(2)]
                    for kq in range(2):
                        p = [jnp.exp2(buf[q, rr, pl.ds(kq * LANES, LANES)] - m[q // 2]) * il[q // 2]
                             for q in range(4)]
                        for o, v in enumerate(_lhs_combos(*p)):
                            pbuf[o, 2 * rq + kq, pl.ds(r, 8), pl.ds(k * LANES, LANES)] = v

        def pv_unit(u, hook, r0=0, r1=Q):
            rows = pl.ds(r0, r1 - r0)
            keys = pl.ds(al(u * CU * LANES, LANES), CU * LANES)
            for o in range(7):
                for i in range(7):
                    lhs = _lhs_combo(i, lambda t: pbuf[o, t, rows, :])
                    v = _dot(lhs, vr[7 * o + i, keys, :])
                    acc[7 * o + i, rows, :] = jnp.where(u > 0, acc[7 * o + i, rows, :], 0.0) + v
                    hook(7 * o + i, v)

        def conv(j, t, half, slot):
            base = half * H
            r0 = j * BQ + base
            for a in range(0, H // 8, CV):
                n = min(CV, H // 8 - a)
                o = None
                cnt = 0
                if CM == 2:
                    win = gs[t, pl.ds(al(r0 + 8 * a, 8), 8 * (n + 4)), :]
                for r in range(8):
                    taps = [i for i in range(KT) if (i + 1) % 8 == r]
                    lo, hi = (taps[0] + 1) // 8, (taps[-1] + 1) // 8
                    if CM == 2:
                        g = win[8 * lo + r:8 * lo + r + 8 * (n + hi - lo)]
                    else:
                        g = gs[t, pl.ds(r0 + 8 * (a + lo) + r, 8 * (n + hi - lo)), :]
                    g = g.reshape(n + hi - lo, 8, LANES)
                    for i in taps:
                        w = dwb[t, i]
                        if cnt % CG == 0:
                            tok = yield
                            w = gate(w, tok)
                        cnt += 1
                        k = (i + 1) // 8 - lo
                        term = g[k:k + n] * w[None]
                        o = term if o is None else o + term
                rows_in = pl.ds(al(r0 + 8 * a, 8), 8 * n)
                rows_out = pl.ds(al(base + 8 * a, 8), 8 * n)
                uc[slot, t, rows_out, :] = us[t, rows_in, :] * o.reshape(8 * n, LANES)

        def out_combos(m):
            c12 = m[2] + m[4]
            c21 = m[1] + m[3]
            u = m[0] + m[3] + m[2]
            return [(u - c12) + m[6], c12, c21, (u - c21) + m[5]]

        def attn_rows():
            for r in range(0, Q, 8):
                tok = yield
                rr = pl.ds(r, 8)
                inner = []
                for o in range(7):
                    m = [acc[7 * o + i, rr, :] for i in range(7)]
                    m[2], m[3] = gate(m[2], tok), gate(m[3], tok)
                    inner.append(out_combos(m))
                for t in range(4):
                    for q, v in enumerate(out_combos([inner[o][t] for o in range(7)])):
                        sx[q, pl.ds((t // 2) * Q + r, 8), pl.ds((t % 2) * LANES, LANES)] = v

        def finish_block(b, j, slot, oslot):
            def even_odd_rows(t, h):
                lo = uc[slot, t, pl.ds(h * H, H // 2, stride=2), :].reshape(H // 16, 1, 8, LANES)
                hi = uc[slot, t, pl.ds(h * H + 1, H // 2, stride=2), :].reshape(H // 16, 1, 8, LANES)
                return jnp.concatenate([lo, hi], axis=1).reshape(H, LANES)

            def quad(q):
                return jnp.concatenate([even_odd_rows(2 * (q % 2) + t, q // 2) for t in range(2)], axis=1)

            def M(i):
                return _dot(_lhs_combo(i - 1, quad), ld(wr, (4, i - 1), 0, DH))

            def fin(q, v):
                if q in (1, 2):
                    tq[q] = v
                cols = pl.ds((q % 2) * DH, DH)
                v = (sx[q] + v).reshape(H // 16, 2, 8, DH)
                xs = x_words(b, j, q // 2, 0, cols, H)
                out = pltpu.pack_elementwise([xs[k] + v[:, k].reshape(H // 2, DH) for k in range(2)],
                                             packed_dtype=BF16)
                obuf[oslot, pl.ds((q // 2) * H, H), cols] = pltpu.bitcast(out, BF16)
            strassen(M, tq, tq, fin, spread([stream(attn_rows(), Q // 8, w_fin),
                                             stream(finish_stats(SR), 4 * H // SR, w_st)], never(j)))

        def chain(gens):
            for g in gens:
                yield from g

        NCV = (-(-(H // 8) // CV)) * (-(-KT // CG))

        def steady(b, j, u):
            nv = never(u)
            sv = ss.at[pl.ds(u * CU, CU)]
            order = list(range(1, CU)) + [0]
            nq = 14 * CU
            wq = w_pc
            pc = stream(chain([p_combos(u * CU + k, sv.at[k], k) for k in order]), CU * Q // 4, wq * CU + (0,) * 49)
            cv = stream(chain([conv(j, u * (CU // 2) + k // 2, k % 2, 0) for k in range(CU)]), CU * NCV,
                        (w_cv[0],) * nq + (w_cv[1],) * w_se + (w_cv[2],) * (49 - w_se))
            late = [k for k in range(CU) if k not in se_early]
            se = [stream(sumexp(u * CU + k, sv.at[k], SR), 2 * H // SR, (0,) * (14 * k + 14) + w_sq + (0,) * 100)
                  for k in se_early]
            se.append(stream(chain([sumexp(u * CU + k, sv.at[k] if k else sx, SR, None if k else sv.at[0])
                                    for k in late]), len(late) * 2 * H // SR,
                             (0,) * nq + (1,) * w_se + (0,) * (49 - w_se)))
            for k in range(CU):
                qk_unit(qslot(b, j + 1), u * CU + k, sv.at[k] if k else sx, spread([pc, cv] + se, nv, 14 * k))
            pv_unit(u, spread([cv] + se, nv, nq))

        def first(b, c):
            p = jnp.maximum(c - 1, 0)
            se = stream(sumexp(jnp.where(c > 0, p, NC), ss.at[p], SR), 2 * H // SR, w_s0)
            qk_unit(qslot(b, 0), c, ss.at[c], spread([se], never(c)))

        QS = Q // 16 * 8

        def last_rows(u, r0, r1):
            return chain([p_combos(u * CU + k, ss.at[u * CU + k], k, r0, r1) for k in range(CU)])

        def last(u):
            nv = never(u)
            cv = stream(chain([conv(NQ - 1, u * (CU // 2) + k // 2, k % 2, 0) for k in range(CU)]), CU * NCV, (1,) * 98)
            pv_unit(u, spread([stream(last_rows(u, QS, Q), CU * (Q - QS) // 4, (1,) * 49), cv], nv), 0, QS)
            nu = jnp.minimum(u + 1, NC // CU - 1)
            pv_unit(u, spread([stream(last_rows(nu, 0, QS), CU * QS // 4, (0,) * 49 + (1,) * 49), cv], nv, 49),
                    QS, Q)

        def loop(n, f):
            def body(i, _):
                f(i)
                return 0
            lax.fori_loop(0, n, body, 0)

        def batch(b):
            def pbody(j):
                f = b * NQ + j + 1
                nxt = jnp.minimum(f, B * NQ - 1)
                nb, nj = nxt // NQ, nxt % NQ

                @pl.when(f < B * NQ)
                def _():
                    xcopy(nb, nj).wait()
                proj_block(j, nb, nj)
            with scope("pA"):
                if 'pA' not in SKIP:
                    loop(NQ, pbody)
                else:
                    for jj in range(NQ):
                        pl.when(b * NQ + jj + 1 < B * NQ)(lambda: xcopy((b * NQ + jj + 1) // NQ, (b * NQ + jj + 1) % NQ).wait())
            with scope("Q0"):
                loop(NC, lambda c: first(b, c))
            with scope("st0"):
                @pl.when(b == 0)
                def _():
                    wcopies[4].wait()
                    wcopies[5].wait()
                    st_rhs(wr, 0, (4,), product(_dot, wtmp[4], wtmp[5]))
                    drain(sumexp(NC - 1, ss.at[NC - 1], PR))
                    drain(finish_stats(PR))

                @pl.when(b > 0)
                def _():
                    drain(sumexp(NC - 1, ss.at[NC - 1], PR))
                    drain(finish_stats(PR))

            def qblock(j):
                @pl.when(j < NQ - 1)
                def _():
                    with scope("steady"):
                        if 'steady' not in SKIP:
                            loop(NC // CU, lambda u: steady(b, j, u))

                @pl.when(j == NQ - 1)
                def _():
                    with scope("last"):
                        if 'last' not in SKIP:
                            drain(last_rows(0, 0, QS))
                            loop(NC // CU, last)
                f = b * NQ + j

                @pl.when(f >= 2)
                def _():
                    ocopy((f - 2) // NQ, (f - 2) % NQ).wait()
                with scope("sb"):
                    finish_block(b, j, 0, f % 2)
                ocopy(b, j).start()
            loop(NQ, qblock)
        loop(B, batch)
        with scope("owait"):
            ocopy(B - 1, NQ - 2).wait()
            ocopy(B - 1, NQ - 1).wait()

    def run(x, w_q, w_k, w_v, w_ao, w_up, dw, w_dn, w_merge):
        B, T, D = x.shape
        KT = dw.shape[0]
        DH = D // 2
        NT = D // LANES
        NP = T // 2
        NC = -(-NP // DH)
        NQ = T // (2 * H)
        RS = 2 if PACK else 1
        PT = U32 if PACK else BF16
        anyspec = pl.BlockSpec(memory_space=pl.ANY)
        return pl.pallas_call(
            kernel,
            out_shape=jax.ShapeDtypeStruct(x.shape, x.dtype),
            in_specs=[anyspec] * 9,
            out_specs=anyspec,
            scratch_shapes=[
                pltpu.VMEM((B, T, D), BF16),
                pltpu.VMEM((7, D, D), BF16),
                pltpu.VMEM((D, 2 * D), BF16),
                pltpu.VMEM((KT, D), BF16),
                pltpu.VMEM((5, 7, DH // RS, DH), PT),
                pltpu.VMEM((NT, 32, 8, LANES), F32),
                pltpu.VMEM((NQ + 1, 7, 2, H, LANES), F32),
                pltpu.VMEM((8, H // RS, DH), PT),
                pltpu.VMEM((8, H // RS, DH), PT),
                pltpu.VMEM((49, NC * LANES, LANES), BF16),
                pltpu.VMEM((49, NC * LANES, LANES), BF16),
                pltpu.VMEM((NT, T + 2 * HALO, LANES), F32),
                pltpu.VMEM((NT, T, LANES), F32),
                pltpu.VMEM((1, NT, 2 * H, LANES), F32),
                pltpu.VMEM((NC, 4, H, DH), F32),
                pltpu.VMEM((4, H, DH), F32),
                pltpu.VMEM((3, H, DH), F32),
                pltpu.VMEM((4, H // 2, LANES), F32),
                pltpu.VMEM((4, 3, H // 2, LANES), F32),
                pltpu.VMEM((7, 4, H // 2, CU * LANES), F32),
                pltpu.VMEM((52, H // 2, LANES), F32),
                pltpu.VMEM((2, H, LANES), F32),
                pltpu.VMEM((2, H, LANES), F32),
                pltpu.VMEM((2, H, LANES), F32),
                pltpu.VMEM((2, H, LANES), F32),
                pltpu.VMEM((2, 2, 2, H // 2, LANES), F32),
                pltpu.VMEM((2, 2 * H, D), BF16),
                pltpu.SemaphoreType.DMA((9,)),
                pltpu.SemaphoreType.DMA((B * NQ,)),
                pltpu.SemaphoreType.DMA((2,)),
            ],
            compiler_params=pltpu.CompilerParams(vmem_limit_bytes=124 * 1024 * 1024, flags=flags),
        )(x, w_q, w_k, w_v, w_ao, w_up, dw, w_dn, w_merge)
    return jax.jit(run)


@jax.jit
def pallas_standalone__conformer_family_branchformer__speech_kernel(x, w_q, w_k, w_v, w_ao, w_up, dw, w_dn, w_merge):
    return make()(x, w_q, w_k, w_v, w_ao, w_up, dw, w_dn, w_merge)
```

```python
import contextlib
import math
import jax
import numpy as np
import jax.numpy as jnp
from jax import lax
import jax.experimental.pallas as pl
import jax.experimental.pallas.tpu as pltpu

F32 = jnp.float32
BF16 = jnp.bfloat16
U32 = jnp.uint32
LANES = 128
HALO = 16
EPS = 1e-5
LOWEST = float(np.finfo(np.float32).min)


def _dot(a, b):
    return jnp.dot(a, b, preferred_element_type=F32)


def _dot_nt(a, b):
    return lax.dot_general(a, b, (((1,), (1,)), ((), ())), preferred_element_type=F32)


def _layernorm(x):
    m = jnp.mean(x, axis=-1, keepdims=True)
    d = x - m
    v = jnp.mean(d * d, axis=-1, keepdims=True)
    return d * lax.rsqrt(v + EPS)


def _gelu(x):
    c = math.sqrt(2.0 / math.pi)
    hx = 0.5 * x
    return hx + hx * jnp.tanh(x * (c + (c * 0.044715) * (x * x)))


def _lhs_combos(a11, a12, a21, a22):
    return [a11 + a22, a21 + a22, a11, a22, a11 + a12, a21 - a11, a12 - a22]


def _lhs_combo(i, quad):
    a, b, sign = ((0, 3, 1), (2, 3, 1), (0, None, 0), (3, None, 0), (0, 1, 1), (2, 0, -1), (1, 3, -1))[i]
    if b is None:
        return quad(a)
    return quad(a) + quad(b) if sign > 0 else quad(a) - quad(b)


def _rhs_combo(i, quad):
    a, b, sign = ((0, 3, 1), (0, None, 0), (1, 3, -1), (2, 0, -1), (3, None, 0), (0, 1, 1), (2, 3, 1))[i]
    if b is None:
        return quad(a)
    return quad(a) + quad(b) if sign > 0 else quad(a) - quad(b)


def _rhs_combos(b11, b12, b21, b22):
    return [b11 + b22, b11, b12 - b22, b21 - b11, b22, b11 + b12, b21 + b22]


def _even(n, w):
    tot = sum(w)
    cum = [sum(w[:k]) for k in range(len(w) + 1)]
    return [n * cum[k + 1] // tot - n * cum[k] // tot for k in range(len(w))]


ONES = (1, 1, 1, 1, 1, 1, 1)


def make(H=400, CV=5, CG=3, PACK=True, PR=80, flags=None, SC=False, SR=8, GR=8, CU=4,
         CM=1, SKIP=(), UQ=2, QS=96, PF=2, w_se=40, w_cv=(0, 1, 1), w_sq=(4, 3) * 3 + (0,) * 8, se_early=(),
         w_pc=(5, 4, 5, 4, 2, 2) + (4, 3) * 4, w_s0=(4, 3) * 3 + (0,) * 8, w_cv0=(1,) * 8 + (0, 0, 1, 1, 0, 0),
         w_fin=(1, 1, 1, 0, 0, 0, 0), w_st=(0, 0, 0, 1, 1, 1, 1), a_order=(1, 2, 3, 0),
         a_fill=(("s", 0, (1,) * 4), ("n", 4, (1,) * 4), ("g", 8, (1,) * 8), ("k", 14, (1,) * 8),
                 ("p", 9, (1,) * 12), ("v", 21, (1,) * 7))):
    def kernel(x_hbm, wq_hbm, wk_hbm, wv_hbm, wao_hbm, wup_hbm, dw_hbm, wdn_hbm, wm_hbm,
               o_hbm,
               xin, wtmp, wup, dwv, wr, dwb, ql, la, lnext, kr, vr, gs, us, uc, ss, sx, tq, ti, to, pbuf, acc,
               mrun, lrun, mfin, linv, xst, obuf,
               wsem, xsem, osem):
        B, T, D = xin.shape
        DH = D // 2
        KT = dwv.shape[0]
        BQ = 2 * H
        NQ = T // BQ
        NP = T // 2
        NC = ss.shape[0]
        Q = H // 2
        QM = Q // 16 * 16
        WP = NC * LANES
        CU = pbuf.shape[-1] // LANES
        NT = D // LANES
        RS = 2 if PACK else 1
        scope = jax.named_scope if SC else (lambda n: contextlib.nullcontext())

        def al(i, m):
            return i if isinstance(i, int) else pl.multiple_of(i, m)

        def st(ref, idx, r0, val):
            n, w = val.shape
            rows = pl.ds(al(r0 // RS, 8), n // RS)
            if PACK:
                v = val.reshape(n // 16, 2, 8, w)
                p = pltpu.pack_elementwise([v[:, 0], v[:, 1]], packed_dtype=BF16)
                ref[(*idx, rows, slice(None))] = p.reshape(n // 2, w)
            else:
                ref[(*idx, rows, slice(None))] = val.astype(BF16)

        def st_nat(ref, idx, r0, val):
            n, w = val.shape
            rows = pl.ds(al(r0 // RS, 8), n // RS)
            v = val.astype(BF16)
            ref[(*idx, rows, slice(None))] = pltpu.bitcast(v, U32) if PACK else v

        def un(v):
            return pltpu.bitcast(v, BF16) if PACK else v

        def ld(ref, idx, r0, n):
            return un(ref[(*idx, pl.ds(al(r0 // RS, 8), n // RS), slice(None))])

        def never(i):
            return lax.broadcasted_iota(jnp.int32, (8, LANES), 1) + i < 0

        def gate(x, tok):
            if tok is None:
                return x
            t, nv = tok
            n, w = x.shape
            reps = (n // 8, w // LANES)
            return jnp.where(jnp.tile(nv, reps), jnp.tile(t, reps), x)

        def stream(gen, steps, weights):
            next(gen)
            return gen, _even(steps, weights)

        def step(gen, tok):
            try:
                gen.send(tok)
            except StopIteration:
                pass

        def drain(gen):
            for _ in gen:
                pass

        def spread(streams, nv, first=0):
            def hook(k, v):
                todo = []
                for gen, counts in streams:
                    cnt = counts[first + k]
                    for n in range(cnt):
                        todo.append(((v.shape[0] // 8) * n // cnt * 8, gen))
                todo.sort(key=lambda p: p[0])
                for r, gen in todo:
                    step(gen, (v[r:r + 8, :LANES], nv))
            return hook

        def x_words(b, j, h, r, cols, n=16):
            w = pltpu.bitcast(xin[b, pl.ds(al(j * BQ + h * H + r, 16), n), cols], U32)
            return [pltpu.unpack_elementwise(w, index=k, packed_dtype=BF16, unpacked_dtype=F32) for k in range(2)]

        def norm_stats(b, j, n=16):
            for r in range(0, H, n):
                for h in range(2):
                    tok = yield
                    v = jnp.concatenate(x_words(b, j, h, r, slice(None), n), axis=0)
                    v = jnp.concatenate([gate(v[:, :LANES], tok), v[:, LANES:]], axis=1)
                    m = jnp.mean(v, axis=-1, keepdims=True)
                    d = v - m
                    rs = lax.rsqrt(jnp.mean(d * d, axis=-1, keepdims=True) + EPS)
                    for k in range(2):
                        rows = slice(k * n // 2, (k + 1) * n // 2)
                        xst[0, h, k, pl.ds(r // 2, n // 2), :] = jnp.broadcast_to(m[rows], (n // 2, LANES))
                        xst[1, h, k, pl.ds(r // 2, n // 2), :] = jnp.broadcast_to(rs[rows], (n // 2, LANES))

        def qslot(b, j):
            return (b * NQ + j) % (NQ + 1)

        def norm_apply(b, j):
            for r in range(0, H, 16):
                for t in range(DH // LANES):
                    tok = yield
                    q = {}
                    for h in range(2):
                        for k in range(2):
                            q[h, k] = (gate(xst[0, h, k, pl.ds(r // 2, 8), :], tok), xst[1, h, k, pl.ds(r // 2, 8), :])
                    a = [[None] * 4, [None] * 4]
                    for h in range(2):
                        for e in range(2):
                            for k, v in enumerate(x_words(b, j, h, r, pl.ds(e * DH + t * LANES, LANES))):
                                a[k][2 * h + e] = (v - q[h, k][0]) * q[h, k][1]
                    for k in range(2):
                        for i, v in enumerate(_lhs_combos(*a[k])):
                            ql[qslot(b, j), i, t, pl.ds(r + 8 * k, 8), :] = v

        def norm_pack(b, j):
            for r in range(0, H, 16):
                tok = yield
                for i in range(7):
                    for t in range(DH // LANES):
                        pair = [ql[qslot(b, j), i, t, pl.ds(r + 8 * k, 8), :] for k in range(2)]
                        if t == 0:
                            pair[0] = gate(pair[0], tok)
                        lnext[i, pl.ds(r // 2, 8), pl.ds(t * LANES, LANES)] = pltpu.pack_elementwise(
                            pair, packed_dtype=BF16)

        w_src = (wq_hbm, wk_hbm, wv_hbm, wao_hbm, wdn_hbm, wm_hbm.at[pl.ds(D, D)], wm_hbm.at[pl.ds(0, D)])
        wcopies = [pltpu.make_async_copy(s, wtmp.at[i], wsem.at[i]) for i, s in enumerate(w_src)]
        wup_copy = pltpu.make_async_copy(wup_hbm, wup, wsem.at[7])
        dw_copy = pltpu.make_async_copy(dw_hbm, dwv, wsem.at[8])

        def xcopy(b, j):
            r0 = al(j * BQ, BQ)
            return pltpu.make_async_copy(x_hbm.at[b, pl.ds(r0, BQ)], xin.at[b, pl.ds(r0, BQ)], xsem.at[b * NQ + j])

        def ocopy(b, j, h):
            slot = (b * NQ + j) % 2
            return pltpu.make_async_copy(obuf.at[slot, pl.ds(h * H, H)], o_hbm.at[b, pl.ds(al(j * BQ + h * H, H), H)],
                                         osem.at[2 * slot + h])

        def halves(u):
            return [pltpu.unpack_elementwise(u, index=k, packed_dtype=BF16, unpacked_dtype=F32) for k in range(2)]

        def even_odd(w):
            return halves(pltpu.bitcast(w, U32))

        def st_rhs(ref, r0, idx, halves):
            n = DH // 2
            cs = [_rhs_combos(w[:n, :DH], w[:n, DH:], w[n:, :DH], w[n:, DH:]) for w in halves]
            for i, pair in enumerate(zip(*cs)):
                ref[(*idx, i, pl.ds(r0 // 2, n), slice(None))] = pltpu.pack_elementwise(list(pair), packed_dtype=BF16)

        def product(dot, a, b):
            v = dot(jnp.concatenate(even_odd(a), axis=0).astype(BF16), b)
            return [v[:D // 2], v[D // 2:]]

        for c in (wcopies[0], wcopies[1], wcopies[2], wcopies[3], dw_copy, xcopy(0, 0), wcopies[6], wup_copy):
            c.start()
        kr[:, pl.ds(QM * NQ // 2, (WP - QM * NQ) // 2), :] = jnp.zeros((49, (WP - QM * NQ) // 2, LANES), U32)
        vr[:, pl.ds(QM * NQ // 2, (WP - QM * NQ) // 2), :] = jnp.zeros((49, (WP - QM * NQ) // 2, LANES), U32)
        gs[:, pl.ds(0, HALO), :] = jnp.zeros((NT, HALO, LANES), F32)
        gs[:, pl.ds(HALO + T, HALO), :] = jnp.zeros((NT, HALO, LANES), F32)
        mrun[...] = jnp.full(mrun.shape, LOWEST, F32)
        lrun[...] = jnp.zeros(lrun.shape, F32)
        with scope("w01"):
            wcopies[0].wait()
            wcopies[1].wait()
        scale = float(D) ** -0.5 * math.log2(math.e)
        st_rhs(wr, 0, (2,), [v * scale for v in product(_dot_nt, wtmp[1], wtmp[0])])
        with scope("w23"):
            wcopies[2].wait()
            wcopies[3].wait()
            dw_copy.wait()
        wva = _dot(wtmp[2], wtmp[3]).astype(BF16)
        dwf = dwv[...].astype(F32)
        for t in range(NT):
            for i in range(KT):
                dwb[t, i] = jnp.broadcast_to(dwf[i:i + 1, t * LANES:(t + 1) * LANES], (8, LANES))
        with scope("w45"):
            xcopy(0, 0).wait()
            wcopies[6].wait()
        st_rhs(wr, 0, (3,), product(_dot, wva, wtmp[6]))
        drain(norm_stats(0, 0, PR))
        drain(norm_apply(0, 0))
        drain(norm_pack(0, 0))
        with scope("w6"):
            wup_copy.wait()
        wcopies[4].start()
        wcopies[5].start()
        for b in range(B):
            for j in range(NQ):
                if b or j:
                    xcopy(b, j).start()
        st_rhs(wr, 0, (0,), even_odd(wup[:, pl.ds(0, D)]))
        st_rhs(wr, 0, (1,), even_odd(wup[:, pl.ds(D, D)]))

        def strassen(M, tmp, out, fin, hook):
            v = M(4)
            tmp[2] = v
            hook(0, v)
            v = M(1) + tmp[2]
            tmp[0] = v
            hook(1, v)
            v = M(3)
            tmp[0] = tmp[0] + v
            tmp[1] = v
            hook(2, v)
            v = tmp[2] + M(2)
            fin(2, v)
            hook(3, v)
            v = (tmp[0] - out[2]) + M(6)
            fin(3, v)
            hook(4, v)
            v = tmp[1] + M(5)
            fin(1, v)
            hook(5, v)
            v = (tmp[0] - out[1]) + M(7)
            fin(0, v)
            hook(6, v)

        def post_act(j, m):
            buf = ss.at[m]
            dst = gs if m == 1 else us
            for h in (1, 0):
                for r in range(0, H, GR):
                    tok = yield
                    rr = pl.ds(r, GR)
                    v = _gelu(gate(jnp.concatenate([buf[2 * h, rr, :], buf[2 * h + 1, rr, :]], axis=1), tok))
                    if m == 1:
                        v = _layernorm(v)
                    off = j * BQ + h * H + r + (HALO if m == 1 else 0)
                    for t in range(NT):
                        dst[t, pl.ds(al(off, 8), GR), :] = v[:, t * LANES:(t + 1) * LANES]

        def post_kv(j, m):
            buf = ss.at[m]
            dst = kr if m == 2 else vr
            perm = (0, 2, 1, 3) if m == 2 else (0, 1, 2, 3)
            for r in range(0, Q, 16):
                n = min(16, Q - r)
                for o in range(7):
                    tok = yield

                    def tile(t):
                        rows, cols = pl.ds((t // 2) * Q + r, n), pl.ds((t % 2) * LANES, LANES)
                        return _rhs_combo(o, lambda q: buf[perm[q], rows, cols])
                    t = [gate(tile(0), tok), tile(perm[1]), tile(perm[2]), gate(tile(3), tok)]
                    for i, c in enumerate(_rhs_combos(*t)):
                        if n == 16:
                            rows, pair = pl.ds(al((j * QM + r) // 2, 8), 8), [c[:8], c[8:]]
                        else:
                            rows = pl.ds(al(NQ * QM // 2 + 8 * (j // 2), 8), 8)
                            old = halves(dst[7 * o + i, rows, :])
                            pair = [jnp.where(j % 2 == 0, c, old[0]), jnp.where(j % 2 == 0, old[1], c)]
                        dst[7 * o + i, rows, :] = pltpu.pack_elementwise(pair, packed_dtype=BF16)

        def proj_block(j, nb, nj):
            nv = never(j)
            gens = {"k": (post_kv(j, 2), 7 * -(-Q // 16)), "v": (post_kv(j, 3), 7 * -(-Q // 16)),
                    "g": (post_act(j, 1), 2 * H // GR), "u": (post_act(j, 0), 2 * H // GR),
                    "s": (norm_stats(nb, nj), H // 8), "n": (norm_apply(nb, nj), H // 8),
                    "p": (norm_pack(nb, nj), H // 16)}
            streams = [stream(*gens[name], (0,) * pos + tuple(w) + (0,) * (28 - pos - len(w)))
                       for name, pos, w in a_fill]
            for pos, m in enumerate(a_order):
                buf = ss.at[m]

                def fin(q, v):
                    buf[q] = v

                def M(i):
                    if pos == 0:
                        v = lnext[i - 1]
                        la[i - 1] = v
                    else:
                        v = la[i - 1]
                    return _dot(un(v), ld(wr, (m, i - 1), 0, DH))
                strassen(M, buf, buf, fin, spread(streams, nv, 7 * pos))
            drain(gens["ugkv"[a_order[-1]]][0])

        col = lax.broadcasted_iota(jnp.int32, (8, LANES), 1)

        def valid_keys(c):
            w = col + c * LANES
            full = NQ * QM + 16 * (NQ // 2)
            return (w < full) | ((w < full + 16 * (NQ % 2)) & (w % 2 == 0))

        def qk_unit(slot, c, buf, hook):
            for n, o in enumerate((4, 1, 3, 2, 6, 5, 7)):
                def M(i):
                    return _dot_nt(_lhs_combo(i - 1, lambda t: ql[slot, o - 1, t % 2, pl.ds((t // 2) * Q, Q), :]),
                                   ld(kr, (7 * (o - 1) + i - 1,), c * LANES, LANES))

                def emit(t, v):
                    rows, cols = pl.ds((t // 2) * Q, Q), pl.ds((t % 2) * LANES, LANES)

                    def fin(q, w):
                        buf[q, rows, cols] = w
                    if o == 4:
                        to[t, 2] = v
                    elif o == 1:
                        to[t, 0] = to[t, 2] + v
                    elif o == 3:
                        to[t, 0] = to[t, 0] + v
                        to[t, 1] = v
                    elif o == 2:
                        fin(2, to[t, 2] + v)
                    elif o == 6:
                        fin(3, (to[t, 0] - buf[2, rows, cols]) + v)
                    elif o == 5:
                        fin(1, to[t, 1] + v)
                    else:
                        fin(0, (to[t, 0] - buf[1, rows, cols]) + v)
                m3, m5, m2, m4 = M(3), M(5), M(2), M(4)
                ti[0] = m4 - m5
                ti[1] = m3 - m2
                c12 = m3 + m5
                emit(1, c12)
                emit(2, m2 + m4)
                hook(2 * n, c12)
                m1, m6, m7 = M(1), M(6), M(7)
                c22 = (m1 + ti[1]) + m6
                emit(3, c22)
                emit(0, (m1 + ti[0]) + m7)
                hook(2 * n + 1, c22)

        def sumexp(c, buf, n, copy_to=None):
            vn = jnp.tile(valid_keys(c), (n // 8, 1))
            for h in (1, 0):
                for r in range(0, H, n):
                    tok = yield
                    rr = pl.ds(r, n)
                    old = gate(mrun[h, rr, :], tok)
                    v = []
                    for q in (2 * h, 2 * h + 1):
                        for t in range(2):
                            v.append(buf[q, rr, pl.ds(t * LANES, LANES)])
                            if copy_to is not None:
                                copy_to[q, rr, pl.ds(t * LANES, LANES)] = v[-1]
                    top = jnp.maximum(jnp.maximum(v[0], v[1]), jnp.maximum(v[2], v[3]))
                    m = jnp.maximum(old, jnp.where(vn, top, LOWEST))
                    e = [jnp.exp2(x - m) for x in v]
                    l = lrun[h, rr, :] * jnp.exp2(old - m)
                    lrun[h, rr, :] = l + jnp.where(vn, (e[0] + e[1]) + (e[2] + e[3]), 0.0)
                    mrun[h, rr, :] = m

        def finish_stats(n):
            for h in range(2):
                for r in range(0, H, n):
                    tok = yield
                    rr = pl.ds(r, n)
                    m = jnp.max(gate(mrun[h, rr, :], tok), axis=-1, keepdims=True)
                    mfin[h, rr, :] = jnp.broadcast_to(m, (n, LANES))
            for h in range(2):
                for r in range(0, H, n):
                    tok = yield
                    rr = pl.ds(r, n)
                    e = jnp.exp2(gate(mrun[h, rr, :], tok) - mfin[h, rr, :])
                    l = jnp.sum(lrun[h, rr, :] * e, axis=-1, keepdims=True)
                    linv[h, rr, :] = jnp.broadcast_to(pl.reciprocal(l, full_range=False), (n, LANES))
                    mrun[h, rr, :] = jnp.full((n, LANES), LOWEST, F32)
                    lrun[h, rr, :] = jnp.zeros((n, LANES), F32)

        def p_combos(c, buf, k, r0=0, r1=Q):
            valid = valid_keys(c)
            for r in range(r0, r1, 8):
                for rq in range(2):
                    rr = pl.ds(rq * Q + r, 8)
                    for kq in range(2):
                        if kq == 0 or PF == 2:
                            tok = yield
                            top = gate(jnp.full((8, LANES), jnp.inf, F32), tok)
                            m = [jnp.where(valid, mfin[h, rr, :], top) for h in range(2)]
                            il = [linv[h, rr, :] for h in range(2)]
                        p = [jnp.exp2(buf[q, rr, pl.ds(kq * LANES, LANES)] - m[q // 2]) * il[q // 2]
                             for q in range(4)]
                        for o, v in enumerate(_lhs_combos(*p)):
                            pbuf[o, 2 * rq + kq, pl.ds(r, 8), pl.ds(k * LANES, LANES)] = v

        def pv_unit(u, hook, r0=0, r1=Q):
            rows = pl.ds(r0, r1 - r0)
            for o in range(7):
                for i in range(7):
                    lhs = _lhs_combo(i, lambda t: pbuf[o, t, rows, :])
                    v = _dot(lhs, ld(vr, (7 * o + i,), u * CU * LANES, CU * LANES))
                    acc[7 * o + i, rows, :] = jnp.where(u > 0, acc[7 * o + i, rows, :], 0.0) + v
                    hook(7 * o + i, v)

        def conv(j, t, half, slot):
            base = half * H
            r0 = j * BQ + base
            for a in range(0, H // 8, CV):
                n = min(CV, H // 8 - a)
                o = None
                cnt = 0
                if CM == 2:
                    win = gs[t, pl.ds(al(r0 + 8 * a, 8), 8 * (n + 4)), :]
                for r in range(8):
                    taps = [i for i in range(KT) if (i + 1) % 8 == r]
                    lo, hi = (taps[0] + 1) // 8, (taps[-1] + 1) // 8
                    if CM == 2:
                        g = win[8 * lo + r:8 * lo + r + 8 * (n + hi - lo)]
                    else:
                        g = gs[t, pl.ds(r0 + 8 * (a + lo) + r, 8 * (n + hi - lo)), :]
                    g = g.reshape(n + hi - lo, 8, LANES)
                    for i in taps:
                        w = dwb[t, i]
                        if cnt % CG == 0:
                            tok = yield
                            w = gate(w, tok)
                        cnt += 1
                        k = (i + 1) // 8 - lo
                        term = g[k:k + n] * w[None]
                        o = term if o is None else o + term
                rows_in = pl.ds(al(r0 + 8 * a, 8), 8 * n)
                rows_out = pl.ds(al(base + 8 * a, 8), 8 * n)
                uc[slot, t, rows_out, :] = us[t, rows_in, :] * o.reshape(8 * n, LANES)

        def out_combos(m):
            c12 = m[2] + m[4]
            c21 = m[1] + m[3]
            u = m[0] + m[3] + m[2]
            return [(u - c12) + m[6], c12, c21, (u - c21) + m[5]]

        def attn_rows():
            for r in range(0, Q, 8):
                tok = yield
                rr = pl.ds(r, 8)
                inner = []
                for o in range(7):
                    m = [acc[7 * o + i, rr, :] for i in range(7)]
                    m[2], m[3] = gate(m[2], tok), gate(m[3], tok)
                    inner.append(out_combos(m))
                for t in range(4):
                    for q, v in enumerate(out_combos([inner[o][t] for o in range(7)])):
                        sx[q, pl.ds((t // 2) * Q + r, 8), pl.ds((t % 2) * LANES, LANES)] = v

        def finish_block(b, j, slot, oslot):
            def even_odd_rows(t, h):
                lo = uc[slot, t, pl.ds(h * H, H // 2, stride=2), :].reshape(H // 16, 1, 8, LANES)
                hi = uc[slot, t, pl.ds(h * H + 1, H // 2, stride=2), :].reshape(H // 16, 1, 8, LANES)
                return jnp.concatenate([lo, hi], axis=1).reshape(H, LANES)

            def quad(q):
                return jnp.concatenate([even_odd_rows(2 * (q % 2) + t, q // 2) for t in range(2)], axis=1)

            def M(i):
                return _dot(_lhs_combo(i - 1, quad), ld(wr, (4, i - 1), 0, DH))

            def fin(q, v):
                if q in (1, 2):
                    tq[q] = v
                cols = pl.ds((q % 2) * DH, DH)
                v = (sx[q] + v).reshape(H // 16, 2, 8, DH)
                xs = x_words(b, j, q // 2, 0, cols, H)
                out = pltpu.pack_elementwise([xs[k] + v[:, k].reshape(H // 2, DH) for k in range(2)],
                                             packed_dtype=BF16)
                obuf[oslot, pl.ds((q // 2) * H, H), cols] = pltpu.bitcast(out, BF16)
                if q in (0, 3):
                    ocopy(b, j, q // 2).start()
            strassen(M, tq, tq, fin, spread([stream(attn_rows(), Q // 8, w_fin),
                                             stream(finish_stats(SR), 4 * H // SR, w_st)], never(j)))

        def chain(gens):
            for g in gens:
                yield from g

        NCV = (-(-(H // 8) // CV)) * (-(-KT // CG))

        def steady(b, j, u):
            nv = never(u)
            sv = ss.at[pl.ds(u * CU, CU)]
            order = list(range(1, CU)) + [0]
            nq = 14 * CU
            wq = w_pc
            pc = stream(chain([p_combos(u * CU + k, sv.at[k], k) for k in order]), PF * CU * Q // 4, wq * CU + (0,) * 49)
            cv = stream(chain([conv(j, u * (CU // 2) + k // 2, k % 2, 0) for k in range(CU)]), CU * NCV,
                        (w_cv[0],) * nq + (w_cv[1],) * w_se + (w_cv[2],) * (49 - w_se))
            late = [k for k in range(CU) if k not in se_early]
            se = [stream(sumexp(u * CU + k, sv.at[k], SR), 2 * H // SR, (0,) * (14 * k + 14) + w_sq + (0,) * 100)
                  for k in se_early]
            se.append(stream(chain([sumexp(u * CU + k, sv.at[k] if k else sx, SR, None if k else sv.at[0])
                                    for k in late]), len(late) * 2 * H // SR,
                             (0,) * nq + (1,) * w_se + (0,) * (49 - w_se)))
            for k in range(CU):
                qk_unit(qslot(b, j + 1), u * CU + k, sv.at[k] if k else sx, spread([pc, cv] + se, nv, 14 * k))
            pv_unit(u, spread([cv] + se, nv, nq))

        def first(b, c):
            p = jnp.maximum(c - 1, 0)
            se = stream(sumexp(jnp.where(c > 0, p, NC), ss.at[p], SR), 2 * H // SR, w_s0)
            qk_unit(qslot(b, 0), c, ss.at[c], spread([se], never(c)))

        def last_rows(u, r0, r1):
            return chain([p_combos(u * CU + k, ss.at[u * CU + k], k, r0, r1) for k in range(CU)])

        def last(u):
            nv = never(u)
            cv = stream(chain([conv(NQ - 1, u * (CU // 2) + k // 2, k % 2, 0) for k in range(CU)]), CU * NCV, (1,) * 98)
            pv_unit(u, spread([stream(last_rows(u, QS, Q), PF * CU * (Q - QS) // 4, (1,) * 49), cv], nv), 0, QS)
            nu = jnp.minimum(u + 1, NC // CU - 1)
            pv_unit(u, spread([stream(last_rows(nu, 0, QS), PF * CU * QS // 4, (0,) * 49 + (1,) * 49), cv], nv, 49),
                    QS, Q)

        def loop(n, f, unroll=1):
            def body(i, _):
                for k in range(unroll):
                    f(i * unroll + k)
                return 0
            lax.fori_loop(0, n // unroll, body, 0)

        def batch(b):
            def pbody(j):
                f = b * NQ + j + 1
                nxt = jnp.minimum(f, B * NQ - 1)
                nb, nj = nxt // NQ, nxt % NQ

                @pl.when(f < B * NQ)
                def _():
                    xcopy(nb, nj).wait()
                proj_block(j, nb, nj)
            with scope("pA"):
                if 'pA' not in SKIP:
                    loop(NQ, pbody)
                else:
                    for jj in range(NQ):
                        pl.when(b * NQ + jj + 1 < B * NQ)(lambda: xcopy((b * NQ + jj + 1) // NQ, (b * NQ + jj + 1) % NQ).wait())
            with scope("Q0"):
                loop(NC, lambda c: first(b, c), UQ)
            with scope("st0"):
                @pl.when(b == 0)
                def _():
                    wcopies[4].wait()
                    wcopies[5].wait()
                    st_rhs(wr, 0, (4,), product(_dot, wtmp[4], wtmp[5]))
                    drain(sumexp(NC - 1, ss.at[NC - 1], PR))
                    drain(finish_stats(PR))

                @pl.when(b > 0)
                def _():
                    drain(sumexp(NC - 1, ss.at[NC - 1], PR))
                    drain(finish_stats(PR))

            def qblock(j):
                @pl.when(j < NQ - 1)
                def _():
                    with scope("steady"):
                        if 'steady' not in SKIP:
                            loop(NC // CU, lambda u: steady(b, j, u))

                @pl.when(j == NQ - 1)
                def _():
                    with scope("last"):
                        if 'last' not in SKIP:
                            drain(last_rows(0, 0, QS))
                            loop(NC // CU, last)
                f = b * NQ + j

                @pl.when(f >= 2)
                def _():
                    for h in range(2):
                        ocopy((f - 2) // NQ, (f - 2) % NQ, h).wait()
                with scope("sb"):
                    finish_block(b, j, 0, f % 2)
            loop(NQ, qblock)
        loop(B, batch)
        with scope("owait"):
            for j in (NQ - 2, NQ - 1):
                for h in range(2):
                    ocopy(B - 1, j, h).wait()

    def run(x, w_q, w_k, w_v, w_ao, w_up, dw, w_dn, w_merge):
        B, T, D = x.shape
        KT = dw.shape[0]
        DH = D // 2
        NT = D // LANES
        NP = T // 2
        NC = -(-NP // DH)
        NQ = T // (2 * H)
        RS = 2 if PACK else 1
        PT = U32 if PACK else BF16
        anyspec = pl.BlockSpec(memory_space=pl.ANY)
        return pl.pallas_call(
            kernel,
            out_shape=jax.ShapeDtypeStruct(x.shape, x.dtype),
            in_specs=[anyspec] * 9,
            out_specs=anyspec,
            scratch_shapes=[
                pltpu.VMEM((B, T, D), BF16),
                pltpu.VMEM((7, D, D), BF16),
                pltpu.VMEM((D, 2 * D), BF16),
                pltpu.VMEM((KT, D), BF16),
                pltpu.VMEM((5, 7, DH // RS, DH), PT),
                pltpu.VMEM((NT, 32, 8, LANES), F32),
                pltpu.VMEM((NQ + 1, 7, 2, H, LANES), F32),
                pltpu.VMEM((8, H // RS, DH), PT),
                pltpu.VMEM((8, H // RS, DH), PT),
                pltpu.VMEM((49, NC * LANES // 2, LANES), U32),
                pltpu.VMEM((49, NC * LANES // 2, LANES), U32),
                pltpu.VMEM((NT, T + 2 * HALO, LANES), F32),
                pltpu.VMEM((NT, T, LANES), F32),
                pltpu.VMEM((1, NT, 2 * H, LANES), F32),
                pltpu.VMEM((NC, 4, H, DH), F32),
                pltpu.VMEM((4, H, DH), F32),
                pltpu.VMEM((3, H, DH), F32),
                pltpu.VMEM((4, H // 2, LANES), F32),
                pltpu.VMEM((4, 3, H // 2, LANES), F32),
                pltpu.VMEM((7, 4, H // 2, CU * LANES), F32),
                pltpu.VMEM((52, H // 2, LANES), F32),
                pltpu.VMEM((2, H, LANES), F32),
                pltpu.VMEM((2, H, LANES), F32),
                pltpu.VMEM((2, H, LANES), F32),
                pltpu.VMEM((2, H, LANES), F32),
                pltpu.VMEM((2, 2, 2, H // 2, LANES), F32),
                pltpu.VMEM((2, 2 * H, D), BF16),
                pltpu.SemaphoreType.DMA((9,)),
                pltpu.SemaphoreType.DMA((B * NQ,)),
                pltpu.SemaphoreType.DMA((4,)),
            ],
            compiler_params=pltpu.CompilerParams(vmem_limit_bytes=124 * 1024 * 1024, flags=flags),
        )(x, w_q, w_k, w_v, w_ao, w_up, dw, w_dn, w_merge)
    return jax.jit(run)


@jax.jit
def pallas_standalone__conformer_family_branchformer__speech_kernel(x, w_q, w_k, w_v, w_ao, w_up, dw, w_dn, w_merge):
    return make()(x, w_q, w_k, w_v, w_ao, w_up, dw, w_dn, w_merge)
```

```python
import contextlib
import math
import jax
import numpy as np
import jax.numpy as jnp
from jax import lax
import jax.experimental.pallas as pl
import jax.experimental.pallas.tpu as pltpu

F32 = jnp.float32
BF16 = jnp.bfloat16
U32 = jnp.uint32
LANES = 128
HALO = 16
EPS = 1e-5
LOWEST = float(np.finfo(np.float32).min)


def _dot(a, b):
    return jnp.dot(a, b, preferred_element_type=F32)


def _dot_nt(a, b):
    return lax.dot_general(a, b, (((1,), (1,)), ((), ())), preferred_element_type=F32)


def _layernorm(x):
    m = jnp.mean(x, axis=-1, keepdims=True)
    d = x - m
    v = jnp.mean(d * d, axis=-1, keepdims=True)
    return d * lax.rsqrt(v + EPS)


def _gelu(x):
    c = math.sqrt(2.0 / math.pi)
    hx = 0.5 * x
    return hx + hx * jnp.tanh(x * (c + (c * 0.044715) * (x * x)))


def _lhs_combos(a11, a12, a21, a22):
    return [a11 + a22, a21 + a22, a11, a22, a11 + a12, a21 - a11, a12 - a22]


def _lhs_combo(i, quad):
    a, b, sign = ((0, 3, 1), (2, 3, 1), (0, None, 0), (3, None, 0), (0, 1, 1), (2, 0, -1), (1, 3, -1))[i]
    if b is None:
        return quad(a)
    return quad(a) + quad(b) if sign > 0 else quad(a) - quad(b)


def _rhs_combo(i, quad):
    a, b, sign = ((0, 3, 1), (0, None, 0), (1, 3, -1), (2, 0, -1), (3, None, 0), (0, 1, 1), (2, 3, 1))[i]
    if b is None:
        return quad(a)
    return quad(a) + quad(b) if sign > 0 else quad(a) - quad(b)


def _rhs_combos(b11, b12, b21, b22):
    return [b11 + b22, b11, b12 - b22, b21 - b11, b22, b11 + b12, b21 + b22]


def _even(n, w):
    tot = sum(w)
    cum = [sum(w[:k]) for k in range(len(w) + 1)]
    return [n * cum[k + 1] // tot - n * cum[k] // tot for k in range(len(w))]


ONES = (1, 1, 1, 1, 1, 1, 1)


def make(H=400, CV=5, CG=3, PACK=True, PR=80, flags=None, SC=False, SR=8, GR=8, CU=4,
         CM=1, SKIP=(), UQ=2, QS=96, PF=2, w_se=40, w_cv=(0, 1, 1), w_sq=(4, 3) * 3 + (0,) * 8, se_early=(),
         w_pc=(5, 4, 5, 4, 2, 2) + (4, 3) * 4, w_s0=(4, 3) * 3 + (0,) * 8, w_cv0=(1,) * 8 + (0, 0, 1, 1, 0, 0),
         w_fin=(1, 1, 1, 0, 0, 0, 0), w_st=(0, 0, 0, 1, 1, 1, 1), a_order=(1, 2, 3, 0),
         a_fill=(("s", 0, (1,) * 4), ("n", 4, (1,) * 4), ("g", 8, (1,) * 8), ("k", 14, (1,) * 8),
                 ("p", 9, (1,) * 12), ("v", 21, (1,) * 7))):
    def kernel(x_hbm, wq_hbm, wk_hbm, wv_hbm, wao_hbm, wup_hbm, dw_hbm, wdn_hbm, wm_hbm,
               o_hbm,
               xin, wtmp, wup, dwv, wr, dwb, ql, la, lnext, kr, vr, gs, us, uc, ss, sx, tq, ti, to, pbuf, acc,
               mrun, lrun, mfin, linv, xst, obuf,
               wsem, xsem, osem):
        B, T, D = xin.shape
        DH = D // 2
        KT = dwv.shape[0]
        BQ = 2 * H
        NQ = T // BQ
        NP = T // 2
        NC = ss.shape[0]
        Q = H // 2
        QM = Q // 16 * 16
        WP = NC * LANES
        CU = pbuf.shape[-1] // LANES
        NT = D // LANES
        RS = 2 if PACK else 1
        scope = jax.named_scope if SC else (lambda n: contextlib.nullcontext())

        def al(i, m):
            return i if isinstance(i, int) else pl.multiple_of(i, m)

        def st(ref, idx, r0, val):
            n, w = val.shape
            rows = pl.ds(al(r0 // RS, 8), n // RS)
            if PACK:
                v = val.reshape(n // 16, 2, 8, w)
                p = pltpu.pack_elementwise([v[:, 0], v[:, 1]], packed_dtype=BF16)
                ref[(*idx, rows, slice(None))] = p.reshape(n // 2, w)
            else:
                ref[(*idx, rows, slice(None))] = val.astype(BF16)

        def st_nat(ref, idx, r0, val):
            n, w = val.shape
            rows = pl.ds(al(r0 // RS, 8), n // RS)
            v = val.astype(BF16)
            ref[(*idx, rows, slice(None))] = pltpu.bitcast(v, U32) if PACK else v

        def un(v):
            return pltpu.bitcast(v, BF16) if PACK else v

        def ld(ref, idx, r0, n):
            return un(ref[(*idx, pl.ds(al(r0 // RS, 8), n // RS), slice(None))])

        def never(i):
            return lax.broadcasted_iota(jnp.int32, (8, LANES), 1) + i < 0

        def gate(x, tok):
            if tok is None:
                return x
            t, nv = tok
            n, w = x.shape
            reps = (n // 8, w // LANES)
            return jnp.where(jnp.tile(nv, reps), jnp.tile(t, reps), x)

        def stream(gen, steps, weights):
            next(gen)
            return gen, _even(steps, weights)

        def step(gen, tok):
            try:
                gen.send(tok)
            except StopIteration:
                pass

        def chain(gens):
            for g in gens:
                yield from g

        def drain(gen):
            for _ in gen:
                pass

        def spread(streams, nv, first=0):
            def hook(k, v):
                todo = []
                for gen, counts in streams:
                    cnt = counts[first + k]
                    for n in range(cnt):
                        todo.append(((v.shape[0] // 8) * n // cnt * 8, gen))
                todo.sort(key=lambda p: p[0])
                for r, gen in todo:
                    step(gen, (v[r:r + 8, :LANES], nv))
            return hook

        def x_words(b, j, h, r, cols, n=16):
            w = pltpu.bitcast(xin[b, pl.ds(al(j * BQ + h * H + r, 16), n), cols], U32)
            return [pltpu.unpack_elementwise(w, index=k, packed_dtype=BF16, unpacked_dtype=F32) for k in range(2)]

        def norm_stats(b, j, n=16):
            for r in range(0, H, n):
                for h in range(2):
                    tok = yield
                    v = jnp.concatenate(x_words(b, j, h, r, slice(None), n), axis=0)
                    v = jnp.concatenate([gate(v[:, :LANES], tok), v[:, LANES:]], axis=1)
                    m = jnp.mean(v, axis=-1, keepdims=True)
                    d = v - m
                    rs = lax.rsqrt(jnp.mean(d * d, axis=-1, keepdims=True) + EPS)
                    for k in range(2):
                        rows = slice(k * n // 2, (k + 1) * n // 2)
                        xst[0, h, k, pl.ds(r // 2, n // 2), :] = jnp.broadcast_to(m[rows], (n // 2, LANES))
                        xst[1, h, k, pl.ds(r // 2, n // 2), :] = jnp.broadcast_to(rs[rows], (n // 2, LANES))

        def qslot(b, j):
            return (b * NQ + j) % (NQ + 1)

        def norm_apply(b, j):
            for r in range(0, H, 16):
                for t in range(DH // LANES):
                    tok = yield
                    q = {}
                    for h in range(2):
                        for k in range(2):
                            q[h, k] = (gate(xst[0, h, k, pl.ds(r // 2, 8), :], tok), xst[1, h, k, pl.ds(r // 2, 8), :])
                    a = [[None] * 4, [None] * 4]
                    for h in range(2):
                        for e in range(2):
                            for k, v in enumerate(x_words(b, j, h, r, pl.ds(e * DH + t * LANES, LANES))):
                                a[k][2 * h + e] = (v - q[h, k][0]) * q[h, k][1]
                    for k in range(2):
                        for i, v in enumerate(_lhs_combos(*a[k])):
                            ql[qslot(b, j), i, t, pl.ds(r + 8 * k, 8), :] = v

        def norm_pack(b, j):
            for r in range(0, H, 16):
                tok = yield
                for i in range(7):
                    for t in range(DH // LANES):
                        pair = [ql[qslot(b, j), i, t, pl.ds(r + 8 * k, 8), :] for k in range(2)]
                        if t == 0:
                            pair[0] = gate(pair[0], tok)
                        lnext[i, pl.ds(r // 2, 8), pl.ds(t * LANES, LANES)] = pltpu.pack_elementwise(
                            pair, packed_dtype=BF16)

        w_src = (wq_hbm, wk_hbm, wv_hbm, wao_hbm, wdn_hbm, wm_hbm.at[pl.ds(D, D)], wm_hbm.at[pl.ds(0, D)])
        wcopies = [pltpu.make_async_copy(s, wtmp.at[i], wsem.at[i]) for i, s in enumerate(w_src)]
        wup_copy = pltpu.make_async_copy(wup_hbm, wup, wsem.at[7])
        dw_copy = pltpu.make_async_copy(dw_hbm, dwv, wsem.at[8])

        def xcopy(b, j):
            r0 = al(j * BQ, BQ)
            return pltpu.make_async_copy(x_hbm.at[b, pl.ds(r0, BQ)], xin.at[b, pl.ds(r0, BQ)], xsem.at[b * NQ + j])

        def ocopy(b, j, h):
            slot = (b * NQ + j) % 2
            return pltpu.make_async_copy(obuf.at[slot, pl.ds(h * H, H)], o_hbm.at[b, pl.ds(al(j * BQ + h * H, H), H)],
                                         osem.at[2 * slot + h])

        def halves(u):
            return [pltpu.unpack_elementwise(u, index=k, packed_dtype=BF16, unpacked_dtype=F32) for k in range(2)]

        def even_odd(w):
            return halves(pltpu.bitcast(w, U32))

        def st_rhs(ref, r0, idx, halves):
            n = DH // 2
            cs = [_rhs_combos(w[:n, :DH], w[:n, DH:], w[n:, :DH], w[n:, DH:]) for w in halves]
            for i, pair in enumerate(zip(*cs)):
                ref[(*idx, i, pl.ds(r0 // 2, n), slice(None))] = pltpu.pack_elementwise(list(pair), packed_dtype=BF16)

        def product(dot, a, b):
            v = dot(jnp.concatenate(even_odd(a), axis=0).astype(BF16), b)
            return [v[:D // 2], v[D // 2:]]

        for c in (wcopies[0], wcopies[1], wcopies[2], wcopies[3], dw_copy, xcopy(0, 0), wcopies[6], wup_copy):
            c.start()
        kr[:, pl.ds(QM * NQ // 2, (WP - QM * NQ) // 2), :] = jnp.zeros((49, (WP - QM * NQ) // 2, LANES), U32)
        vr[:, pl.ds(QM * NQ // 2, (WP - QM * NQ) // 2), :] = jnp.zeros((49, (WP - QM * NQ) // 2, LANES), U32)
        gs[:, pl.ds(0, HALO), :] = jnp.zeros((NT, HALO, LANES), F32)
        gs[:, pl.ds(HALO + T, HALO), :] = jnp.zeros((NT, HALO, LANES), F32)
        mrun[...] = jnp.full(mrun.shape, LOWEST, F32)
        lrun[...] = jnp.zeros(lrun.shape, F32)
        with scope("w01"):
            wcopies[0].wait()
            wcopies[1].wait()
        scale = float(D) ** -0.5 * math.log2(math.e)
        st_rhs(wr, 0, (2,), [v * scale for v in product(_dot_nt, wtmp[1], wtmp[0])])
        with scope("w23"):
            wcopies[2].wait()
            wcopies[3].wait()
            dw_copy.wait()
        wva = jnp.concatenate(product(_dot, wtmp[2], wtmp[3]), axis=0).astype(BF16)
        dwf = dwv[...].astype(F32)
        for t in range(NT):
            for i in range(KT):
                dwb[t, i] = jnp.broadcast_to(dwf[i:i + 1, t * LANES:(t + 1) * LANES], (8, LANES))
        with scope("w45"):
            xcopy(0, 0).wait()
            wcopies[6].wait()
        xcopy(0, 1).start()
        wvam = _dot(wva, wtmp[6])
        wvam = [wvam[:D // 2], wvam[D // 2:]]

        def wup_rows():
            n = DH // 2
            for m in range(2):
                for r in range(0, DH, 16):
                    tok = yield
                    top = even_odd(wup[pl.ds(r, 16), pl.ds(m * D, D)])
                    bot = even_odd(wup[pl.ds(DH + r, 16), pl.ds(m * D, D)])
                    cs = [_rhs_combos(gate(top[k][:, :DH], tok), top[k][:, DH:], bot[k][:, :DH], bot[k][:, DH:])
                          for k in range(2)]
                    for i, pair in enumerate(zip(*cs)):
                        wr[m, i, pl.ds(r // 2, 8), :] = pltpu.pack_elementwise(list(pair), packed_dtype=BF16)

        side = chain([norm_stats(0, 0), norm_apply(0, 0), norm_pack(0, 0)])
        nside = 2 * H // 8 + H // 16
        hook = spread([stream(side, nside, (1,) * 7 + (0,))], never(pl.program_id(0)))
        for t in range(NT):
            for k in range(2):
                hook(2 * t + k, wvam[k][:, t * LANES:(t + 1) * LANES])
        st_rhs(wr, 0, (3,), wvam)
        with scope("w6"):
            wup_copy.wait()
        wcopies[4].start()
        wcopies[5].start()
        for b in range(B):
            for j in range(NQ):
                if b or j > 1:
                    xcopy(b, j).start()
        drain(wup_rows())

        def strassen(M, tmp, out, fin, hook):
            v = M(4)
            tmp[2] = v
            hook(0, v)
            v = M(1) + tmp[2]
            tmp[0] = v
            hook(1, v)
            v = M(3)
            tmp[0] = tmp[0] + v
            tmp[1] = v
            hook(2, v)
            v = tmp[2] + M(2)
            fin(2, v)
            hook(3, v)
            v = (tmp[0] - out[2]) + M(6)
            fin(3, v)
            hook(4, v)
            v = tmp[1] + M(5)
            fin(1, v)
            hook(5, v)
            v = (tmp[0] - out[1]) + M(7)
            fin(0, v)
            hook(6, v)

        def post_act(j, m):
            buf = ss.at[m]
            dst = gs if m == 1 else us
            for h in (1, 0):
                for r in range(0, H, GR):
                    tok = yield
                    rr = pl.ds(r, GR)
                    v = _gelu(gate(jnp.concatenate([buf[2 * h, rr, :], buf[2 * h + 1, rr, :]], axis=1), tok))
                    if m == 1:
                        v = _layernorm(v)
                    off = j * BQ + h * H + r + (HALO if m == 1 else 0)
                    for t in range(NT):
                        dst[t, pl.ds(al(off, 8), GR), :] = v[:, t * LANES:(t + 1) * LANES]

        def post_kv(j, m):
            buf = ss.at[m]
            dst = kr if m == 2 else vr
            perm = (0, 2, 1, 3) if m == 2 else (0, 1, 2, 3)
            for r in range(0, Q, 16):
                n = min(16, Q - r)
                for o in range(7):
                    tok = yield

                    def tile(t):
                        rows, cols = pl.ds((t // 2) * Q + r, n), pl.ds((t % 2) * LANES, LANES)
                        return _rhs_combo(o, lambda q: buf[perm[q], rows, cols])
                    t = [gate(tile(0), tok), tile(perm[1]), tile(perm[2]), gate(tile(3), tok)]
                    for i, c in enumerate(_rhs_combos(*t)):
                        if n == 16:
                            rows, pair = pl.ds(al((j * QM + r) // 2, 8), 8), [c[:8], c[8:]]
                        else:
                            rows = pl.ds(al(NQ * QM // 2 + 8 * (j // 2), 8), 8)
                            old = halves(dst[7 * o + i, rows, :])
                            pair = [jnp.where(j % 2 == 0, c, old[0]), jnp.where(j % 2 == 0, old[1], c)]
                        dst[7 * o + i, rows, :] = pltpu.pack_elementwise(pair, packed_dtype=BF16)

        def proj_block(j, nb, nj):
            nv = never(j)
            gens = {"k": (post_kv(j, 2), 7 * -(-Q // 16)), "v": (post_kv(j, 3), 7 * -(-Q // 16)),
                    "g": (post_act(j, 1), 2 * H // GR), "u": (post_act(j, 0), 2 * H // GR),
                    "s": (norm_stats(nb, nj), H // 8), "n": (norm_apply(nb, nj), H // 8),
                    "p": (norm_pack(nb, nj), H // 16)}
            streams = [stream(*gens[name], (0,) * pos + tuple(w) + (0,) * (28 - pos - len(w)))
                       for name, pos, w in a_fill]
            for pos, m in enumerate(a_order):
                buf = ss.at[m]

                def fin(q, v):
                    buf[q] = v

                def M(i):
                    if pos == 0:
                        v = lnext[i - 1]
                        la[i - 1] = v
                    else:
                        v = la[i - 1]
                    return _dot(un(v), ld(wr, (m, i - 1), 0, DH))
                strassen(M, buf, buf, fin, spread(streams, nv, 7 * pos))
            drain(gens["ugkv"[a_order[-1]]][0])

        col = lax.broadcasted_iota(jnp.int32, (8, LANES), 1)

        def valid_keys(c):
            w = col + c * LANES
            full = NQ * QM + 16 * (NQ // 2)
            return (w < full) | ((w < full + 16 * (NQ % 2)) & (w % 2 == 0))

        def qk_unit(slot, c, buf, hook):
            for n, o in enumerate((4, 1, 3, 2, 6, 5, 7)):
                def M(i):
                    return _dot_nt(_lhs_combo(i - 1, lambda t: ql[slot, o - 1, t % 2, pl.ds((t // 2) * Q, Q), :]),
                                   ld(kr, (7 * (o - 1) + i - 1,), c * LANES, LANES))

                def emit(t, v):
                    rows, cols = pl.ds((t // 2) * Q, Q), pl.ds((t % 2) * LANES, LANES)

                    def fin(q, w):
                        buf[q, rows, cols] = w
                    if o == 4:
                        to[t, 2] = v
                    elif o == 1:
                        to[t, 0] = to[t, 2] + v
                    elif o == 3:
                        to[t, 0] = to[t, 0] + v
                        to[t, 1] = v
                    elif o == 2:
                        fin(2, to[t, 2] + v)
                    elif o == 6:
                        fin(3, (to[t, 0] - buf[2, rows, cols]) + v)
                    elif o == 5:
                        fin(1, to[t, 1] + v)
                    else:
                        fin(0, (to[t, 0] - buf[1, rows, cols]) + v)
                m3, m5, m2, m4 = M(3), M(5), M(2), M(4)
                ti[0] = m4 - m5
                ti[1] = m3 - m2
                c12 = m3 + m5
                emit(1, c12)
                emit(2, m2 + m4)
                hook(2 * n, c12)
                m1, m6, m7 = M(1), M(6), M(7)
                c22 = (m1 + ti[1]) + m6
                emit(3, c22)
                emit(0, (m1 + ti[0]) + m7)
                hook(2 * n + 1, c22)

        def sumexp(c, buf, n, copy_to=None):
            vn = jnp.tile(valid_keys(c), (n // 8, 1))
            for h in (1, 0):
                for r in range(0, H, n):
                    tok = yield
                    rr = pl.ds(r, n)
                    old = gate(mrun[h, rr, :], tok)
                    v = []
                    for q in (2 * h, 2 * h + 1):
                        for t in range(2):
                            v.append(buf[q, rr, pl.ds(t * LANES, LANES)])
                            if copy_to is not None:
                                copy_to[q, rr, pl.ds(t * LANES, LANES)] = v[-1]
                    top = jnp.maximum(jnp.maximum(v[0], v[1]), jnp.maximum(v[2], v[3]))
                    m = jnp.maximum(old, jnp.where(vn, top, LOWEST))
                    e = [jnp.exp2(x - m) for x in v]
                    l = lrun[h, rr, :] * jnp.exp2(old - m)
                    lrun[h, rr, :] = l + jnp.where(vn, (e[0] + e[1]) + (e[2] + e[3]), 0.0)
                    mrun[h, rr, :] = m

        def finish_stats(n):
            for h in range(2):
                for r in range(0, H, n):
                    tok = yield
                    rr = pl.ds(r, n)
                    m = jnp.max(gate(mrun[h, rr, :], tok), axis=-1, keepdims=True)
                    mfin[h, rr, :] = jnp.broadcast_to(m, (n, LANES))
            for h in range(2):
                for r in range(0, H, n):
                    tok = yield
                    rr = pl.ds(r, n)
                    e = jnp.exp2(gate(mrun[h, rr, :], tok) - mfin[h, rr, :])
                    l = jnp.sum(lrun[h, rr, :] * e, axis=-1, keepdims=True)
                    linv[h, rr, :] = jnp.broadcast_to(pl.reciprocal(l, full_range=False), (n, LANES))
                    mrun[h, rr, :] = jnp.full((n, LANES), LOWEST, F32)
                    lrun[h, rr, :] = jnp.zeros((n, LANES), F32)

        def p_combos(c, buf, k, r0=0, r1=Q):
            valid = valid_keys(c)
            for r in range(r0, r1, 8):
                for rq in range(2):
                    rr = pl.ds(rq * Q + r, 8)
                    for kq in range(2):
                        if kq == 0 or PF == 2:
                            tok = yield
                            top = gate(jnp.full((8, LANES), jnp.inf, F32), tok)
                            m = [jnp.where(valid, mfin[h, rr, :], top) for h in range(2)]
                            il = [linv[h, rr, :] for h in range(2)]
                        p = [jnp.exp2(buf[q, rr, pl.ds(kq * LANES, LANES)] - m[q // 2]) * il[q // 2]
                             for q in range(4)]
                        for o, v in enumerate(_lhs_combos(*p)):
                            pbuf[o, 2 * rq + kq, pl.ds(r, 8), pl.ds(k * LANES, LANES)] = v

        def pv_unit(u, hook, r0=0, r1=Q):
            rows = pl.ds(r0, r1 - r0)
            for o in range(7):
                for i in range(7):
                    lhs = _lhs_combo(i, lambda t: pbuf[o, t, rows, :])
                    v = _dot(lhs, ld(vr, (7 * o + i,), u * CU * LANES, CU * LANES))
                    acc[7 * o + i, rows, :] = jnp.where(u > 0, acc[7 * o + i, rows, :], 0.0) + v
                    hook(7 * o + i, v)

        def conv(j, t, half, slot):
            base = half * H
            r0 = j * BQ + base
            for a in range(0, H // 8, CV):
                n = min(CV, H // 8 - a)
                o = None
                cnt = 0
                if CM == 2:
                    win = gs[t, pl.ds(al(r0 + 8 * a, 8), 8 * (n + 4)), :]
                for r in range(8):
                    taps = [i for i in range(KT) if (i + 1) % 8 == r]
                    lo, hi = (taps[0] + 1) // 8, (taps[-1] + 1) // 8
                    if CM == 2:
                        g = win[8 * lo + r:8 * lo + r + 8 * (n + hi - lo)]
                    else:
                        g = gs[t, pl.ds(r0 + 8 * (a + lo) + r, 8 * (n + hi - lo)), :]
                    g = g.reshape(n + hi - lo, 8, LANES)
                    for i in taps:
                        w = dwb[t, i]
                        if cnt % CG == 0:
                            tok = yield
                            w = gate(w, tok)
                        cnt += 1
                        k = (i + 1) // 8 - lo
                        term = g[k:k + n] * w[None]
                        o = term if o is None else o + term
                rows_in = pl.ds(al(r0 + 8 * a, 8), 8 * n)
                rows_out = pl.ds(al(base + 8 * a, 8), 8 * n)
                uc[slot, t, rows_out, :] = us[t, rows_in, :] * o.reshape(8 * n, LANES)

        def out_combos(m):
            c12 = m[2] + m[4]
            c21 = m[1] + m[3]
            u = m[0] + m[3] + m[2]
            return [(u - c12) + m[6], c12, c21, (u - c21) + m[5]]

        def attn_rows():
            for r in range(0, Q, 8):
                tok = yield
                rr = pl.ds(r, 8)
                inner = []
                for o in range(7):
                    m = [acc[7 * o + i, rr, :] for i in range(7)]
                    m[2], m[3] = gate(m[2], tok), gate(m[3], tok)
                    inner.append(out_combos(m))
                for t in range(4):
                    for q, v in enumerate(out_combos([inner[o][t] for o in range(7)])):
                        sx[q, pl.ds((t // 2) * Q + r, 8), pl.ds((t % 2) * LANES, LANES)] = v

        def finish_block(b, j, slot, oslot):
            def even_odd_rows(t, h):
                lo = uc[slot, t, pl.ds(h * H, H // 2, stride=2), :].reshape(H // 16, 1, 8, LANES)
                hi = uc[slot, t, pl.ds(h * H + 1, H // 2, stride=2), :].reshape(H // 16, 1, 8, LANES)
                return jnp.concatenate([lo, hi], axis=1).reshape(H, LANES)

            def quad(q):
                return jnp.concatenate([even_odd_rows(2 * (q % 2) + t, q // 2) for t in range(2)], axis=1)

            def M(i):
                return _dot(_lhs_combo(i - 1, quad), ld(wr, (4, i - 1), 0, DH))

            def fin(q, v):
                if q in (1, 2):
                    tq[q] = v
                cols = pl.ds((q % 2) * DH, DH)
                v = (sx[q] + v).reshape(H // 16, 2, 8, DH)
                xs = x_words(b, j, q // 2, 0, cols, H)
                out = pltpu.pack_elementwise([xs[k] + v[:, k].reshape(H // 2, DH) for k in range(2)],
                                             packed_dtype=BF16)
                obuf[oslot, pl.ds((q // 2) * H, H), cols] = pltpu.bitcast(out, BF16)
                if q in (0, 3):
                    ocopy(b, j, q // 2).start()
            strassen(M, tq, tq, fin, spread([stream(attn_rows(), Q // 8, w_fin),
                                             stream(finish_stats(SR), 4 * H // SR, w_st)], never(j)))

        NCV = (-(-(H // 8) // CV)) * (-(-KT // CG))

        def steady(b, j, u):
            nv = never(u)
            sv = ss.at[pl.ds(u * CU, CU)]
            order = list(range(1, CU)) + [0]
            nq = 14 * CU
            wq = w_pc
            pc = stream(chain([p_combos(u * CU + k, sv.at[k], k) for k in order]), PF * CU * Q // 4, wq * CU + (0,) * 49)
            cv = stream(chain([conv(j, u * (CU // 2) + k // 2, k % 2, 0) for k in range(CU)]), CU * NCV,
                        (w_cv[0],) * nq + (w_cv[1],) * w_se + (w_cv[2],) * (49 - w_se))
            late = [k for k in range(CU) if k not in se_early]
            se = [stream(sumexp(u * CU + k, sv.at[k], SR), 2 * H // SR, (0,) * (14 * k + 14) + w_sq + (0,) * 100)
                  for k in se_early]
            se.append(stream(chain([sumexp(u * CU + k, sv.at[k] if k else sx, SR, None if k else sv.at[0])
                                    for k in late]), len(late) * 2 * H // SR,
                             (0,) * nq + (1,) * w_se + (0,) * (49 - w_se)))
            for k in range(CU):
                qk_unit(qslot(b, j + 1), u * CU + k, sv.at[k] if k else sx, spread([pc, cv] + se, nv, 14 * k))
            pv_unit(u, spread([cv] + se, nv, nq))

        def first(b, c):
            p = jnp.maximum(c - 1, 0)
            se = stream(sumexp(jnp.where(c > 0, p, NC), ss.at[p], SR), 2 * H // SR, w_s0)
            qk_unit(qslot(b, 0), c, ss.at[c], spread([se], never(c)))

        def last_rows(u, r0, r1):
            return chain([p_combos(u * CU + k, ss.at[u * CU + k], k, r0, r1) for k in range(CU)])

        def last(u):
            nv = never(u)
            cv = stream(chain([conv(NQ - 1, u * (CU // 2) + k // 2, k % 2, 0) for k in range(CU)]), CU * NCV, (1,) * 98)
            pv_unit(u, spread([stream(last_rows(u, QS, Q), PF * CU * (Q - QS) // 4, (1,) * 49), cv], nv), 0, QS)
            nu = jnp.minimum(u + 1, NC // CU - 1)
            pv_unit(u, spread([stream(last_rows(nu, 0, QS), PF * CU * QS // 4, (0,) * 49 + (1,) * 49), cv], nv, 49),
                    QS, Q)

        def loop(n, f, unroll=1):
            def body(i, _):
                for k in range(unroll):
                    f(i * unroll + k)
                return 0
            lax.fori_loop(0, n // unroll, body, 0)

        def batch(b):
            def pbody(j):
                f = b * NQ + j + 1
                nxt = jnp.minimum(f, B * NQ - 1)
                nb, nj = nxt // NQ, nxt % NQ

                @pl.when(f < B * NQ)
                def _():
                    xcopy(nb, nj).wait()
                proj_block(j, nb, nj)
            with scope("pA"):
                if 'pA' not in SKIP:
                    loop(NQ, pbody)
                else:
                    for jj in range(NQ):
                        pl.when(b * NQ + jj + 1 < B * NQ)(lambda: xcopy((b * NQ + jj + 1) // NQ, (b * NQ + jj + 1) % NQ).wait())
            with scope("Q0"):
                loop(NC, lambda c: first(b, c), UQ)
            with scope("st0"):
                @pl.when(b == 0)
                def _():
                    wcopies[4].wait()
                    wcopies[5].wait()
                    st_rhs(wr, 0, (4,), product(_dot, wtmp[4], wtmp[5]))
                    drain(sumexp(NC - 1, ss.at[NC - 1], PR))
                    drain(finish_stats(PR))

                @pl.when(b > 0)
                def _():
                    drain(sumexp(NC - 1, ss.at[NC - 1], PR))
                    drain(finish_stats(PR))

            def qblock(j):
                @pl.when(j < NQ - 1)
                def _():
                    with scope("steady"):
                        if 'steady' not in SKIP:
                            loop(NC // CU, lambda u: steady(b, j, u))

                @pl.when(j == NQ - 1)
                def _():
                    with scope("last"):
                        if 'last' not in SKIP:
                            drain(last_rows(0, 0, QS))
                            loop(NC // CU, last)
                f = b * NQ + j

                @pl.when(f >= 2)
                def _():
                    for h in range(2):
                        ocopy((f - 2) // NQ, (f - 2) % NQ, h).wait()
                with scope("sb"):
                    finish_block(b, j, 0, f % 2)
            loop(NQ, qblock)
        loop(B, batch)
        with scope("owait"):
            for j in (NQ - 2, NQ - 1):
                for h in range(2):
                    ocopy(B - 1, j, h).wait()

    def run(x, w_q, w_k, w_v, w_ao, w_up, dw, w_dn, w_merge):
        B, T, D = x.shape
        KT = dw.shape[0]
        DH = D // 2
        NT = D // LANES
        NP = T // 2
        NC = -(-NP // DH)
        NQ = T // (2 * H)
        RS = 2 if PACK else 1
        PT = U32 if PACK else BF16
        anyspec = pl.BlockSpec(memory_space=pl.ANY)
        return pl.pallas_call(
            kernel,
            out_shape=jax.ShapeDtypeStruct(x.shape, x.dtype),
            grid=(1,),
            in_specs=[anyspec] * 9,
            out_specs=anyspec,
            scratch_shapes=[
                pltpu.VMEM((B, T, D), BF16),
                pltpu.VMEM((7, D, D), BF16),
                pltpu.VMEM((D, 2 * D), BF16),
                pltpu.VMEM((KT, D), BF16),
                pltpu.VMEM((5, 7, DH // RS, DH), PT),
                pltpu.VMEM((NT, 32, 8, LANES), F32),
                pltpu.VMEM((NQ + 1, 7, 2, H, LANES), F32),
                pltpu.VMEM((8, H // RS, DH), PT),
                pltpu.VMEM((8, H // RS, DH), PT),
                pltpu.VMEM((49, NC * LANES // 2, LANES), U32),
                pltpu.VMEM((49, NC * LANES // 2, LANES), U32),
                pltpu.VMEM((NT, T + 2 * HALO, LANES), F32),
                pltpu.VMEM((NT, T, LANES), F32),
                pltpu.VMEM((1, NT, 2 * H, LANES), F32),
                pltpu.VMEM((NC, 4, H, DH), F32),
                pltpu.VMEM((4, H, DH), F32),
                pltpu.VMEM((3, H, DH), F32),
                pltpu.VMEM((4, H // 2, LANES), F32),
                pltpu.VMEM((4, 3, H // 2, LANES), F32),
                pltpu.VMEM((7, 4, H // 2, CU * LANES), F32),
                pltpu.VMEM((52, H // 2, LANES), F32),
                pltpu.VMEM((2, H, LANES), F32),
                pltpu.VMEM((2, H, LANES), F32),
                pltpu.VMEM((2, H, LANES), F32),
                pltpu.VMEM((2, H, LANES), F32),
                pltpu.VMEM((2, 2, 2, H // 2, LANES), F32),
                pltpu.VMEM((2, 2 * H, D), BF16),
                pltpu.SemaphoreType.DMA((9,)),
                pltpu.SemaphoreType.DMA((B * NQ,)),
                pltpu.SemaphoreType.DMA((4,)),
            ],
            compiler_params=pltpu.CompilerParams(vmem_limit_bytes=124 * 1024 * 1024, flags=flags),
        )(x, w_q, w_k, w_v, w_ao, w_up, dw, w_dn, w_merge)
    return jax.jit(run)


@jax.jit
def pallas_standalone__conformer_family_branchformer__speech_kernel(x, w_q, w_k, w_v, w_ao, w_up, dw, w_dn, w_merge):
    return make()(x, w_q, w_k, w_v, w_ao, w_up, dw, w_dn, w_merge)
```

```python
import contextlib
import math

import jax
import jax.numpy as jnp
import numpy as np
from jax import lax
import jax.experimental.pallas as pl
import jax.experimental.pallas.tpu as pltpu

F32 = jnp.float32
BF16 = jnp.bfloat16
LANES = 128
HALO = 16
EPS = 1e-5
LOWEST = float(np.finfo(np.float32).min)

_LHS = ((0, 3, 1), (2, 3, 1), (0, None, 0), (3, None, 0), (0, 1, 1), (2, 0, -1), (1, 3, -1))
_RHS = ((0, 3, 1), (0, None, 0), (1, 3, -1), (2, 0, -1), (3, None, 0), (0, 1, 1), (2, 3, 1))


def _combo(table, i, quad):
    a, b, sign = table[i]
    if b is None:
        return quad(a)
    return quad(a) + quad(b) if sign > 0 else quad(a) - quad(b)


def _combos(table, quads):
    return [_combo(table, i, quads.__getitem__) for i in range(7)]


def _out_combos(m):
    c12 = m[2] + m[4]
    c21 = m[1] + m[3]
    u = m[0] + m[3] + m[2]
    return [(u - c12) + m[6], c12, c21, (u - c21) + m[5]]


def _dot(a, b):
    return jnp.dot(a, b, preferred_element_type=F32)


def _mm(a, b):
    return lax.dot_general(a, b, (((1,), (0,)), ((), ())), preferred_element_type=F32)


def _mm_nt(a, b):
    return lax.dot_general(a, b, (((1,), (1,)), ((), ())), preferred_element_type=F32)


def _layernorm(x):
    m = jnp.mean(x, axis=-1, keepdims=True)
    d = x - m
    v = jnp.mean(d * d, axis=-1, keepdims=True)
    return d * lax.rsqrt(v + EPS)


def _gelu(x):
    c = math.sqrt(2.0 / math.pi)
    hx = 0.5 * x
    return hx + hx * jnp.tanh(x * (c + (c * 0.044715) * (x * x)))


def _al(i, m):
    return i if isinstance(i, int) else pl.multiple_of(i, m)


def _loop(n, f, unroll=1):
    def body(i, carry):
        for k in range(unroll):
            f(i * unroll + k)
        return carry
    lax.fori_loop(0, n // unroll, body, 0)


def _never(i):
    return lax.broadcasted_iota(jnp.int32, (8, LANES), 1) + i < 0


def _gate(x, tok):
    if tok is None:
        return x
    value, never = tok
    reps = (x.shape[0] // 8, x.shape[1] // LANES)
    return jnp.where(jnp.tile(never, reps), jnp.tile(value, reps), x)


def _stream(gen, steps, weights):
    next(gen)
    cum = [sum(weights[:k]) for k in range(len(weights) + 1)]
    return gen, [steps * cum[k + 1] // cum[-1] - steps * cum[k] // cum[-1] for k in range(len(weights))]


def _chain(gens):
    for g in gens:
        yield from g


def _drain(gen):
    for _ in gen:
        pass


def _spread(streams, never, first=0):
    def hook(k, v):
        todo = []
        for gen, counts in streams:
            cnt = counts[first + k]
            todo += [((v.shape[0] // 8) * n // cnt * 8, gen) for n in range(cnt)]
        todo.sort(key=lambda p: p[0])
        for r, gen in todo:
            try:
                gen.send((v[r:r + 8, :LANES], never))
            except StopIteration:
                pass
    return hook


def _strassen(product, tmp, out, fin, hook):
    v = product(3)
    tmp[2] = v
    hook(0, v)
    v = product(0) + tmp[2]
    tmp[0] = v
    hook(1, v)
    v = product(2)
    tmp[0] = tmp[0] + v
    tmp[1] = v
    hook(2, v)
    v = tmp[2] + product(1)
    fin(2, v)
    hook(3, v)
    v = (tmp[0] - out[2]) + product(5)
    fin(3, v)
    hook(4, v)
    v = tmp[1] + product(4)
    fin(1, v)
    hook(5, v)
    v = (tmp[0] - out[1]) + product(6)
    fin(0, v)
    hook(6, v)


def make(H=400, CU=4, CV=5, CG=3, UQ=2, QS=96, SC=False,
         w_se=40, w_cv=(1, 1), w_pc=(5, 4, 5, 4, 2, 2) + (4, 3) * 4, w_s0=(4, 3) * 3 + (0,) * 8,
         w_fin=(1, 1, 1, 0, 0, 0, 0), w_st=(0, 0, 0, 1, 1, 1, 1),
         a_fill=(("s", 0, (1,) * 6), ("n", 7, (1,) * 8), ("g", 8, (1,) * 9), ("k", 14, (1,) * 8),
                 ("v", 21, (1,) * 7))):
    def kernel(x_hbm, wq_hbm, wk_hbm, wv_hbm, wao_hbm, wup_hbm, dw_hbm, wdn_hbm, wm_hbm,
               o_hbm,
               xin, wtmp, wup, dwv, wr, dwb, ql, lnext, kr, vr, gs, us, uc, ss, sx, tq, ti, to, pbuf, acc,
               mrun, lrun, mfin, linv, xst, obuf,
               wsem, xsem, osem):
        B, T, D = xin.shape
        KT = dwv.shape[0]
        NT = D // LANES
        DH = D // 2
        BQ = 2 * H
        NQ = T // BQ
        Q = H // 2
        QM = Q // 64 * 64
        NC = ss.shape[0]
        NU = NC // CU
        UP, GATE, KEY, VAL, DOWN = range(5)
        scope = jax.named_scope if SC else (lambda n: contextlib.nullcontext())

        w_src = (wq_hbm, wk_hbm, wv_hbm, wao_hbm, wdn_hbm, wm_hbm.at[pl.ds(D, D)], wm_hbm.at[pl.ds(0, D)])
        wcopy = [pltpu.make_async_copy(s, wtmp.at[i], wsem.at[i]) for i, s in enumerate(w_src)]
        wup_copy = pltpu.make_async_copy(wup_hbm, wup, wsem.at[7])
        dw_copy = pltpu.make_async_copy(dw_hbm, dwv, wsem.at[8])

        def xcopy(b, j):
            rows = pl.ds(_al(j * BQ, BQ), BQ)
            return pltpu.make_async_copy(x_hbm.at[b, rows], xin.at[b, rows], xsem.at[b * NQ + j])

        def ocopy(b, j, h):
            slot = (b * NQ + j) % 2
            return pltpu.make_async_copy(obuf.at[slot, pl.ds(h * H, H)],
                                         o_hbm.at[b, pl.ds(_al(j * BQ + h * H, H), H)], osem.at[2 * slot + h])

        def x_rows(b, j, h, r, n, cols):
            return xin[b, pl.ds(_al(j * BQ + h * H + r, 8), n), cols].astype(F32)

        def norm_stats(b, j):
            for r in range(0, H, 16):
                for h in range(2):
                    tok = yield
                    v = x_rows(b, j, h, r, 16, slice(None))
                    v = jnp.concatenate([_gate(v[:, :LANES], tok), v[:, LANES:]], axis=1)
                    m = jnp.mean(v, axis=-1, keepdims=True)
                    d = v - m
                    rs = lax.rsqrt(jnp.mean(d * d, axis=-1, keepdims=True) + EPS)
                    xst[0, h, pl.ds(r, 16), :] = jnp.broadcast_to(m, (16, LANES))
                    xst[1, h, pl.ds(r, 16), :] = jnp.broadcast_to(rs, (16, LANES))

        def norm_apply(b, j):
            for r in range(0, H, 8):
                tok = yield
                mean = [_gate(xst[0, h, pl.ds(r, 8), :], tok) for h in range(2)]
                rstd = [xst[1, h, pl.ds(r, 8), :] for h in range(2)]
                for t in range(2):
                    a = [(x_rows(b, j, q // 2, r, 8, pl.ds((q % 2) * DH + t * LANES, LANES)) - mean[q // 2])
                         * rstd[q // 2] for q in range(4)]
                    for i, v in enumerate(_combos(_LHS, a)):
                        lnext[i, t, pl.ds(r, 8), :] = v

        def store_weights(m, top, bot, r=0):
            quads = [top[:, :DH], top[:, DH:], bot[:, :DH], bot[:, DH:]]
            for i, c in enumerate(_combos(_RHS, quads)):
                wr[m, i, pl.ds(r, top.shape[0]), :] = c.astype(BF16)

        for c in (wcopy[0], wcopy[1], wcopy[2], wcopy[3], dw_copy, xcopy(0, 0), wcopy[6], wup_copy):
            c.start()
        for ref in (kr, vr):
            pad = ref.shape[1] - T // 4
            ref[:, pl.ds(T // 4, pad), :] = jnp.zeros((49, pad, LANES), BF16)
        gs[:, pl.ds(0, HALO), :] = jnp.zeros((NT, HALO, LANES), F32)
        gs[:, pl.ds(HALO + T, HALO), :] = jnp.zeros((NT, HALO, LANES), F32)
        acc[...] = jnp.zeros(acc.shape, F32)
        mrun[...] = jnp.full(mrun.shape, LOWEST, F32)
        lrun[...] = jnp.zeros(lrun.shape, F32)

        wcopy[0].wait()
        wcopy[1].wait()
        w = _mm_nt(wtmp[1], wtmp[0]) * (float(D) ** -0.5 * math.log2(math.e))
        store_weights(KEY, w[:DH], w[DH:])

        wcopy[2].wait()
        wcopy[3].wait()
        dw_copy.wait()
        wva = _dot(wtmp[2], wtmp[3]).astype(BF16)
        dwf = dwv[...].astype(F32)
        for t in range(NT):
            for i in range(KT):
                dwb[t, i] = jnp.broadcast_to(dwf[i:i + 1, t * LANES:(t + 1) * LANES], (8, LANES))

        xcopy(0, 0).wait()
        wcopy[6].wait()
        xcopy(0, 1).start()
        w = _dot(wva, wtmp[6])
        side = _stream(_chain([norm_stats(0, 0), norm_apply(0, 0)]), H // 4, (1,) * 7 + (0,))
        hook = _spread([side], _never(pl.program_id(0)))
        for t in range(NT):
            for k in range(2):
                hook(2 * t + k, w[k * DH:(k + 1) * DH, t * LANES:(t + 1) * LANES])
        store_weights(VAL, w[:DH], w[DH:])

        wup_copy.wait()
        wcopy[4].start()
        wcopy[5].start()
        for f in range(2, B * NQ):
            xcopy(f // NQ, f % NQ).start()
        for m in (UP, GATE):
            for r in range(0, DH, 32):
                top, bot = (wup[pl.ds(k * DH + r, 32), pl.ds(m * D, D)].astype(F32) for k in range(2))
                store_weights(m, top, bot, r)

        def post_act(j, m):
            buf = ss.at[m]
            dst, off = (gs, HALO) if m == GATE else (us, 0)
            for h in (1, 0):
                for r in range(0, H, 8):
                    tok = yield
                    rr = pl.ds(r, 8)
                    v = _gelu(_gate(jnp.concatenate([buf[2 * h, rr, :], buf[2 * h + 1, rr, :]], axis=1), tok))
                    if m == GATE:
                        v = _layernorm(v)
                    rows = pl.ds(_al(j * BQ + h * H + r + off, 8), 8)
                    for t in range(NT):
                        dst[t, rows, :] = v[:, t * LANES:(t + 1) * LANES]

        def post_kv(j, m):
            buf = ss.at[m]
            dst = kr if m == KEY else vr
            perm = (0, 2, 1, 3) if m == KEY else (0, 1, 2, 3)
            for r in range(0, Q, 16):
                n = min(16, Q - r)
                pos = _al(j * QM + r, 16) if r < QM else _al(NQ * QM + j * (Q - QM) + r - QM, 8)
                for o in range(7):
                    tok = yield

                    def tile(t):
                        rows, cols = pl.ds((t // 2) * Q + r, n), pl.ds((t % 2) * LANES, LANES)
                        return _combo(_RHS, o, lambda q: buf[perm[q], rows, cols])
                    tiles = [_gate(tile(0), tok), tile(perm[1]), tile(perm[2]), _gate(tile(3), tok)]
                    for i, c in enumerate(_combos(_RHS, tiles)):
                        dst[7 * o + i, pl.ds(pos, n), :] = c.astype(BF16)

        def project(j, nb, nj):
            nkv = 7 * -(-Q // 16)
            gens = {"k": (post_kv(j, KEY), nkv), "v": (post_kv(j, VAL), nkv), "g": (post_act(j, GATE), H // 4),
                    "s": (norm_stats(nb, nj), H // 8), "n": (norm_apply(nb, nj), H // 8)}
            streams = [_stream(*gens[name], (0,) * pos + w + (0,) * (28 - pos - len(w))) for name, pos, w in a_fill]
            for pos, m in enumerate((GATE, KEY, VAL, UP)):
                buf = ss.at[m]

                def fin(q, v):
                    buf[q] = v

                def product(i):
                    if pos == 0:
                        v = [lnext[i, t] for t in range(2)]
                        for t in range(2):
                            ql[j, i, t] = v[t]
                    else:
                        v = [ql[j, i, t] for t in range(2)]
                    return _mm(jnp.concatenate(v, axis=1), wr[m, i])
                _strassen(product, buf, buf, fin, _spread(streams, _never(j), 7 * pos))
            _drain(post_act(j, UP))

        def valid_keys(c):
            return lax.broadcasted_iota(jnp.int32, (8, LANES), 1) < T // 4 - c * LANES

        def qk_unit(j, c, buf, hook):
            keys = pl.ds(_al(c * LANES, LANES), LANES)
            for n, o in enumerate((3, 0, 2, 1, 5, 4, 6)):
                def product(i):
                    lhs = _combo(_LHS, i, lambda t: ql[j, o, t % 2, pl.ds((t // 2) * Q, Q), :])
                    return _mm_nt(lhs, kr[7 * o + i, keys, :])

                def emit(t, v):
                    rows, cols = pl.ds((t // 2) * Q, Q), pl.ds((t % 2) * LANES, LANES)
                    if n == 0:
                        to[t, 2] = v
                    elif n == 1:
                        to[t, 0] = to[t, 2] + v
                    elif n == 2:
                        to[t, 0] = to[t, 0] + v
                        to[t, 1] = v
                    elif n == 3:
                        buf[2, rows, cols] = to[t, 2] + v
                    elif n == 4:
                        buf[3, rows, cols] = (to[t, 0] - buf[2, rows, cols]) + v
                    elif n == 5:
                        buf[1, rows, cols] = to[t, 1] + v
                    else:
                        buf[0, rows, cols] = (to[t, 0] - buf[1, rows, cols]) + v
                m3, m5, m2, m4 = product(2), product(4), product(1), product(3)
                ti[0] = m4 - m5
                ti[1] = m3 - m2
                c12 = m3 + m5
                emit(1, c12)
                emit(2, m2 + m4)
                hook(2 * n, c12)
                m1, m6, m7 = product(0), product(5), product(6)
                c22 = (m1 + ti[1]) + m6
                emit(3, c22)
                emit(0, (m1 + ti[0]) + m7)
                hook(2 * n + 1, c22)

        def sumexp(c, buf, copy_to=None):
            valid = valid_keys(c)
            for h in (1, 0):
                for r in range(0, H, 8):
                    tok = yield
                    rr = pl.ds(r, 8)
                    old = _gate(mrun[h, rr, :], tok)
                    v = []
                    for q in (2 * h, 2 * h + 1):
                        for t in range(2):
                            v.append(buf[q, rr, pl.ds(t * LANES, LANES)])
                            if copy_to is not None:
                                copy_to[q, rr, pl.ds(t * LANES, LANES)] = v[-1]
                    top = jnp.maximum(jnp.maximum(v[0], v[1]), jnp.maximum(v[2], v[3]))
                    m = jnp.maximum(old, jnp.where(valid, top, LOWEST))
                    e = [jnp.exp2(x - m) for x in v]
                    l = lrun[h, rr, :] * jnp.exp2(old - m)
                    lrun[h, rr, :] = l + jnp.where(valid, (e[0] + e[1]) + (e[2] + e[3]), 0.0)
                    mrun[h, rr, :] = m

        def finish_stats(n):
            for h in range(2):
                for r in range(0, H, n):
                    tok = yield
                    rr = pl.ds(r, n)
                    m = jnp.max(_gate(mrun[h, rr, :], tok), axis=-1, keepdims=True)
                    mfin[h, rr, :] = jnp.broadcast_to(m, (n, LANES))
            for h in range(2):
                for r in range(0, H, n):
                    tok = yield
                    rr = pl.ds(r, n)
                    e = jnp.exp2(_gate(mrun[h, rr, :], tok) - mfin[h, rr, :])
                    l = jnp.sum(lrun[h, rr, :] * e, axis=-1, keepdims=True)
                    linv[h, rr, :] = jnp.broadcast_to(1.0 / l, (n, LANES))
                    mrun[h, rr, :] = jnp.full((n, LANES), LOWEST, F32)
                    lrun[h, rr, :] = jnp.zeros((n, LANES), F32)

        def probs(c, buf, k, r0=0, r1=Q):
            valid = valid_keys(c)
            for r in range(r0, r1, 8):
                for t in range(4):
                    tok = yield
                    rr, cols = pl.ds((t // 2) * Q + r, 8), pl.ds((t % 2) * LANES, LANES)
                    top = _gate(jnp.full((8, LANES), jnp.inf, F32), tok)
                    m = [jnp.where(valid, mfin[h, rr, :], top) for h in range(2)]
                    il = [linv[h, rr, :] for h in range(2)]
                    p = [jnp.exp2(buf[q, rr, cols] - m[q // 2]) * il[q // 2] for q in range(4)]
                    for o, v in enumerate(_combos(_LHS, p)):
                        pbuf[o, t, pl.ds(r, 8), pl.ds(k * LANES, LANES)] = v

        def pv_unit(u, hook, r0=0, r1=Q):
            rows = pl.ds(r0, r1 - r0)
            keys = pl.ds(_al(u * CU * LANES, LANES), CU * LANES)
            for n in range(49):
                lhs = _combo(_LHS, n % 7, lambda t: pbuf[n // 7, t, rows, :])
                v = _mm(lhs, vr[n, keys, :])
                acc[n, rows, :] = jnp.where(u > 0, acc[n, rows, :], 0.0) + v
                hook(n, v)

        def attn_rows():
            for r in range(0, Q, 8):
                tok = yield
                inner = []
                for o in range(7):
                    m = [acc[7 * o + i, pl.ds(r, 8), :] for i in range(7)]
                    m[2], m[3] = _gate(m[2], tok), _gate(m[3], tok)
                    inner.append(_out_combos(m))
                for t in range(4):
                    for q, v in enumerate(_out_combos([inner[o][t] for o in range(7)])):
                        sx[q, pl.ds((t // 2) * Q + r, 8), pl.ds((t % 2) * LANES, LANES)] = v

        def conv(j, t, h):
            r0 = j * BQ + h * H
            shift = HALO - KT // 2
            for a in range(0, H // 8, CV):
                o = None
                cnt = 0
                for r in range(8):
                    taps = [i for i in range(KT) if (i + shift) % 8 == r]
                    lo, hi = (taps[0] + shift) // 8, (taps[-1] + shift) // 8
                    g = gs[t, pl.ds(r0 + 8 * (a + lo) + r, 8 * (CV + hi - lo)), :].reshape(CV + hi - lo, 8, LANES)
                    for i in taps:
                        w = dwb[t, i]
                        if cnt % CG == 0:
                            tok = yield
                            w = _gate(w, tok)
                        cnt += 1
                        k = (i + shift) // 8 - lo
                        term = g[k:k + CV] * w[None]
                        o = term if o is None else o + term
                uc[t, pl.ds(h * H + 8 * a, 8 * CV), :] = (
                    us[t, pl.ds(_al(r0 + 8 * a, 8), 8 * CV), :] * o.reshape(8 * CV, LANES))

        def conv_unit(j, u, weights):
            per = 2 * NT // NU
            steps = per * (H // 8 // CV) * -(-KT // CG)
            return _stream(_chain([conv(j, u * (per // 2) + k // 2, k % 2) for k in range(per)]), steps, weights)

        def first(c):
            p = jnp.maximum(c - 1, 0)
            se = _stream(sumexp(jnp.where(c > 0, p, NC), ss.at[p]), H // 4, w_s0)
            qk_unit(0, c, ss.at[c], _spread([se], _never(c)))

        def steady(j, u):
            never = _never(u)
            sv = ss.at[pl.ds(u * CU, CU)]
            nq = 14 * CU
            pc = _stream(_chain([probs(u * CU + k, sv.at[k], k) for k in list(range(1, CU)) + [0]]),
                         CU * Q // 2, w_pc * CU)
            for k in range(CU):
                qk_unit(j + 1, u * CU + k, sv.at[k] if k else sx, _spread([pc], never, 14 * k))
            se = _stream(_chain([sumexp(u * CU + k, sv.at[k] if k else sx, None if k else sv.at[0])
                                 for k in range(CU)]), CU * H // 4, (1,) * w_se + (0,) * (49 - w_se))
            cv = conv_unit(j, u, (w_cv[0],) * w_se + (w_cv[1],) * (49 - w_se))
            pv_unit(u, _spread([cv, se], never))

        def last_probs(u, r0, r1):
            return _chain([probs(u * CU + k, ss.at[u * CU + k], k, r0, r1) for k in range(CU)])

        def last(u):
            never = _never(u)
            cv = conv_unit(NQ - 1, u, (1,) * 98)
            pc = _stream(last_probs(u, QS, Q), CU * (Q - QS) // 2, (1,) * 49)
            pv_unit(u, _spread([pc, cv], never), 0, QS)
            pc = _stream(last_probs(jnp.minimum(u + 1, NU - 1), 0, QS), CU * QS // 2, (0,) * 49 + (1,) * 49)
            pv_unit(u, _spread([pc, cv], never, 49), QS, Q)

        def finish_block(b, j, slot):
            def quad(q):
                return jnp.concatenate([uc[2 * (q % 2) + t, pl.ds((q // 2) * H, H), :] for t in range(2)], axis=1)

            def fin(q, v):
                if q in (1, 2):
                    tq[q] = v
                cols = pl.ds((q % 2) * DH, DH)
                obuf[slot, pl.ds((q // 2) * H, H), cols] = (
                    x_rows(b, j, q // 2, 0, H, cols) + (sx[q] + v)).astype(BF16)
                if q in (0, 3):
                    ocopy(b, j, q // 2).start()
            streams = [_stream(attn_rows(), Q // 8, w_fin), _stream(finish_stats(8), H // 2, w_st)]
            _strassen(lambda i: _mm(_combo(_LHS, i, quad), wr[DOWN, i]), tq, tq, fin, _spread(streams, _never(j)))

        def batch(b):
            def project_block(j):
                f = b * NQ + j + 1
                nxt = jnp.minimum(f, B * NQ - 1)

                @pl.when(f < B * NQ)
                def _():
                    xcopy(nxt // NQ, nxt % NQ).wait()
                project(j, nxt // NQ, nxt % NQ)
            with scope("pA"):
                _loop(NQ, project_block)
            with scope("Q0"):
                _loop(NC, first, UQ)

            def first_stats():
                for _ in sumexp(NC - 1, ss.at[NC - 1]):
                    pass
                _drain(finish_stats(80))

            with scope("st0"):
                @pl.when(b == 0)
                def _():
                    wcopy[4].wait()
                    wcopy[5].wait()
                    w = _dot(wtmp[4], wtmp[5])
                    store_weights(DOWN, w[:DH], w[DH:])
                    first_stats()

                @pl.when(b > 0)
                def _():
                    first_stats()

            def query_block(j):
                @pl.when(j < NQ - 1)
                def _():
                    with scope("steady"):
                        _loop(NU, lambda u: steady(j, u))

                @pl.when(j == NQ - 1)
                def _():
                    with scope("last"):
                        _drain(last_probs(0, 0, QS))
                        _loop(NU, last)
                f = b * NQ + j

                @pl.when(f >= 2)
                def _():
                    for h in range(2):
                        ocopy((f - 2) // NQ, (f - 2) % NQ, h).wait()
                with scope("sb"):
                    finish_block(b, j, f % 2)
            _loop(NQ, query_block)
        _loop(B, batch)
        with scope("owait"):
            for j in (NQ - 2, NQ - 1):
                for h in range(2):
                    ocopy(B - 1, j, h).wait()

    def run(x, w_q, w_k, w_v, w_ao, w_up, dw, w_dn, w_merge):
        B, T, D = x.shape
        KT = dw.shape[0]
        DH, NT, Q = D // 2, D // LANES, H // 2
        NQ = T // (2 * H)
        NC = -(-(T // 4) // LANES)
        assert D == 4 * LANES and T % (2 * H) == 0 and NQ >= 2 and NC % CU == 0 and NC >= 4
        assert KT % 2 == 1 and 8 <= KT <= 2 * HALO - 1
        scratch = [
            pltpu.VMEM((B, T, D), BF16),
            pltpu.VMEM((7, D, D), BF16),
            pltpu.VMEM((D, 2 * D), BF16),
            pltpu.VMEM((KT, D), BF16),
            pltpu.VMEM((5, 7, DH, DH), BF16),
            pltpu.VMEM((NT, 2 * HALO, 8, LANES), F32),
            pltpu.VMEM((NQ, 7, 2, H, LANES), F32),
            pltpu.VMEM((7, 2, H, LANES), F32),
            pltpu.VMEM((49, NC * LANES, LANES), BF16),
            pltpu.VMEM((49, NC * LANES, LANES), BF16),
            pltpu.VMEM((NT, T + 2 * HALO, LANES), F32),
            pltpu.VMEM((NT, T, LANES), F32),
            pltpu.VMEM((NT, 2 * H, LANES), F32),
            pltpu.VMEM((NC, 4, H, DH), F32),
            pltpu.VMEM((4, H, DH), F32),
            pltpu.VMEM((3, H, DH), F32),
            pltpu.VMEM((4, Q, LANES), F32),
            pltpu.VMEM((4, 3, Q, LANES), F32),
            pltpu.VMEM((7, 4, Q, CU * LANES), F32),
            pltpu.VMEM((52, Q, LANES), F32),
            pltpu.VMEM((2, H, LANES), F32),
            pltpu.VMEM((2, H, LANES), F32),
            pltpu.VMEM((2, H, LANES), F32),
            pltpu.VMEM((2, H, LANES), F32),
            pltpu.VMEM((2, 2, H, LANES), F32),
            pltpu.VMEM((2, 2 * H, D), BF16),
            pltpu.SemaphoreType.DMA((9,)),
            pltpu.SemaphoreType.DMA((B * NQ,)),
            pltpu.SemaphoreType.DMA((4,)),
        ]
        anyspec = pl.BlockSpec(memory_space=pl.ANY)
        return pl.pallas_call(
            kernel,
            out_shape=jax.ShapeDtypeStruct(x.shape, x.dtype),
            grid=(1,),
            in_specs=[anyspec] * 9,
            out_specs=anyspec,
            scratch_shapes=scratch,
            compiler_params=pltpu.CompilerParams(vmem_limit_bytes=124 * 1024 * 1024),
        )(x, w_q, w_k, w_v, w_ao, w_up, dw, w_dn, w_merge)
    return jax.jit(run)


@jax.jit
def pallas_standalone__conformer_family_branchformer__speech_kernel(x, w_q, w_k, w_v, w_ao, w_up, dw, w_dn, w_merge):
    return make()(x, w_q, w_k, w_v, w_ao, w_up, dw, w_dn, w_merge)
```

```python
import contextlib
import math

import jax
import jax.numpy as jnp
import numpy as np
from jax import lax
import jax.experimental.pallas as pl
import jax.experimental.pallas.tpu as pltpu

F32 = jnp.float32
BF16 = jnp.bfloat16
LANES = 128
HALO = 16
EPS = 1e-5
LOWEST = float(np.finfo(np.float32).min)

_LHS = ((0, 3, 1), (2, 3, 1), (0, None, 0), (3, None, 0), (0, 1, 1), (2, 0, -1), (1, 3, -1))
_RHS = ((0, 3, 1), (0, None, 0), (1, 3, -1), (2, 0, -1), (3, None, 0), (0, 1, 1), (2, 3, 1))


def _combo(table, i, quad):
    a, b, sign = table[i]
    if b is None:
        return quad(a)
    return quad(a) + quad(b) if sign > 0 else quad(a) - quad(b)


def _combos(table, quads):
    return [_combo(table, i, quads.__getitem__) for i in range(7)]


def _out_combos(m):
    c12 = m[2] + m[4]
    c21 = m[1] + m[3]
    u = m[0] + m[3] + m[2]
    return [(u - c12) + m[6], c12, c21, (u - c21) + m[5]]


def _dot(a, b):
    return jnp.dot(a, b, preferred_element_type=F32)


def _mm(a, b):
    return lax.dot_general(a, b, (((1,), (0,)), ((), ())), preferred_element_type=F32)


def _mm_nt(a, b):
    return lax.dot_general(a, b, (((1,), (1,)), ((), ())), preferred_element_type=F32)


def _layernorm(x):
    m = jnp.mean(x, axis=-1, keepdims=True)
    d = x - m
    v = jnp.mean(d * d, axis=-1, keepdims=True)
    return d * lax.rsqrt(v + EPS)


def _gelu(x):
    c = math.sqrt(2.0 / math.pi)
    hx = 0.5 * x
    return hx + hx * jnp.tanh(x * (c + (c * 0.044715) * (x * x)))


def _al(i, m):
    return i if isinstance(i, int) else pl.multiple_of(i, m)


def _loop(n, f, unroll=1):
    def body(i, carry):
        for k in range(unroll):
            f(i * unroll + k)
        return carry
    lax.fori_loop(0, n // unroll, body, 0)


def _never(i):
    return lax.broadcasted_iota(jnp.int32, (8, LANES), 1) + i < 0


def _gate(x, tok):
    if tok is None:
        return x
    value, never = tok
    reps = (x.shape[0] // 8, x.shape[1] // LANES)
    return jnp.where(jnp.tile(never, reps), jnp.tile(value, reps), x)


def _stream(gen, steps, weights):
    next(gen)
    cum = [sum(weights[:k]) for k in range(len(weights) + 1)]
    return gen, [steps * cum[k + 1] // cum[-1] - steps * cum[k] // cum[-1] for k in range(len(weights))]


def _chain(gens):
    for g in gens:
        yield from g


def _drain(gen):
    for _ in gen:
        pass


def _spread(streams, never, first=0):
    def hook(k, v):
        todo = []
        for gen, counts in streams:
            cnt = counts[first + k]
            todo += [((v.shape[0] // 8) * n // cnt * 8, gen) for n in range(cnt)]
        todo.sort(key=lambda p: p[0])
        for r, gen in todo:
            try:
                gen.send((v[r:r + 8, :LANES], never))
            except StopIteration:
                pass
    return hook


def _strassen(product, tmp, out, fin, hook):
    v = product(3)
    tmp[2] = v
    hook(0, v)
    v = product(0) + tmp[2]
    tmp[0] = v
    hook(1, v)
    v = product(2)
    tmp[0] = tmp[0] + v
    tmp[1] = v
    hook(2, v)
    v = tmp[2] + product(1)
    fin(2, v)
    hook(3, v)
    v = (tmp[0] - out[2]) + product(5)
    fin(3, v)
    hook(4, v)
    v = tmp[1] + product(4)
    fin(1, v)
    hook(5, v)
    v = (tmp[0] - out[1]) + product(6)
    fin(0, v)
    hook(6, v)


def make(H=400, CU=4, CV=5, CG=3, UQ=2, QS=96, SC=False,
         w_se=40, w_cv=(1, 1), w_pc=(5, 4, 5, 4, 2, 2) + (4, 3) * 4, w_s0=(4, 3) * 3 + (0,) * 8,
         w_fin=(1, 1, 1, 1, 1, 0), w_st=(1, 1, 1, 1, 1, 0),
         a_fill=(("s", 0, (1,) * 5), ("n", 7, (1,) * 7), ("g", 8, (1,) * 10), ("k", 14, (1,) * 8),
                 ("v", 21, (1,) * 6))):
    def kernel(x_hbm, wq_hbm, wk_hbm, wv_hbm, wao_hbm, wup_hbm, dw_hbm, wdn_hbm, wm_hbm,
               o_hbm,
               xin, wtmp, wup, dwv, wr, dwb, ql, lnext, kr, vr, gs, us, uc, ss, sx, tq, ti, to, pbuf, acc,
               mrun, lrun, mfin, linv, xst, obuf,
               wsem, xsem, osem):
        B, T, D = xin.shape
        KT = dwv.shape[0]
        NT = D // LANES
        DH = D // 2
        BQ = 2 * H
        NQ = T // BQ
        Q = H // 2
        QM = Q // 64 * 64
        NC = ss.shape[0]
        NU = NC // CU
        UP, GATE, KEY, VAL, DOWN = range(5)
        scope = jax.named_scope if SC else (lambda n: contextlib.nullcontext())

        w_src = (wq_hbm, wk_hbm, wv_hbm, wao_hbm, wdn_hbm, wm_hbm.at[pl.ds(D, D)], wm_hbm.at[pl.ds(0, D)])
        wcopy = [pltpu.make_async_copy(s, wtmp.at[i], wsem.at[i]) for i, s in enumerate(w_src)]
        wup_copy = pltpu.make_async_copy(wup_hbm, wup, wsem.at[7])
        dw_copy = pltpu.make_async_copy(dw_hbm, dwv, wsem.at[8])

        def xcopy(b, j):
            rows = pl.ds(_al(j * BQ, BQ), BQ)
            return pltpu.make_async_copy(x_hbm.at[b, rows], xin.at[b, rows], xsem.at[b * NQ + j])

        def ocopy(b, j, h):
            slot = (b * NQ + j) % 2
            return pltpu.make_async_copy(obuf.at[slot, pl.ds(h * H, H)],
                                         o_hbm.at[b, pl.ds(_al(j * BQ + h * H, H), H)], osem.at[2 * slot + h])

        def x_rows(b, j, h, r, n, cols):
            return xin[b, pl.ds(_al(j * BQ + h * H + r, 8), n), cols].astype(F32)

        def norm_stats(b, j):
            for r in range(0, H, 16):
                for h in range(2):
                    tok = yield
                    v = x_rows(b, j, h, r, 16, slice(None))
                    v = jnp.concatenate([_gate(v[:, :LANES], tok), v[:, LANES:]], axis=1)
                    m = jnp.mean(v, axis=-1, keepdims=True)
                    d = v - m
                    rs = lax.rsqrt(jnp.mean(d * d, axis=-1, keepdims=True) + EPS)
                    xst[0, h, pl.ds(r, 16), :] = jnp.broadcast_to(m, (16, LANES))
                    xst[1, h, pl.ds(r, 16), :] = jnp.broadcast_to(rs, (16, LANES))

        def norm_apply(b, j):
            for r in range(0, H, 8):
                tok = yield
                mean = [_gate(xst[0, h, pl.ds(r, 8), :], tok) for h in range(2)]
                rstd = [xst[1, h, pl.ds(r, 8), :] for h in range(2)]
                for t in range(2):
                    a = [(x_rows(b, j, q // 2, r, 8, pl.ds((q % 2) * DH + t * LANES, LANES)) - mean[q // 2])
                         * rstd[q // 2] for q in range(4)]
                    for i, v in enumerate(_combos(_LHS, a)):
                        lnext[i, t, pl.ds(r, 8), :] = v

        def store_weights(m, top, bot, r=0):
            quads = [top[:, :DH], top[:, DH:], bot[:, :DH], bot[:, DH:]]
            for i, c in enumerate(_combos(_RHS, quads)):
                wr[m, i, pl.ds(r, top.shape[0]), :] = c.astype(BF16)

        for c in (wcopy[0], wcopy[1], wcopy[2], wcopy[3], dw_copy, xcopy(0, 0), wcopy[6], wup_copy):
            c.start()

        wcopy[0].wait()
        wcopy[1].wait()
        w = _mm_nt(wtmp[1], wtmp[0]) * (float(D) ** -0.5 * math.log2(math.e))
        store_weights(KEY, w[:DH], w[DH:])
        for ref in (kr, vr):
            pad = ref.shape[1] - T // 4
            ref[:, pl.ds(T // 4, pad), :] = jnp.zeros((49, pad, LANES), BF16)
        gs[:, pl.ds(0, HALO), :] = jnp.zeros((NT, HALO, LANES), F32)
        gs[:, pl.ds(HALO + T, HALO), :] = jnp.zeros((NT, HALO, LANES), F32)
        mrun[...] = jnp.full(mrun.shape, LOWEST, F32)
        lrun[...] = jnp.zeros(lrun.shape, F32)

        wcopy[2].wait()
        wcopy[3].wait()
        dw_copy.wait()
        wva = _dot(wtmp[2], wtmp[3]).astype(BF16)
        dwf = dwv[...].astype(F32)
        for t in range(NT):
            for i in range(KT):
                dwb[t, i] = jnp.broadcast_to(dwf[i:i + 1, t * LANES:(t + 1) * LANES], (8, LANES))
        acc[...] = jnp.zeros(acc.shape, F32)

        xcopy(0, 0).wait()
        wcopy[6].wait()
        xcopy(0, 1).start()
        w = _dot(wva, wtmp[6])
        side = _stream(_chain([norm_stats(0, 0), norm_apply(0, 0)]), H // 4, (1,) * 7 + (0,))
        hook = _spread([side], _never(pl.program_id(0)))
        for t in range(NT):
            for k in range(2):
                hook(2 * t + k, w[k * DH:(k + 1) * DH, t * LANES:(t + 1) * LANES])
        store_weights(VAL, w[:DH], w[DH:])

        wup_copy.wait()
        wcopy[4].start()
        wcopy[5].start()
        for f in range(2, B * NQ):
            xcopy(f // NQ, f % NQ).start()
        for m in (UP, GATE):
            for r in range(0, DH, 32):
                top, bot = (wup[pl.ds(k * DH + r, 32), pl.ds(m * D, D)].astype(F32) for k in range(2))
                store_weights(m, top, bot, r)

        def post_act(j, m):
            buf = ss.at[m]
            dst, off = (gs, HALO) if m == GATE else (us, 0)
            for h in (1, 0):
                for r in range(0, H, 8):
                    tok = yield
                    rr = pl.ds(r, 8)
                    v = _gelu(_gate(jnp.concatenate([buf[2 * h, rr, :], buf[2 * h + 1, rr, :]], axis=1), tok))
                    if m == GATE:
                        v = _layernorm(v)
                    rows = pl.ds(_al(j * BQ + h * H + r + off, 8), 8)
                    for t in range(NT):
                        dst[t, rows, :] = v[:, t * LANES:(t + 1) * LANES]

        def post_kv(j, m):
            buf = ss.at[m]
            dst = kr if m == KEY else vr
            perm = (0, 2, 1, 3) if m == KEY else (0, 1, 2, 3)
            for r in range(0, Q, 16):
                n = min(16, Q - r)
                pos = _al(j * QM + r, 16) if r < QM else _al(NQ * QM + j * (Q - QM) + r - QM, 8)
                for o in range(7):
                    tok = yield

                    def tile(t):
                        rows, cols = pl.ds((t // 2) * Q + r, n), pl.ds((t % 2) * LANES, LANES)
                        return _combo(_RHS, o, lambda q: buf[perm[q], rows, cols])
                    tiles = [_gate(tile(0), tok), tile(perm[1]), tile(perm[2]), _gate(tile(3), tok)]
                    for i, c in enumerate(_combos(_RHS, tiles)):
                        dst[7 * o + i, pl.ds(pos, n), :] = c.astype(BF16)

        def project(j, nb, nj):
            nkv = 7 * -(-Q // 16)
            gens = {"k": (post_kv(j, KEY), nkv), "v": (post_kv(j, VAL), nkv), "g": (post_act(j, GATE), H // 4),
                    "s": (norm_stats(nb, nj), H // 8), "n": (norm_apply(nb, nj), H // 8)}
            streams = [_stream(*gens[name], (0,) * pos + w + (0,) * (28 - pos - len(w))) for name, pos, w in a_fill]
            for pos, m in enumerate((GATE, KEY, VAL, UP)):
                buf = ss.at[m]

                def fin(q, v):
                    buf[q] = v

                def product(i):
                    if pos == 0:
                        v = [lnext[i, t] for t in range(2)]
                        for t in range(2):
                            ql[j, i, t] = v[t]
                    else:
                        v = [ql[j, i, t] for t in range(2)]
                    return _mm(jnp.concatenate(v, axis=1), wr[m, i])
                _strassen(product, buf, buf, fin, _spread(streams, _never(j), 7 * pos))
            _drain(post_act(j, UP))

        def valid_keys(c):
            return lax.broadcasted_iota(jnp.int32, (8, LANES), 1) < T // 4 - c * LANES

        def qk_unit(j, c, buf, hook):
            keys = pl.ds(_al(c * LANES, LANES), LANES)
            for n, o in enumerate((3, 0, 2, 1, 5, 4, 6)):
                def product(i):
                    lhs = _combo(_LHS, i, lambda t: ql[j, o, t % 2, pl.ds((t // 2) * Q, Q), :])
                    return _mm_nt(lhs, kr[7 * o + i, keys, :])

                def emit(t, v):
                    rows, cols = pl.ds((t // 2) * Q, Q), pl.ds((t % 2) * LANES, LANES)
                    if n == 0:
                        to[t, 2] = v
                    elif n == 1:
                        to[t, 0] = to[t, 2] + v
                    elif n == 2:
                        to[t, 0] = to[t, 0] + v
                        to[t, 1] = v
                    elif n == 3:
                        buf[2, rows, cols] = to[t, 2] + v
                    elif n == 4:
                        buf[3, rows, cols] = (to[t, 0] - buf[2, rows, cols]) + v
                    elif n == 5:
                        buf[1, rows, cols] = to[t, 1] + v
                    else:
                        buf[0, rows, cols] = (to[t, 0] - buf[1, rows, cols]) + v
                m3, m5, m2, m4 = product(2), product(4), product(1), product(3)
                ti[0] = m4 - m5
                ti[1] = m3 - m2
                c12 = m3 + m5
                emit(1, c12)
                emit(2, m2 + m4)
                hook(2 * n, c12)
                m1, m6, m7 = product(0), product(5), product(6)
                c22 = (m1 + ti[1]) + m6
                emit(3, c22)
                emit(0, (m1 + ti[0]) + m7)
                hook(2 * n + 1, c22)

        def sumexp(c, buf, copy_to=None):
            valid = valid_keys(c)
            for h in (1, 0):
                for r in range(0, H, 8):
                    tok = yield
                    rr = pl.ds(r, 8)
                    old = _gate(mrun[h, rr, :], tok)
                    v = []
                    for q in (2 * h, 2 * h + 1):
                        for t in range(2):
                            v.append(buf[q, rr, pl.ds(t * LANES, LANES)])
                            if copy_to is not None:
                                copy_to[q, rr, pl.ds(t * LANES, LANES)] = v[-1]
                    top = jnp.maximum(jnp.maximum(v[0], v[1]), jnp.maximum(v[2], v[3]))
                    m = jnp.maximum(old, jnp.where(valid, top, LOWEST))
                    e = [jnp.exp2(x - m) for x in v]
                    l = lrun[h, rr, :] * jnp.exp2(old - m)
                    lrun[h, rr, :] = l + jnp.where(valid, (e[0] + e[1]) + (e[2] + e[3]), 0.0)
                    mrun[h, rr, :] = m

        def finish_stats(n):
            for h in range(2):
                for r in range(0, H, n):
                    tok = yield
                    rr = pl.ds(r, n)
                    m = jnp.max(_gate(mrun[h, rr, :], tok), axis=-1, keepdims=True)
                    mfin[h, rr, :] = jnp.broadcast_to(m, (n, LANES))
            for h in range(2):
                for r in range(0, H, n):
                    tok = yield
                    rr = pl.ds(r, n)
                    e = jnp.exp2(_gate(mrun[h, rr, :], tok) - mfin[h, rr, :])
                    l = jnp.sum(lrun[h, rr, :] * e, axis=-1, keepdims=True)
                    linv[h, rr, :] = jnp.broadcast_to(1.0 / l, (n, LANES))
                    mrun[h, rr, :] = jnp.full((n, LANES), LOWEST, F32)
                    lrun[h, rr, :] = jnp.zeros((n, LANES), F32)

        def probs(c, buf, k, r0=0, r1=Q):
            valid = valid_keys(c)
            for r in range(r0, r1, 8):
                for t in range(4):
                    tok = yield
                    rr, cols = pl.ds((t // 2) * Q + r, 8), pl.ds((t % 2) * LANES, LANES)
                    top = _gate(jnp.full((8, LANES), jnp.inf, F32), tok)
                    m = [jnp.where(valid, mfin[h, rr, :], top) for h in range(2)]
                    il = [linv[h, rr, :] for h in range(2)]
                    p = [jnp.exp2(buf[q, rr, cols] - m[q // 2]) * il[q // 2] for q in range(4)]
                    for o, v in enumerate(_combos(_LHS, p)):
                        pbuf[o, t, pl.ds(r, 8), pl.ds(k * LANES, LANES)] = v

        def pv_unit(u, hook, r0=0, r1=Q):
            rows = pl.ds(r0, r1 - r0)
            keys = pl.ds(_al(u * CU * LANES, LANES), CU * LANES)
            for n in range(49):
                lhs = _combo(_LHS, n % 7, lambda t: pbuf[n // 7, t, rows, :])
                v = _mm(lhs, vr[n, keys, :])
                acc[n, rows, :] = jnp.where(u > 0, acc[n, rows, :], 0.0) + v
                hook(n, v)

        def attn_rows():
            for r in range(0, Q, 8):
                tok = yield
                inner = []
                for o in range(7):
                    m = [acc[7 * o + i, pl.ds(r, 8), :] for i in range(7)]
                    m[2], m[3] = _gate(m[2], tok), _gate(m[3], tok)
                    inner.append(_out_combos(m))
                for t in range(4):
                    for q, v in enumerate(_out_combos([inner[o][t] for o in range(7)])):
                        sx[q, pl.ds((t // 2) * Q + r, 8), pl.ds((t % 2) * LANES, LANES)] = v

        def conv(j, t, h):
            r0 = j * BQ + h * H
            shift = HALO - KT // 2
            for a in range(0, H // 8, CV):
                o = None
                cnt = 0
                for r in range(8):
                    taps = [i for i in range(KT) if (i + shift) % 8 == r]
                    lo, hi = (taps[0] + shift) // 8, (taps[-1] + shift) // 8
                    g = gs[t, pl.ds(r0 + 8 * (a + lo) + r, 8 * (CV + hi - lo)), :].reshape(CV + hi - lo, 8, LANES)
                    for i in taps:
                        w = dwb[t, i]
                        if cnt % CG == 0:
                            tok = yield
                            w = _gate(w, tok)
                        cnt += 1
                        k = (i + shift) // 8 - lo
                        term = g[k:k + CV] * w[None]
                        o = term if o is None else o + term
                uc[t, pl.ds(h * H + 8 * a, 8 * CV), :] = (
                    us[t, pl.ds(_al(r0 + 8 * a, 8), 8 * CV), :] * o.reshape(8 * CV, LANES))

        def conv_unit(j, u, weights):
            per = 2 * NT // NU
            steps = per * (H // 8 // CV) * -(-KT // CG)
            return _stream(_chain([conv(j, u * (per // 2) + k // 2, k % 2) for k in range(per)]), steps, weights)

        def first(c):
            p = jnp.maximum(c - 1, 0)
            se = _stream(sumexp(jnp.where(c > 0, p, NC), ss.at[p]), H // 4, w_s0)
            qk_unit(0, c, ss.at[c], _spread([se], _never(c)))

        def steady(j, u):
            never = _never(u)
            sv = ss.at[pl.ds(u * CU, CU)]
            nq = 14 * CU
            pc = _stream(_chain([probs(u * CU + k, sv.at[k], k) for k in list(range(1, CU)) + [0]]),
                         CU * Q // 2, w_pc * CU)
            for k in range(CU):
                qk_unit(j + 1, u * CU + k, sv.at[k] if k else sx, _spread([pc], never, 14 * k))
            se = _stream(_chain([sumexp(u * CU + k, sv.at[k] if k else sx, None if k else sv.at[0])
                                 for k in range(CU)]), CU * H // 4, (1,) * w_se + (0,) * (49 - w_se))
            cv = conv_unit(j, u, (w_cv[0],) * w_se + (w_cv[1],) * (49 - w_se))
            pv_unit(u, _spread([cv, se], never))

        def last_probs(u, r0, r1):
            return _chain([probs(u * CU + k, ss.at[u * CU + k], k, r0, r1) for k in range(CU)])

        def last(u):
            never = _never(u)
            cv = conv_unit(NQ - 1, u, (1,) * 98)
            pc = _stream(last_probs(u, QS, Q), CU * (Q - QS) // 2, (1,) * 49)
            pv_unit(u, _spread([pc, cv], never), 0, QS)
            pc = _stream(last_probs(jnp.minimum(u + 1, NU - 1), 0, QS), CU * QS // 2, (0,) * 49 + (1,) * 49)
            pv_unit(u, _spread([pc, cv], never, 49), QS, Q)

        def finish_block(b, j, slot):
            def quad(q):
                return jnp.concatenate([uc[2 * (q % 2) + t, pl.ds((q // 2) * H, H), :] for t in range(2)], axis=1)

            def fin(q, v):
                cols = pl.ds((q % 2) * DH, DH)
                obuf[slot, pl.ds((q // 2) * H, H), cols] = (
                    x_rows(b, j, q // 2, 0, H, cols) + (sx[q] + v)).astype(BF16)

            def product(i):
                return _mm(_combo(_LHS, i, quad), wr[DOWN, i])
            hook = _spread([_stream(attn_rows(), Q // 8, w_fin), _stream(finish_stats(8), H // 2, w_st)], _never(j))
            v = product(0)
            tq[0] = v
            hook(0, v)
            v = tq[0] + product(6)
            tq[1] = v
            hook(1, v)
            v = tq[0] + product(5)
            tq[0] = v
            hook(2, v)
            v = product(2)
            tq[0] = tq[0] + v
            tq[2] = v
            hook(3, v)
            v = product(3)
            tq[1] = tq[1] + v
            tq[3] = v
            hook(4, v)
            v = product(1)
            fin(2, tq[3] + v)
            fin(3, tq[0] - v)
            ocopy(b, j, 1).start()
            hook(5, v)
            v = product(4)
            fin(1, tq[2] + v)
            fin(0, tq[1] - v)
            ocopy(b, j, 0).start()

        def batch(b):
            def project_block(j):
                f = b * NQ + j + 1
                nxt = jnp.minimum(f, B * NQ - 1)

                @pl.when(f < B * NQ)
                def _():
                    xcopy(nxt // NQ, nxt % NQ).wait()
                project(j, nxt // NQ, nxt % NQ)
            with scope("pA"):
                _loop(NQ, project_block)
            with scope("Q0"):
                _loop(NC, first, UQ)

            def first_stats():
                for _ in sumexp(NC - 1, ss.at[NC - 1]):
                    pass
                _drain(finish_stats(80))

            with scope("st0"):
                @pl.when(b == 0)
                def _():
                    wcopy[4].wait()
                    wcopy[5].wait()
                    w = _dot(wtmp[4], wtmp[5])
                    store_weights(DOWN, w[:DH], w[DH:])
                    first_stats()

                @pl.when(b > 0)
                def _():
                    first_stats()

            def query_block(j):
                @pl.when(j < NQ - 1)
                def _():
                    with scope("steady"):
                        _loop(NU, lambda u: steady(j, u))

                @pl.when(j == NQ - 1)
                def _():
                    with scope("last"):
                        _drain(last_probs(0, 0, QS))
                        _loop(NU, last)
                f = b * NQ + j

                @pl.when(f >= 2)
                def _():
                    for h in range(2):
                        ocopy((f - 2) // NQ, (f - 2) % NQ, h).wait()
                with scope("sb"):
                    finish_block(b, j, f % 2)
            _loop(NQ, query_block)
        _loop(B, batch)
        with scope("owait"):
            for j in (NQ - 2, NQ - 1):
                for h in range(2):
                    ocopy(B - 1, j, h).wait()

    def run(x, w_q, w_k, w_v, w_ao, w_up, dw, w_dn, w_merge):
        B, T, D = x.shape
        KT = dw.shape[0]
        DH, NT, Q = D // 2, D // LANES, H // 2
        NQ = T // (2 * H)
        NC = -(-(T // 4) // LANES)
        assert D == 4 * LANES and T % (2 * H) == 0 and NQ >= 2 and NC % CU == 0 and NC >= 4
        assert KT % 2 == 1 and 8 <= KT <= 2 * HALO - 1
        scratch = [
            pltpu.VMEM((B, T, D), BF16),
            pltpu.VMEM((7, D, D), BF16),
            pltpu.VMEM((D, 2 * D), BF16),
            pltpu.VMEM((KT, D), BF16),
            pltpu.VMEM((5, 7, DH, DH), BF16),
            pltpu.VMEM((NT, 2 * HALO, 8, LANES), F32),
            pltpu.VMEM((NQ, 7, 2, H, LANES), F32),
            pltpu.VMEM((7, 2, H, LANES), F32),
            pltpu.VMEM((49, NC * LANES, LANES), BF16),
            pltpu.VMEM((49, NC * LANES, LANES), BF16),
            pltpu.VMEM((NT, T + 2 * HALO, LANES), F32),
            pltpu.VMEM((NT, T, LANES), F32),
            pltpu.VMEM((NT, 2 * H, LANES), F32),
            pltpu.VMEM((NC, 4, H, DH), F32),
            pltpu.VMEM((4, H, DH), F32),
            pltpu.VMEM((4, H, DH), F32),
            pltpu.VMEM((4, Q, LANES), F32),
            pltpu.VMEM((4, 3, Q, LANES), F32),
            pltpu.VMEM((7, 4, Q, CU * LANES), F32),
            pltpu.VMEM((52, Q, LANES), F32),
            pltpu.VMEM((2, H, LANES), F32),
            pltpu.VMEM((2, H, LANES), F32),
            pltpu.VMEM((2, H, LANES), F32),
            pltpu.VMEM((2, H, LANES), F32),
            pltpu.VMEM((2, 2, H, LANES), F32),
            pltpu.VMEM((2, 2 * H, D), BF16),
            pltpu.SemaphoreType.DMA((9,)),
            pltpu.SemaphoreType.DMA((B * NQ,)),
            pltpu.SemaphoreType.DMA((4,)),
        ]
        anyspec = pl.BlockSpec(memory_space=pl.ANY)
        return pl.pallas_call(
            kernel,
            out_shape=jax.ShapeDtypeStruct(x.shape, x.dtype),
            grid=(1,),
            in_specs=[anyspec] * 9,
            out_specs=anyspec,
            scratch_shapes=scratch,
            compiler_params=pltpu.CompilerParams(vmem_limit_bytes=124 * 1024 * 1024),
        )(x, w_q, w_k, w_v, w_ao, w_up, dw, w_dn, w_merge)
    return jax.jit(run)


@jax.jit
def pallas_standalone__conformer_family_branchformer__speech_kernel(x, w_q, w_k, w_v, w_ao, w_up, dw, w_dn, w_merge):
    return make()(x, w_q, w_k, w_v, w_ao, w_up, dw, w_dn, w_merge)
```

```python
import math

import jax
import jax.numpy as jnp
import numpy as np
from jax import lax
import jax.experimental.pallas as pl
import jax.experimental.pallas.tpu as pltpu

F32 = jnp.float32
BF16 = jnp.bfloat16
LANES = 128
HALO = 16
EPS = 1e-5
LOWEST = float(np.finfo(np.float32).min)

H = 400
CU = 4
CV, CG = 5, 3
QS = 96
W_SE = 40
W_PC = (5, 4, 5, 4, 2, 2) + (4, 3) * 4
W_S0 = (4, 3) * 3 + (0,) * 8
W_FIN = (1, 1, 1, 1, 1, 0)
A_FILL = (("s", 0, 5), ("n", 7, 7), ("g", 8, 10), ("k", 14, 8), ("v", 21, 6))

_LHS = ((0, 3, 1), (2, 3, 1), (0, None, 0), (3, None, 0), (0, 1, 1), (2, 0, -1), (1, 3, -1))
_RHS = ((0, 3, 1), (0, None, 0), (1, 3, -1), (2, 0, -1), (3, None, 0), (0, 1, 1), (2, 3, 1))


def _combo(table, i, quad):
    a, b, sign = table[i]
    if b is None:
        return quad(a)
    return quad(a) + quad(b) if sign > 0 else quad(a) - quad(b)


def _combos(table, quads):
    return [_combo(table, i, quads.__getitem__) for i in range(7)]


def _out_combos(m):
    c12 = m[2] + m[4]
    c21 = m[1] + m[3]
    u = m[0] + m[3] + m[2]
    return [(u - c12) + m[6], c12, c21, (u - c21) + m[5]]


def _dot(a, b):
    return jnp.dot(a, b, preferred_element_type=F32)


def _mm(a, b):
    return lax.dot_general(a, b, (((1,), (0,)), ((), ())), preferred_element_type=F32)


def _mm_nt(a, b):
    return lax.dot_general(a, b, (((1,), (1,)), ((), ())), preferred_element_type=F32)


def _layernorm(x):
    m = jnp.mean(x, axis=-1, keepdims=True)
    d = x - m
    v = jnp.mean(d * d, axis=-1, keepdims=True)
    return d * lax.rsqrt(v + EPS)


def _gelu(x):
    c = math.sqrt(2.0 / math.pi)
    hx = 0.5 * x
    return hx + hx * jnp.tanh(x * (c + (c * 0.044715) * (x * x)))


def _al(i, m):
    return i if isinstance(i, int) else pl.multiple_of(i, m)


def _loop(n, f, unroll=1):
    def body(i, carry):
        for k in range(unroll):
            f(i * unroll + k)
        return carry
    lax.fori_loop(0, n // unroll, body, 0)


def _never(i):
    return lax.broadcasted_iota(jnp.int32, (8, LANES), 1) + i < 0


def _gate(x, tok):
    if tok is None:
        return x
    value, never = tok
    reps = (x.shape[0] // 8, x.shape[1] // LANES)
    return jnp.where(jnp.tile(never, reps), jnp.tile(value, reps), x)


def _stream(gen, steps, weights):
    next(gen)
    cum = [sum(weights[:k]) for k in range(len(weights) + 1)]
    return gen, [steps * cum[k + 1] // cum[-1] - steps * cum[k] // cum[-1] for k in range(len(weights))]


def _chain(gens):
    for g in gens:
        yield from g


def _drain(gen):
    for _ in gen:
        pass


def _spread(streams, never, first=0):
    def hook(k, v):
        todo = []
        for gen, counts in streams:
            cnt = counts[first + k]
            todo += [((v.shape[0] // 8) * n // cnt * 8, gen) for n in range(cnt)]
        todo.sort(key=lambda p: p[0])
        for r, gen in todo:
            try:
                gen.send((v[r:r + 8, :LANES], never))
            except StopIteration:
                pass
    return hook


def _strassen(product, tmp, out, fin, hook):
    v = product(3)
    tmp[2] = v
    hook(0, v)
    v = product(0) + tmp[2]
    tmp[0] = v
    hook(1, v)
    v = product(2)
    tmp[0] = tmp[0] + v
    tmp[1] = v
    hook(2, v)
    v = tmp[2] + product(1)
    fin(2, v)
    hook(3, v)
    v = (tmp[0] - out[2]) + product(5)
    fin(3, v)
    hook(4, v)
    v = tmp[1] + product(4)
    fin(1, v)
    hook(5, v)
    v = (tmp[0] - out[1]) + product(6)
    fin(0, v)
    hook(6, v)


def _kernel(x_hbm, wq_hbm, wk_hbm, wv_hbm, wao_hbm, wup_hbm, dw_hbm, wdn_hbm, wm_hbm,
            o_hbm,
            xin, wtmp, wup, dwv, wr, dwb, ql, lnext, kr, vr, gs, us, uc, ss, sx, tq, ti, to, pbuf, acc,
            mrun, lrun, mfin, linv, xst, obuf,
            wsem, xsem, osem):
    B, T, D = xin.shape
    KT = dwv.shape[0]
    NT = D // LANES
    DH = D // 2
    BQ = 2 * H
    NQ = T // BQ
    Q = H // 2
    QM = Q // 64 * 64
    NC = ss.shape[0]
    NU = NC // CU
    UP, GATE, KEY, VAL, DOWN = range(5)

    w_src = (wq_hbm, wk_hbm, wv_hbm, wao_hbm, wdn_hbm, wm_hbm.at[pl.ds(D, D)], wm_hbm.at[pl.ds(0, D)])
    wcopy = [pltpu.make_async_copy(s, wtmp.at[i], wsem.at[i]) for i, s in enumerate(w_src)]
    wup_copy = pltpu.make_async_copy(wup_hbm, wup, wsem.at[7])
    dw_copy = pltpu.make_async_copy(dw_hbm, dwv, wsem.at[8])

    def xcopy(b, j):
        rows = pl.ds(_al(j * BQ, BQ), BQ)
        return pltpu.make_async_copy(x_hbm.at[b, rows], xin.at[b, rows], xsem.at[b * NQ + j])

    def ocopy(b, j, h):
        slot = (b * NQ + j) % 2
        return pltpu.make_async_copy(obuf.at[slot, pl.ds(h * H, H)],
                                     o_hbm.at[b, pl.ds(_al(j * BQ + h * H, H), H)], osem.at[2 * slot + h])

    def x_rows(b, j, h, r, n, cols):
        return xin[b, pl.ds(_al(j * BQ + h * H + r, 8), n), cols].astype(F32)

    def norm_stats(b, j):
        for r in range(0, H, 16):
            for h in range(2):
                tok = yield
                v = x_rows(b, j, h, r, 16, slice(None))
                v = jnp.concatenate([_gate(v[:, :LANES], tok), v[:, LANES:]], axis=1)
                m = jnp.mean(v, axis=-1, keepdims=True)
                d = v - m
                rs = lax.rsqrt(jnp.mean(d * d, axis=-1, keepdims=True) + EPS)
                xst[0, h, pl.ds(r, 16), :] = jnp.broadcast_to(m, (16, LANES))
                xst[1, h, pl.ds(r, 16), :] = jnp.broadcast_to(rs, (16, LANES))

    def norm_apply(b, j):
        for r in range(0, H, 8):
            tok = yield
            mean = [_gate(xst[0, h, pl.ds(r, 8), :], tok) for h in range(2)]
            rstd = [xst[1, h, pl.ds(r, 8), :] for h in range(2)]
            for t in range(2):
                a = [(x_rows(b, j, q // 2, r, 8, pl.ds((q % 2) * DH + t * LANES, LANES)) - mean[q // 2])
                     * rstd[q // 2] for q in range(4)]
                for i, v in enumerate(_combos(_LHS, a)):
                    lnext[i, t, pl.ds(r, 8), :] = v

    def store_weights(m, top, bot, r=0):
        quads = [top[:, :DH], top[:, DH:], bot[:, :DH], bot[:, DH:]]
        for i, c in enumerate(_combos(_RHS, quads)):
            wr[m, i, pl.ds(r, top.shape[0]), :] = c.astype(BF16)

    for c in (wcopy[0], wcopy[1], wcopy[2], wcopy[3], dw_copy, xcopy(0, 0), wcopy[6], wup_copy):
        c.start()

    wcopy[0].wait()
    wcopy[1].wait()
    w = _mm_nt(wtmp[1], wtmp[0]) * (float(D) ** -0.5 * math.log2(math.e))
    store_weights(KEY, w[:DH], w[DH:])
    for ref in (kr, vr):
        pad = ref.shape[1] - T // 4
        ref[:, pl.ds(T // 4, pad), :] = jnp.zeros((49, pad, LANES), BF16)
    gs[:, pl.ds(0, HALO), :] = jnp.zeros((NT, HALO, LANES), F32)
    gs[:, pl.ds(HALO + T, HALO), :] = jnp.zeros((NT, HALO, LANES), F32)
    mrun[...] = jnp.full(mrun.shape, LOWEST, F32)
    lrun[...] = jnp.zeros(lrun.shape, F32)

    wcopy[2].wait()
    wcopy[3].wait()
    dw_copy.wait()
    wva = _dot(wtmp[2], wtmp[3]).astype(BF16)
    dwf = dwv[...].astype(F32)
    for t in range(NT):
        for i in range(KT):
            dwb[t, i] = jnp.broadcast_to(dwf[i:i + 1, t * LANES:(t + 1) * LANES], (8, LANES))
    acc[...] = jnp.zeros(acc.shape, F32)

    xcopy(0, 0).wait()
    wcopy[6].wait()
    xcopy(0, 1).start()
    w = _dot(wva, wtmp[6])
    side = _stream(_chain([norm_stats(0, 0), norm_apply(0, 0)]), H // 4, (1,) * 7 + (0,))
    hook = _spread([side], _never(pl.program_id(0)))
    for t in range(NT):
        for k in range(2):
            hook(2 * t + k, w[k * DH:(k + 1) * DH, t * LANES:(t + 1) * LANES])
    store_weights(VAL, w[:DH], w[DH:])

    wup_copy.wait()
    wcopy[4].start()
    wcopy[5].start()
    for f in range(2, B * NQ):
        xcopy(f // NQ, f % NQ).start()
    for m in (UP, GATE):
        for r in range(0, DH, 32):
            top, bot = (wup[pl.ds(k * DH + r, 32), pl.ds(m * D, D)].astype(F32) for k in range(2))
            store_weights(m, top, bot, r)

    def post_act(j, m):
        buf = ss.at[m]
        dst, off = (gs, HALO) if m == GATE else (us, 0)
        for h in (1, 0):
            for r in range(0, H, 8):
                tok = yield
                rr = pl.ds(r, 8)
                v = _gelu(_gate(jnp.concatenate([buf[2 * h, rr, :], buf[2 * h + 1, rr, :]], axis=1), tok))
                if m == GATE:
                    v = _layernorm(v)
                rows = pl.ds(_al(j * BQ + h * H + r + off, 8), 8)
                for t in range(NT):
                    dst[t, rows, :] = v[:, t * LANES:(t + 1) * LANES]

    def post_kv(j, m):
        buf = ss.at[m]
        dst = kr if m == KEY else vr
        perm = (0, 2, 1, 3) if m == KEY else (0, 1, 2, 3)
        for r in range(0, Q, 16):
            n = min(16, Q - r)
            pos = _al(j * QM + r, 16) if r < QM else _al(NQ * QM + j * (Q - QM) + r - QM, 8)
            for o in range(7):
                tok = yield

                def tile(t):
                    rows, cols = pl.ds((t // 2) * Q + r, n), pl.ds((t % 2) * LANES, LANES)
                    return _combo(_RHS, o, lambda q: buf[perm[q], rows, cols])
                tiles = [_gate(tile(0), tok), tile(perm[1]), tile(perm[2]), _gate(tile(3), tok)]
                for i, c in enumerate(_combos(_RHS, tiles)):
                    dst[7 * o + i, pl.ds(pos, n), :] = c.astype(BF16)

    def project(j, nb, nj):
        nkv = 7 * -(-Q // 16)
        gens = {"k": (post_kv(j, KEY), nkv), "v": (post_kv(j, VAL), nkv), "g": (post_act(j, GATE), H // 4),
                "s": (norm_stats(nb, nj), H // 8), "n": (norm_apply(nb, nj), H // 8)}
        streams = [_stream(*gens[name], (0,) * pos + (1,) * n + (0,) * (28 - pos - n))
                   for name, pos, n in A_FILL]
        for pos, m in enumerate((GATE, KEY, VAL, UP)):
            buf = ss.at[m]

            def fin(q, v):
                buf[q] = v

            def product(i):
                if pos == 0:
                    v = [lnext[i, t] for t in range(2)]
                    for t in range(2):
                        ql[j, i, t] = v[t]
                else:
                    v = [ql[j, i, t] for t in range(2)]
                return _mm(jnp.concatenate(v, axis=1), wr[m, i])
            _strassen(product, buf, buf, fin, _spread(streams, _never(j), 7 * pos))
        _drain(post_act(j, UP))

    def valid_keys(c):
        return lax.broadcasted_iota(jnp.int32, (8, LANES), 1) < T // 4 - c * LANES

    def qk_unit(j, c, buf, hook):
        keys = pl.ds(_al(c * LANES, LANES), LANES)
        for n, o in enumerate((3, 0, 2, 1, 5, 4, 6)):
            def product(i):
                lhs = _combo(_LHS, i, lambda t: ql[j, o, t % 2, pl.ds((t // 2) * Q, Q), :])
                return _mm_nt(lhs, kr[7 * o + i, keys, :])

            def emit(t, v):
                rows, cols = pl.ds((t // 2) * Q, Q), pl.ds((t % 2) * LANES, LANES)
                if n == 0:
                    to[t, 2] = v
                elif n == 1:
                    to[t, 0] = to[t, 2] + v
                elif n == 2:
                    to[t, 0] = to[t, 0] + v
                    to[t, 1] = v
                elif n == 3:
                    buf[2, rows, cols] = to[t, 2] + v
                elif n == 4:
                    buf[3, rows, cols] = (to[t, 0] - buf[2, rows, cols]) + v
                elif n == 5:
                    buf[1, rows, cols] = to[t, 1] + v
                else:
                    buf[0, rows, cols] = (to[t, 0] - buf[1, rows, cols]) + v
            m3, m5, m2, m4 = product(2), product(4), product(1), product(3)
            ti[0] = m4 - m5
            ti[1] = m3 - m2
            c12 = m3 + m5
            emit(1, c12)
            emit(2, m2 + m4)
            hook(2 * n, c12)
            m1, m6, m7 = product(0), product(5), product(6)
            c22 = (m1 + ti[1]) + m6
            emit(3, c22)
            emit(0, (m1 + ti[0]) + m7)
            hook(2 * n + 1, c22)

    def sumexp(c, buf, copy_to=None):
        valid = valid_keys(c)
        for h in (1, 0):
            for r in range(0, H, 8):
                tok = yield
                rr = pl.ds(r, 8)
                old = _gate(mrun[h, rr, :], tok)
                v = []
                for q in (2 * h, 2 * h + 1):
                    for t in range(2):
                        v.append(buf[q, rr, pl.ds(t * LANES, LANES)])
                        if copy_to is not None:
                            copy_to[q, rr, pl.ds(t * LANES, LANES)] = v[-1]
                top = jnp.maximum(jnp.maximum(v[0], v[1]), jnp.maximum(v[2], v[3]))
                m = jnp.maximum(old, jnp.where(valid, top, LOWEST))
                e = [jnp.exp2(x - m) for x in v]
                l = lrun[h, rr, :] * jnp.exp2(old - m)
                lrun[h, rr, :] = l + jnp.where(valid, (e[0] + e[1]) + (e[2] + e[3]), 0.0)
                mrun[h, rr, :] = m

    def finish_stats(n):
        for h in range(2):
            for r in range(0, H, n):
                tok = yield
                rr = pl.ds(r, n)
                m = jnp.max(_gate(mrun[h, rr, :], tok), axis=-1, keepdims=True)
                mfin[h, rr, :] = jnp.broadcast_to(m, (n, LANES))
        for h in range(2):
            for r in range(0, H, n):
                tok = yield
                rr = pl.ds(r, n)
                e = jnp.exp2(_gate(mrun[h, rr, :], tok) - mfin[h, rr, :])
                l = jnp.sum(lrun[h, rr, :] * e, axis=-1, keepdims=True)
                linv[h, rr, :] = jnp.broadcast_to(1.0 / l, (n, LANES))
                mrun[h, rr, :] = jnp.full((n, LANES), LOWEST, F32)
                lrun[h, rr, :] = jnp.zeros((n, LANES), F32)

    def probs(c, buf, k, r0=0, r1=Q):
        valid = valid_keys(c)
        for r in range(r0, r1, 8):
            for t in range(4):
                tok = yield
                rr, cols = pl.ds((t // 2) * Q + r, 8), pl.ds((t % 2) * LANES, LANES)
                top = _gate(jnp.full((8, LANES), jnp.inf, F32), tok)
                m = [jnp.where(valid, mfin[h, rr, :], top) for h in range(2)]
                il = [linv[h, rr, :] for h in range(2)]
                p = [jnp.exp2(buf[q, rr, cols] - m[q // 2]) * il[q // 2] for q in range(4)]
                for o, v in enumerate(_combos(_LHS, p)):
                    pbuf[o, t, pl.ds(r, 8), pl.ds(k * LANES, LANES)] = v

    def pv_unit(u, hook, r0=0, r1=Q):
        rows = pl.ds(r0, r1 - r0)
        keys = pl.ds(_al(u * CU * LANES, LANES), CU * LANES)
        for n in range(49):
            lhs = _combo(_LHS, n % 7, lambda t: pbuf[n // 7, t, rows, :])
            v = _mm(lhs, vr[n, keys, :])
            acc[n, rows, :] = jnp.where(u > 0, acc[n, rows, :], 0.0) + v
            hook(n, v)

    def attn_rows():
        for r in range(0, Q, 8):
            tok = yield
            inner = []
            for o in range(7):
                m = [acc[7 * o + i, pl.ds(r, 8), :] for i in range(7)]
                m[2], m[3] = _gate(m[2], tok), _gate(m[3], tok)
                inner.append(_out_combos(m))
            for t in range(4):
                for q, v in enumerate(_out_combos([inner[o][t] for o in range(7)])):
                    sx[q, pl.ds((t // 2) * Q + r, 8), pl.ds((t % 2) * LANES, LANES)] = v

    def conv(j, t, h):
        r0 = j * BQ + h * H
        shift = HALO - KT // 2
        for a in range(0, H // 8, CV):
            o = None
            cnt = 0
            for r in range(8):
                taps = [i for i in range(KT) if (i + shift) % 8 == r]
                lo, hi = (taps[0] + shift) // 8, (taps[-1] + shift) // 8
                g = gs[t, pl.ds(r0 + 8 * (a + lo) + r, 8 * (CV + hi - lo)), :].reshape(CV + hi - lo, 8, LANES)
                for i in taps:
                    w = dwb[t, i]
                    if cnt % CG == 0:
                        tok = yield
                        w = _gate(w, tok)
                    cnt += 1
                    k = (i + shift) // 8 - lo
                    term = g[k:k + CV] * w[None]
                    o = term if o is None else o + term
            uc[t, pl.ds(h * H + 8 * a, 8 * CV), :] = (
                us[t, pl.ds(_al(r0 + 8 * a, 8), 8 * CV), :] * o.reshape(8 * CV, LANES))

    def conv_unit(j, u, weights):
        per = 2 * NT // NU
        steps = per * (H // 8 // CV) * -(-KT // CG)
        return _stream(_chain([conv(j, u * (per // 2) + k // 2, k % 2) for k in range(per)]), steps, weights)

    def first(c):
        p = jnp.maximum(c - 1, 0)
        se = _stream(sumexp(jnp.where(c > 0, p, NC), ss.at[p]), H // 4, W_S0)
        qk_unit(0, c, ss.at[c], _spread([se], _never(c)))

    def steady(j, u):
        never = _never(u)
        sv = ss.at[pl.ds(u * CU, CU)]
        nq = 14 * CU
        pc = _stream(_chain([probs(u * CU + k, sv.at[k], k) for k in list(range(1, CU)) + [0]]),
                     CU * Q // 2, W_PC * CU)
        for k in range(CU):
            qk_unit(j + 1, u * CU + k, sv.at[k] if k else sx, _spread([pc], never, 14 * k))
        se = _stream(_chain([sumexp(u * CU + k, sv.at[k] if k else sx, None if k else sv.at[0])
                             for k in range(CU)]), CU * H // 4, (1,) * W_SE + (0,) * (49 - W_SE))
        cv = conv_unit(j, u, (1,) * 49)
        pv_unit(u, _spread([cv, se], never))

    def last_probs(u, r0, r1):
        return _chain([probs(u * CU + k, ss.at[u * CU + k], k, r0, r1) for k in range(CU)])

    def last(u):
        never = _never(u)
        cv = conv_unit(NQ - 1, u, (1,) * 98)
        pc = _stream(last_probs(u, QS, Q), CU * (Q - QS) // 2, (1,) * 49)
        pv_unit(u, _spread([pc, cv], never), 0, QS)
        pc = _stream(last_probs(jnp.minimum(u + 1, NU - 1), 0, QS), CU * QS // 2, (0,) * 49 + (1,) * 49)
        pv_unit(u, _spread([pc, cv], never, 49), QS, Q)

    def finish_block(b, j, slot):
        def quad(q):
            return jnp.concatenate([uc[2 * (q % 2) + t, pl.ds((q // 2) * H, H), :] for t in range(2)], axis=1)

        def fin(q, v):
            cols = pl.ds((q % 2) * DH, DH)
            obuf[slot, pl.ds((q // 2) * H, H), cols] = (
                x_rows(b, j, q // 2, 0, H, cols) + (sx[q] + v)).astype(BF16)

        def product(i):
            return _mm(_combo(_LHS, i, quad), wr[DOWN, i])
        hook = _spread([_stream(attn_rows(), Q // 8, W_FIN), _stream(finish_stats(8), H // 2, W_FIN)], _never(j))
        v = product(0)
        tq[0] = v
        hook(0, v)
        v = tq[0] + product(6)
        tq[1] = v
        hook(1, v)
        v = tq[0] + product(5)
        tq[0] = v
        hook(2, v)
        v = product(2)
        tq[0] = tq[0] + v
        tq[2] = v
        hook(3, v)
        v = product(3)
        tq[1] = tq[1] + v
        tq[3] = v
        hook(4, v)
        v = product(1)
        fin(2, tq[3] + v)
        fin(3, tq[0] - v)
        ocopy(b, j, 1).start()
        hook(5, v)
        v = product(4)
        fin(1, tq[2] + v)
        fin(0, tq[1] - v)
        ocopy(b, j, 0).start()

    def batch(b):
        def project_block(j):
            f = b * NQ + j + 1
            nxt = jnp.minimum(f, B * NQ - 1)

            @pl.when(f < B * NQ)
            def _():
                xcopy(nxt // NQ, nxt % NQ).wait()
            project(j, nxt // NQ, nxt % NQ)
        _loop(NQ, project_block)
        _loop(NC, first, 2)

        def first_stats():
            _drain(sumexp(NC - 1, ss.at[NC - 1]))
            _drain(finish_stats(80))

        @pl.when(b == 0)
        def _():
            wcopy[4].wait()
            wcopy[5].wait()
            w = _dot(wtmp[4], wtmp[5])
            store_weights(DOWN, w[:DH], w[DH:])
            first_stats()

        @pl.when(b > 0)
        def _():
            first_stats()

        def query_block(j):
            @pl.when(j < NQ - 1)
            def _():
                _loop(NU, lambda u: steady(j, u))

            @pl.when(j == NQ - 1)
            def _():
                _drain(last_probs(0, 0, QS))
                _loop(NU, last)
            f = b * NQ + j

            @pl.when(f >= 2)
            def _():
                for h in range(2):
                    ocopy((f - 2) // NQ, (f - 2) % NQ, h).wait()
            finish_block(b, j, f % 2)
        _loop(NQ, query_block)
    _loop(B, batch)
    for j in (NQ - 2, NQ - 1):
        for h in range(2):
            ocopy(B - 1, j, h).wait()


@jax.jit
def pallas_standalone__conformer_family_branchformer__speech_kernel(
        x, w_q, w_k, w_v, w_ao, w_up, dw, w_dn, w_merge):
    B, T, D = x.shape
    KT = dw.shape[0]
    DH, NT, Q = D // 2, D // LANES, H // 2
    NQ = T // (2 * H)
    NC = -(-(T // 4) // LANES)
    assert D == 4 * LANES and T % (2 * H) == 0 and NQ >= 2 and NC % CU == 0 and NC >= 4
    assert KT % 2 == 1 and 8 <= KT <= 2 * HALO - 1
    scratch = [
        pltpu.VMEM((B, T, D), BF16),
        pltpu.VMEM((7, D, D), BF16),
        pltpu.VMEM((D, 2 * D), BF16),
        pltpu.VMEM((KT, D), BF16),
        pltpu.VMEM((5, 7, DH, DH), BF16),
        pltpu.VMEM((NT, 2 * HALO, 8, LANES), F32),
        pltpu.VMEM((NQ, 7, 2, H, LANES), F32),
        pltpu.VMEM((7, 2, H, LANES), F32),
        pltpu.VMEM((49, NC * LANES, LANES), BF16),
        pltpu.VMEM((49, NC * LANES, LANES), BF16),
        pltpu.VMEM((NT, T + 2 * HALO, LANES), F32),
        pltpu.VMEM((NT, T, LANES), F32),
        pltpu.VMEM((NT, 2 * H, LANES), F32),
        pltpu.VMEM((NC, 4, H, DH), F32),
        pltpu.VMEM((4, H, DH), F32),
        pltpu.VMEM((4, H, DH), F32),
        pltpu.VMEM((4, Q, LANES), F32),
        pltpu.VMEM((4, 3, Q, LANES), F32),
        pltpu.VMEM((7, 4, Q, CU * LANES), F32),
        pltpu.VMEM((52, Q, LANES), F32),
        pltpu.VMEM((2, H, LANES), F32),
        pltpu.VMEM((2, H, LANES), F32),
        pltpu.VMEM((2, H, LANES), F32),
        pltpu.VMEM((2, H, LANES), F32),
        pltpu.VMEM((2, 2, H, LANES), F32),
        pltpu.VMEM((2, 2 * H, D), BF16),
        pltpu.SemaphoreType.DMA((9,)),
        pltpu.SemaphoreType.DMA((B * NQ,)),
        pltpu.SemaphoreType.DMA((4,)),
    ]
    anyspec = pl.BlockSpec(memory_space=pl.ANY)
    return pl.pallas_call(
        _kernel,
        out_shape=jax.ShapeDtypeStruct(x.shape, x.dtype),
        grid=(1,),
        in_specs=[anyspec] * 9,
        out_specs=anyspec,
        scratch_shapes=scratch,
        compiler_params=pltpu.CompilerParams(vmem_limit_bytes=124 * 1024 * 1024),
    )(x, w_q, w_k, w_v, w_ao, w_up, dw, w_dn, w_merge)
```

```python
import math

import jax
import jax.numpy as jnp
import numpy as np
from jax import lax
import jax.experimental.pallas as pl
import jax.experimental.pallas.tpu as pltpu

F32 = jnp.float32
BF16 = jnp.bfloat16
LANES = 128
HALO = 16
EPS = 1e-5
LOWEST = float(np.finfo(np.float32).min)

H = 400
CU = 4
CV, CG = 5, 3
QS = 96
W_SE = 40
W_PC = (5, 4, 5, 4, 2, 2) + (4, 3) * 4
W_S0 = (4, 3) * 2 + (0,) * 10
W_S1 = (0,) * 9 + (1, 1, 1, 1, 0)
W_FIN = (1, 1, 1, 1, 1, 0)
A_FILL = (("s", 0, 5), ("n", 7, 7), ("g", 8, 10), ("k", 14, 8), ("v", 21, 6))

_LHS = ((0, 3, 1), (2, 3, 1), (0, None, 0), (3, None, 0), (0, 1, 1), (2, 0, -1), (1, 3, -1))
_RHS = ((0, 3, 1), (0, None, 0), (1, 3, -1), (2, 0, -1), (3, None, 0), (0, 1, 1), (2, 3, 1))


def _combo(table, i, quad):
    a, b, sign = table[i]
    if b is None:
        return quad(a)
    return quad(a) + quad(b) if sign > 0 else quad(a) - quad(b)


def _combos(table, quads):
    return [_combo(table, i, quads.__getitem__) for i in range(7)]


def _out_combos(m):
    c12 = m[2] + m[4]
    c21 = m[1] + m[3]
    u = m[0] + m[3] + m[2]
    return [(u - c12) + m[6], c12, c21, (u - c21) + m[5]]


def _dot(a, b):
    return jnp.dot(a, b, preferred_element_type=F32)


def _mm(a, b):
    return lax.dot_general(a, b, (((1,), (0,)), ((), ())), preferred_element_type=F32)


def _mm_nt(a, b):
    return lax.dot_general(a, b, (((1,), (1,)), ((), ())), preferred_element_type=F32)


def _layernorm(x):
    m = jnp.mean(x, axis=-1, keepdims=True)
    d = x - m
    v = jnp.mean(d * d, axis=-1, keepdims=True)
    return d * lax.rsqrt(v + EPS)


def _gelu(x):
    c = math.sqrt(2.0 / math.pi)
    hx = 0.5 * x
    return hx + hx * jnp.tanh(x * (c + (c * 0.044715) * (x * x)))


def _al(i, m):
    return i if isinstance(i, int) else pl.multiple_of(i, m)


def _loop(n, f, unroll=1):
    def body(i, carry):
        for k in range(unroll):
            f(i * unroll + k)
        return carry
    lax.fori_loop(0, n // unroll, body, 0)


def _never(i):
    return lax.broadcasted_iota(jnp.int32, (8, LANES), 1) + i < 0


def _gate(x, tok):
    if tok is None:
        return x
    value, never = tok
    reps = (x.shape[0] // 8, x.shape[1] // LANES)
    return jnp.where(jnp.tile(never, reps), jnp.tile(value, reps), x)


def _stream(gen, steps, weights):
    next(gen)
    cum = [sum(weights[:k]) for k in range(len(weights) + 1)]
    return gen, [steps * cum[k + 1] // cum[-1] - steps * cum[k] // cum[-1] for k in range(len(weights))]


def _chain(gens):
    for g in gens:
        yield from g


def _drain(gen):
    for _ in gen:
        pass


def _spread(streams, never, first=0):
    def hook(k, v):
        todo = []
        for gen, counts in streams:
            cnt = counts[first + k]
            todo += [((v.shape[0] // 8) * n // cnt * 8, gen) for n in range(cnt)]
        todo.sort(key=lambda p: p[0])
        for r, gen in todo:
            try:
                gen.send((v[r:r + 8, :LANES], never))
            except StopIteration:
                pass
    return hook


def _strassen(product, tmp, out, fin, hook):
    v = product(3)
    tmp[2] = v
    hook(0, v)
    v = product(0) + tmp[2]
    tmp[0] = v
    hook(1, v)
    v = product(2)
    tmp[0] = tmp[0] + v
    tmp[1] = v
    hook(2, v)
    v = tmp[2] + product(1)
    fin(2, v)
    hook(3, v)
    v = (tmp[0] - out[2]) + product(5)
    fin(3, v)
    hook(4, v)
    v = tmp[1] + product(4)
    fin(1, v)
    hook(5, v)
    v = (tmp[0] - out[1]) + product(6)
    fin(0, v)
    hook(6, v)


def _kernel(x_hbm, wq_hbm, wk_hbm, wv_hbm, wao_hbm, wup_hbm, dw_hbm, wdn_hbm, wm_hbm,
            o_hbm,
            xin, wtmp, wup, dwv, wr, dwb, ql, lnext, kr, vr, gs, us, uc, ss, sx, tq, ti, to, pbuf, acc,
            mrun, lrun, mfin, linv, xst, obuf,
            wsem, xsem, osem):
    B, T, D = xin.shape
    KT = dwv.shape[0]
    NT = D // LANES
    DH = D // 2
    BQ = 2 * H
    NQ = T // BQ
    Q = H // 2
    QM = Q // 64 * 64
    NC = ss.shape[0]
    NU = NC // CU
    UP, GATE, KEY, VAL, DOWN = range(5)

    w_src = (wq_hbm, wk_hbm, wv_hbm, wao_hbm, wdn_hbm, wm_hbm.at[pl.ds(D, D)], wm_hbm.at[pl.ds(0, D)])
    wcopy = [pltpu.make_async_copy(s, wtmp.at[i], wsem.at[i]) for i, s in enumerate(w_src)]
    wup_copy = pltpu.make_async_copy(wup_hbm, wup, wsem.at[7])
    dw_copy = pltpu.make_async_copy(dw_hbm, dwv, wsem.at[8])

    def xcopy(b, j):
        rows = pl.ds(_al(j * BQ, BQ), BQ)
        return pltpu.make_async_copy(x_hbm.at[b, rows], xin.at[b, rows], xsem.at[b * NQ + j])

    def ocopy(b, j, h):
        slot = (b * NQ + j) % 2
        return pltpu.make_async_copy(obuf.at[slot, pl.ds(h * H, H)],
                                     o_hbm.at[b, pl.ds(_al(j * BQ + h * H, H), H)], osem.at[2 * slot + h])

    def x_rows(b, j, h, r, n, cols):
        return xin[b, pl.ds(_al(j * BQ + h * H + r, 8), n), cols].astype(F32)

    def norm_stats(b, j):
        for r in range(0, H, 16):
            for h in range(2):
                tok = yield
                v = x_rows(b, j, h, r, 16, slice(None))
                v = jnp.concatenate([_gate(v[:, :LANES], tok), v[:, LANES:]], axis=1)
                m = jnp.mean(v, axis=-1, keepdims=True)
                d = v - m
                rs = lax.rsqrt(jnp.mean(d * d, axis=-1, keepdims=True) + EPS)
                xst[0, h, pl.ds(r, 16), :] = jnp.broadcast_to(m, (16, LANES))
                xst[1, h, pl.ds(r, 16), :] = jnp.broadcast_to(rs, (16, LANES))

    def norm_apply(b, j):
        for r in range(0, H, 8):
            tok = yield
            mean = [_gate(xst[0, h, pl.ds(r, 8), :], tok) for h in range(2)]
            rstd = [xst[1, h, pl.ds(r, 8), :] for h in range(2)]
            for t in range(2):
                a = [(x_rows(b, j, q // 2, r, 8, pl.ds((q % 2) * DH + t * LANES, LANES)) - mean[q // 2])
                     * rstd[q // 2] for q in range(4)]
                for i, v in enumerate(_combos(_LHS, a)):
                    lnext[i, t, pl.ds(r, 8), :] = v

    def store_weights(m, top, bot, r=0):
        quads = [top[:, :DH], top[:, DH:], bot[:, :DH], bot[:, DH:]]
        for i, c in enumerate(_combos(_RHS, quads)):
            wr[m, i, pl.ds(r, top.shape[0]), :] = c.astype(BF16)

    for c in (wcopy[0], wcopy[1], wcopy[2], wcopy[3], dw_copy, xcopy(0, 0), wcopy[6], wup_copy):
        c.start()

    wcopy[0].wait()
    wcopy[1].wait()
    w = _mm_nt(wtmp[1], wtmp[0]) * (float(D) ** -0.5 * math.log2(math.e))
    store_weights(KEY, w[:DH], w[DH:])
    for ref in (kr, vr):
        pad = ref.shape[1] - T // 4
        ref[:, pl.ds(T // 4, pad), :] = jnp.zeros((49, pad, LANES), BF16)
    gs[:, pl.ds(0, HALO), :] = jnp.zeros((NT, HALO, LANES), F32)
    gs[:, pl.ds(HALO + T, HALO), :] = jnp.zeros((NT, HALO, LANES), F32)
    mrun[...] = jnp.full(mrun.shape, LOWEST, F32)
    lrun[...] = jnp.zeros(lrun.shape, F32)

    wcopy[2].wait()
    wcopy[3].wait()
    dw_copy.wait()
    wva = _dot(wtmp[2], wtmp[3]).astype(BF16)
    dwf = dwv[...].astype(F32)
    for t in range(NT):
        for i in range(KT):
            dwb[t, i] = jnp.broadcast_to(dwf[i:i + 1, t * LANES:(t + 1) * LANES], (8, LANES))
    acc[...] = jnp.zeros(acc.shape, F32)

    xcopy(0, 0).wait()
    wcopy[6].wait()
    xcopy(0, 1).start()
    w = _dot(wva, wtmp[6])
    side = _stream(_chain([norm_stats(0, 0), norm_apply(0, 0)]), H // 4, (1,) * 7 + (0,))
    hook = _spread([side], _never(pl.program_id(0)))
    for t in range(NT):
        for k in range(2):
            hook(2 * t + k, w[k * DH:(k + 1) * DH, t * LANES:(t + 1) * LANES])
    store_weights(VAL, w[:DH], w[DH:])

    wup_copy.wait()
    wcopy[4].start()
    wcopy[5].start()
    for f in range(2, B * NQ):
        xcopy(f // NQ, f % NQ).start()
    for m in (UP, GATE):
        for r in range(0, DH, 32):
            top, bot = (wup[pl.ds(k * DH + r, 32), pl.ds(m * D, D)].astype(F32) for k in range(2))
            store_weights(m, top, bot, r)

    def post_act(j, m):
        buf = ss.at[m]
        dst, off = (gs, HALO) if m == GATE else (us, 0)
        for h in (1, 0):
            for r in range(0, H, 8):
                tok = yield
                rr = pl.ds(r, 8)
                v = _gelu(_gate(jnp.concatenate([buf[2 * h, rr, :], buf[2 * h + 1, rr, :]], axis=1), tok))
                if m == GATE:
                    v = _layernorm(v)
                rows = pl.ds(_al(j * BQ + h * H + r + off, 8), 8)
                for t in range(NT):
                    dst[t, rows, :] = v[:, t * LANES:(t + 1) * LANES]

    def post_kv(j, m):
        buf = ss.at[m]
        dst = kr if m == KEY else vr
        perm = (0, 2, 1, 3) if m == KEY else (0, 1, 2, 3)
        for r in range(0, Q, 16):
            n = min(16, Q - r)
            pos = _al(j * QM + r, 16) if r < QM else _al(NQ * QM + j * (Q - QM) + r - QM, 8)
            for o in range(7):
                tok = yield

                def tile(t):
                    rows, cols = pl.ds((t // 2) * Q + r, n), pl.ds((t % 2) * LANES, LANES)
                    return _combo(_RHS, o, lambda q: buf[perm[q], rows, cols])
                tiles = [_gate(tile(0), tok), tile(perm[1]), tile(perm[2]), _gate(tile(3), tok)]
                for i, c in enumerate(_combos(_RHS, tiles)):
                    dst[7 * o + i, pl.ds(pos, n), :] = c.astype(BF16)

    def project(j, nb, nj):
        nkv = 7 * -(-Q // 16)
        gens = {"k": (post_kv(j, KEY), nkv), "v": (post_kv(j, VAL), nkv), "g": (post_act(j, GATE), H // 4),
                "s": (norm_stats(nb, nj), H // 8), "n": (norm_apply(nb, nj), H // 8)}
        streams = [_stream(*gens[name], (0,) * pos + (1,) * n + (0,) * (28 - pos - n))
                   for name, pos, n in A_FILL]
        for pos, m in enumerate((GATE, KEY, VAL, UP)):
            buf = ss.at[m]

            def fin(q, v):
                buf[q] = v

            def product(i):
                if pos == 0:
                    v = [lnext[i, t] for t in range(2)]
                    for t in range(2):
                        ql[j, i, t] = v[t]
                else:
                    v = [ql[j, i, t] for t in range(2)]
                return _mm(jnp.concatenate(v, axis=1), wr[m, i])
            _strassen(product, buf, buf, fin, _spread(streams, _never(j), 7 * pos))
        _drain(post_act(j, UP))

    def valid_keys(c):
        return lax.broadcasted_iota(jnp.int32, (8, LANES), 1) < T // 4 - c * LANES

    def qk_unit(j, c, buf, hook):
        keys = pl.ds(_al(c * LANES, LANES), LANES)
        for n, o in enumerate((3, 0, 2, 1, 5, 4, 6)):
            def product(i):
                lhs = _combo(_LHS, i, lambda t: ql[j, o, t % 2, pl.ds((t // 2) * Q, Q), :])
                return _mm_nt(lhs, kr[7 * o + i, keys, :])

            def emit(t, v):
                rows, cols = pl.ds((t // 2) * Q, Q), pl.ds((t % 2) * LANES, LANES)
                if n == 0:
                    to[t, 2] = v
                elif n == 1:
                    to[t, 0] = to[t, 2] + v
                elif n == 2:
                    to[t, 0] = to[t, 0] + v
                    to[t, 1] = v
                elif n == 3:
                    buf[2, rows, cols] = to[t, 2] + v
                elif n == 4:
                    buf[3, rows, cols] = (to[t, 0] - buf[2, rows, cols]) + v
                elif n == 5:
                    buf[1, rows, cols] = to[t, 1] + v
                else:
                    buf[0, rows, cols] = (to[t, 0] - buf[1, rows, cols]) + v
            m3, m5, m2, m4 = product(2), product(4), product(1), product(3)
            ti[0] = m4 - m5
            ti[1] = m3 - m2
            c12 = m3 + m5
            emit(1, c12)
            emit(2, m2 + m4)
            hook(2 * n, c12)
            m1, m6, m7 = product(0), product(5), product(6)
            c22 = (m1 + ti[1]) + m6
            emit(3, c22)
            emit(0, (m1 + ti[0]) + m7)
            hook(2 * n + 1, c22)

    def sumexp(c, buf, copy_to=None, halves=(1, 0)):
        valid = valid_keys(c)
        for h in halves:
            for r in range(0, H, 8):
                tok = yield
                rr = pl.ds(r, 8)
                old = _gate(mrun[h, rr, :], tok)
                v = []
                for q in (2 * h, 2 * h + 1):
                    for t in range(2):
                        v.append(buf[q, rr, pl.ds(t * LANES, LANES)])
                        if copy_to is not None:
                            copy_to[q, rr, pl.ds(t * LANES, LANES)] = v[-1]
                top = jnp.maximum(jnp.maximum(v[0], v[1]), jnp.maximum(v[2], v[3]))
                m = jnp.maximum(old, jnp.where(valid, top, LOWEST))
                e = [jnp.exp2(x - m) for x in v]
                l = lrun[h, rr, :] * jnp.exp2(old - m)
                lrun[h, rr, :] = l + jnp.where(valid, (e[0] + e[1]) + (e[2] + e[3]), 0.0)
                mrun[h, rr, :] = m

    def finish_stats(n):
        for h in range(2):
            for r in range(0, H, n):
                tok = yield
                rr = pl.ds(r, n)
                m = jnp.max(_gate(mrun[h, rr, :], tok), axis=-1, keepdims=True)
                mfin[h, rr, :] = jnp.broadcast_to(m, (n, LANES))
        for h in range(2):
            for r in range(0, H, n):
                tok = yield
                rr = pl.ds(r, n)
                e = jnp.exp2(_gate(mrun[h, rr, :], tok) - mfin[h, rr, :])
                l = jnp.sum(lrun[h, rr, :] * e, axis=-1, keepdims=True)
                linv[h, rr, :] = jnp.broadcast_to(1.0 / l, (n, LANES))
                mrun[h, rr, :] = jnp.full((n, LANES), LOWEST, F32)
                lrun[h, rr, :] = jnp.zeros((n, LANES), F32)

    def probs(c, buf, k, r0=0, r1=Q):
        valid = valid_keys(c)
        for r in range(r0, r1, 8):
            for t in range(4):
                tok = yield
                rr, cols = pl.ds((t // 2) * Q + r, 8), pl.ds((t % 2) * LANES, LANES)
                top = _gate(jnp.full((8, LANES), jnp.inf, F32), tok)
                m = [jnp.where(valid, mfin[h, rr, :], top) for h in range(2)]
                il = [linv[h, rr, :] for h in range(2)]
                p = [jnp.exp2(buf[q, rr, cols] - m[q // 2]) * il[q // 2] for q in range(4)]
                for o, v in enumerate(_combos(_LHS, p)):
                    pbuf[o, t, pl.ds(r, 8), pl.ds(k * LANES, LANES)] = v

    def pv_unit(u, hook, r0=0, r1=Q):
        rows = pl.ds(r0, r1 - r0)
        keys = pl.ds(_al(u * CU * LANES, LANES), CU * LANES)
        for n in range(49):
            lhs = _combo(_LHS, n % 7, lambda t: pbuf[n // 7, t, rows, :])
            v = _mm(lhs, vr[n, keys, :])
            acc[n, rows, :] = jnp.where(u > 0, acc[n, rows, :], 0.0) + v
            hook(n, v)

    def attn_rows():
        for r in range(0, Q, 8):
            tok = yield
            inner = []
            for o in range(7):
                m = [acc[7 * o + i, pl.ds(r, 8), :] for i in range(7)]
                m[2], m[3] = _gate(m[2], tok), _gate(m[3], tok)
                inner.append(_out_combos(m))
            for t in range(4):
                for q, v in enumerate(_out_combos([inner[o][t] for o in range(7)])):
                    sx[q, pl.ds((t // 2) * Q + r, 8), pl.ds((t % 2) * LANES, LANES)] = v

    def conv(j, t, h):
        r0 = j * BQ + h * H
        shift = HALO - KT // 2
        for a in range(0, H // 8, CV):
            o = None
            cnt = 0
            for r in range(8):
                taps = [i for i in range(KT) if (i + shift) % 8 == r]
                lo, hi = (taps[0] + shift) // 8, (taps[-1] + shift) // 8
                g = gs[t, pl.ds(r0 + 8 * (a + lo) + r, 8 * (CV + hi - lo)), :].reshape(CV + hi - lo, 8, LANES)
                for i in taps:
                    w = dwb[t, i]
                    if cnt % CG == 0:
                        tok = yield
                        w = _gate(w, tok)
                    cnt += 1
                    k = (i + shift) // 8 - lo
                    term = g[k:k + CV] * w[None]
                    o = term if o is None else o + term
            uc[t, pl.ds(h * H + 8 * a, 8 * CV), :] = (
                us[t, pl.ds(_al(r0 + 8 * a, 8), 8 * CV), :] * o.reshape(8 * CV, LANES))

    def conv_unit(j, u, weights):
        per = 2 * NT // NU
        steps = per * (H // 8 // CV) * -(-KT // CG)
        return _stream(_chain([conv(j, u * (per // 2) + k // 2, k % 2) for k in range(per)]), steps, weights)

    def first(c):
        p = jnp.maximum(c - 1, 0)
        se = [_stream(sumexp(jnp.where(c > 0, p, NC), ss.at[p], None, (0,)), H // 8, W_S0),
              _stream(sumexp(c, ss.at[c], None, (1,)), H // 8, W_S1)]
        qk_unit(0, c, ss.at[c], _spread(se, _never(c)))

    def steady(j, u):
        never = _never(u)
        sv = ss.at[pl.ds(u * CU, CU)]
        nq = 14 * CU
        pc = _stream(_chain([probs(u * CU + k, sv.at[k], k) for k in list(range(1, CU)) + [0]]),
                     CU * Q // 2, W_PC * CU)
        for k in range(CU):
            qk_unit(j + 1, u * CU + k, sv.at[k] if k else sx, _spread([pc], never, 14 * k))
        se = _stream(_chain([sumexp(u * CU + k, sv.at[k] if k else sx, None if k else sv.at[0])
                             for k in range(CU)]), CU * H // 4, (1,) * W_SE + (0,) * (49 - W_SE))
        cv = conv_unit(j, u, (1,) * 49)
        pv_unit(u, _spread([cv, se], never))

    def last_probs(u, r0, r1):
        return _chain([probs(u * CU + k, ss.at[u * CU + k], k, r0, r1) for k in range(CU)])

    def last(u):
        never = _never(u)
        cv = conv_unit(NQ - 1, u, (1,) * 98)
        pc = _stream(last_probs(u, QS, Q), CU * (Q - QS) // 2, (1,) * 49)
        pv_unit(u, _spread([pc, cv], never), 0, QS)
        pc = _stream(last_probs(jnp.minimum(u + 1, NU - 1), 0, QS), CU * QS // 2, (0,) * 49 + (1,) * 49)
        pv_unit(u, _spread([pc, cv], never, 49), QS, Q)

    def finish_block(b, j, slot):
        def quad(q):
            return jnp.concatenate([uc[2 * (q % 2) + t, pl.ds((q // 2) * H, H), :] for t in range(2)], axis=1)

        def fin(q, v):
            cols = pl.ds((q % 2) * DH, DH)
            obuf[slot, pl.ds((q // 2) * H, H), cols] = (
                x_rows(b, j, q // 2, 0, H, cols) + (sx[q] + v)).astype(BF16)

        def product(i):
            return _mm(_combo(_LHS, i, quad), wr[DOWN, i])
        hook = _spread([_stream(attn_rows(), Q // 8, W_FIN), _stream(finish_stats(8), H // 2, W_FIN)], _never(j))
        v = product(0)
        tq[0] = v
        hook(0, v)
        v = tq[0] + product(6)
        tq[1] = v
        hook(1, v)
        v = tq[0] + product(5)
        tq[0] = v
        hook(2, v)
        v = product(2)
        tq[0] = tq[0] + v
        tq[2] = v
        hook(3, v)
        v = product(3)
        tq[1] = tq[1] + v
        tq[3] = v
        hook(4, v)
        v = product(1)
        fin(2, tq[3] + v)
        fin(3, tq[0] - v)
        ocopy(b, j, 1).start()
        hook(5, v)
        v = product(4)
        fin(1, tq[2] + v)
        fin(0, tq[1] - v)
        ocopy(b, j, 0).start()

    def batch(b):
        def project_block(j):
            f = b * NQ + j + 1
            nxt = jnp.minimum(f, B * NQ - 1)

            @pl.when(f < B * NQ)
            def _():
                xcopy(nxt // NQ, nxt % NQ).wait()
            project(j, nxt // NQ, nxt % NQ)
        _loop(NQ, project_block)
        _loop(NC, first, 2)

        def first_stats():
            _drain(sumexp(NC - 1, ss.at[NC - 1], None, (0,)))
            _drain(finish_stats(80))

        @pl.when(b == 0)
        def _():
            wcopy[4].wait()
            wcopy[5].wait()
            w = _dot(wtmp[4], wtmp[5])
            store_weights(DOWN, w[:DH], w[DH:])
            first_stats()

        @pl.when(b > 0)
        def _():
            first_stats()

        def query_block(j):
            @pl.when(j < NQ - 1)
            def _():
                _loop(NU, lambda u: steady(j, u))

            @pl.when(j == NQ - 1)
            def _():
                _drain(last_probs(0, 0, QS))
                _loop(NU, last)
            f = b * NQ + j

            @pl.when(f >= 2)
            def _():
                for h in range(2):
                    ocopy((f - 2) // NQ, (f - 2) % NQ, h).wait()
            finish_block(b, j, f % 2)
        _loop(NQ, query_block)
    _loop(B, batch)
    for j in (NQ - 2, NQ - 1):
        for h in range(2):
            ocopy(B - 1, j, h).wait()


@jax.jit
def pallas_standalone__conformer_family_branchformer__speech_kernel(
        x, w_q, w_k, w_v, w_ao, w_up, dw, w_dn, w_merge):
    B, T, D = x.shape
    KT = dw.shape[0]
    DH, NT, Q = D // 2, D // LANES, H // 2
    NQ = T // (2 * H)
    NC = -(-(T // 4) // LANES)
    assert D == 4 * LANES and T % (2 * H) == 0 and NQ >= 2 and NC % CU == 0 and NC >= 4
    assert KT % 2 == 1 and 8 <= KT <= 2 * HALO - 1
    scratch = [
        pltpu.VMEM((B, T, D), BF16),
        pltpu.VMEM((7, D, D), BF16),
        pltpu.VMEM((D, 2 * D), BF16),
        pltpu.VMEM((KT, D), BF16),
        pltpu.VMEM((5, 7, DH, DH), BF16),
        pltpu.VMEM((NT, 2 * HALO, 8, LANES), F32),
        pltpu.VMEM((NQ, 7, 2, H, LANES), F32),
        pltpu.VMEM((7, 2, H, LANES), F32),
        pltpu.VMEM((49, NC * LANES, LANES), BF16),
        pltpu.VMEM((49, NC * LANES, LANES), BF16),
        pltpu.VMEM((NT, T + 2 * HALO, LANES), F32),
        pltpu.VMEM((NT, T, LANES), F32),
        pltpu.VMEM((NT, 2 * H, LANES), F32),
        pltpu.VMEM((NC, 4, H, DH), F32),
        pltpu.VMEM((4, H, DH), F32),
        pltpu.VMEM((4, H, DH), F32),
        pltpu.VMEM((4, Q, LANES), F32),
        pltpu.VMEM((4, 3, Q, LANES), F32),
        pltpu.VMEM((7, 4, Q, CU * LANES), F32),
        pltpu.VMEM((52, Q, LANES), F32),
        pltpu.VMEM((2, H, LANES), F32),
        pltpu.VMEM((2, H, LANES), F32),
        pltpu.VMEM((2, H, LANES), F32),
        pltpu.VMEM((2, H, LANES), F32),
        pltpu.VMEM((2, 2, H, LANES), F32),
        pltpu.VMEM((2, 2 * H, D), BF16),
        pltpu.SemaphoreType.DMA((9,)),
        pltpu.SemaphoreType.DMA((B * NQ,)),
        pltpu.SemaphoreType.DMA((4,)),
    ]
    anyspec = pl.BlockSpec(memory_space=pl.ANY)
    return pl.pallas_call(
        _kernel,
        out_shape=jax.ShapeDtypeStruct(x.shape, x.dtype),
        grid=(1,),
        in_specs=[anyspec] * 9,
        out_specs=anyspec,
        scratch_shapes=scratch,
        compiler_params=pltpu.CompilerParams(vmem_limit_bytes=124 * 1024 * 1024),
    )(x, w_q, w_k, w_v, w_ao, w_up, dw, w_dn, w_merge)
```

```python
import math

import jax
import jax.numpy as jnp
import numpy as np
from jax import lax
import jax.experimental.pallas as pl
import jax.experimental.pallas.tpu as pltpu

F32 = jnp.float32
BF16 = jnp.bfloat16
LANES = 128
HALO = 16
EPS = 1e-5
LOWEST = float(np.finfo(np.float32).min)

H = 400
CU = 4
CV, CG = 5, 3
QS = 96
W_SE = 40
W_PC = (5, 4, 5, 4, 2, 2) + (4, 3) * 4
W_S0 = (4, 3) * 2 + (0,) * 10
W_S1 = (1, 1, 1, 1, 0)
W_FIN = (1, 1, 1, 1, 1, 0)
A_FILL = (("s", 0, (4, 3) * 5), ("n", 21, (1,) * 6), ("g", 14, (1,) * 8), ("k", 22, (1,) * 7), ("v", 28, (1,) * 7))

_LHS = ((0, 3, 1), (2, 3, 1), (0, None, 0), (3, None, 0), (0, 1, 1), (2, 0, -1), (1, 3, -1))
_RHS = ((0, 3, 1), (0, None, 0), (1, 3, -1), (2, 0, -1), (3, None, 0), (0, 1, 1), (2, 3, 1))


def _combo(table, i, quad):
    a, b, sign = table[i]
    if b is None:
        return quad(a)
    return quad(a) + quad(b) if sign > 0 else quad(a) - quad(b)


def _combos(table, quads):
    return [_combo(table, i, quads.__getitem__) for i in range(7)]


def _out_combos(m):
    c12 = m[2] + m[4]
    c21 = m[1] + m[3]
    u = m[0] + m[3] + m[2]
    return [(u - c12) + m[6], c12, c21, (u - c21) + m[5]]


def _dot(a, b):
    return jnp.dot(a, b, preferred_element_type=F32)


def _mm(a, b):
    return lax.dot_general(a, b, (((1,), (0,)), ((), ())), preferred_element_type=F32)


def _mm_nt(a, b):
    return lax.dot_general(a, b, (((1,), (1,)), ((), ())), preferred_element_type=F32)


def _layernorm(x):
    m = jnp.mean(x, axis=-1, keepdims=True)
    d = x - m
    v = jnp.mean(d * d, axis=-1, keepdims=True)
    return d * lax.rsqrt(v + EPS)


def _gelu(x):
    c = math.sqrt(2.0 / math.pi)
    hx = 0.5 * x
    return hx + hx * jnp.tanh(x * (c + (c * 0.044715) * (x * x)))


def _al(i, m):
    return i if isinstance(i, int) else pl.multiple_of(i, m)


def _loop(n, f, unroll=1):
    def body(i, carry):
        for k in range(unroll):
            f(i * unroll + k)
        return carry
    lax.fori_loop(0, n // unroll, body, 0)


def _never(i):
    return lax.broadcasted_iota(jnp.int32, (8, LANES), 1) + i < 0


def _gate(x, tok):
    if tok is None:
        return x
    value, never = tok
    reps = (x.shape[0] // 8, x.shape[1] // LANES)
    return jnp.where(jnp.tile(never, reps), jnp.tile(value, reps), x)


def _stream(gen, steps, weights):
    next(gen)
    cum = [sum(weights[:k]) for k in range(len(weights) + 1)]
    return gen, [steps * cum[k + 1] // cum[-1] - steps * cum[k] // cum[-1] for k in range(len(weights))]


def _chain(gens):
    for g in gens:
        yield from g


def _drain(gen):
    for _ in gen:
        pass


def _spread(streams, never, first=0):
    def hook(k, v):
        todo = []
        for gen, counts in streams:
            cnt = counts[first + k]
            todo += [((v.shape[0] // 8) * n // cnt * 8, gen) for n in range(cnt)]
        todo.sort(key=lambda p: p[0])
        for r, gen in todo:
            try:
                gen.send((v[r:r + 8, :LANES], never))
            except StopIteration:
                pass
    return hook


def _strassen(product, tmp, out, fin, hook):
    v = product(3)
    tmp[2] = v
    hook(0, v)
    v = product(0) + tmp[2]
    tmp[0] = v
    hook(1, v)
    v = product(2)
    tmp[0] = tmp[0] + v
    tmp[1] = v
    hook(2, v)
    v = tmp[2] + product(1)
    fin(2, v)
    hook(3, v)
    v = (tmp[0] - out[2]) + product(5)
    fin(3, v)
    hook(4, v)
    v = tmp[1] + product(4)
    fin(1, v)
    hook(5, v)
    v = (tmp[0] - out[1]) + product(6)
    fin(0, v)
    hook(6, v)


def _kernel(x_hbm, wq_hbm, wk_hbm, wv_hbm, wao_hbm, wup_hbm, dw_hbm, wdn_hbm, wm_hbm,
            o_hbm,
            xin, wtmp, wup, dwv, wr, wg, dwb, ql, lnext, kr, vr, gs, us, uc, ss, sx, tq, ti, to, pbuf, acc,
            mrun, lrun, mfin, linv, xst, obuf,
            wsem, xsem, osem):
    B, T, D = xin.shape
    KT = dwv.shape[0]
    NT = D // LANES
    DH = D // 2
    BQ = 2 * H
    NQ = T // BQ
    Q = H // 2
    QM = Q // 64 * 64
    NC = ss.shape[0]
    NU = NC // CU
    UP, KEY, VAL, DOWN = range(4)
    GATE = 3

    w_src = (wq_hbm, wk_hbm, wv_hbm, wao_hbm, wdn_hbm, wm_hbm.at[pl.ds(D, D)], wm_hbm.at[pl.ds(0, D)])
    wcopy = [pltpu.make_async_copy(s, wtmp.at[i], wsem.at[i]) for i, s in enumerate(w_src)]
    wup_copy = pltpu.make_async_copy(wup_hbm, wup, wsem.at[7])
    dw_copy = pltpu.make_async_copy(dw_hbm, dwv, wsem.at[8])

    def xcopy(b, j):
        rows = pl.ds(_al(j * BQ, BQ), BQ)
        return pltpu.make_async_copy(x_hbm.at[b, rows], xin.at[b, rows], xsem.at[b * NQ + j])

    def ocopy(b, j, h):
        slot = (b * NQ + j) % 2
        return pltpu.make_async_copy(obuf.at[slot, pl.ds(h * H, H)],
                                     o_hbm.at[b, pl.ds(_al(j * BQ + h * H, H), H)], osem.at[2 * slot + h])

    def x_rows(b, j, h, r, n, cols):
        return xin[b, pl.ds(_al(j * BQ + h * H + r, 8), n), cols].astype(F32)

    def norm_stats(b, j):
        for r in range(0, H, 16):
            for h in range(2):
                tok = yield
                v = x_rows(b, j, h, r, 16, slice(None))
                v = jnp.concatenate([_gate(v[:, :LANES], tok), v[:, LANES:]], axis=1)
                m = jnp.mean(v, axis=-1, keepdims=True)
                d = v - m
                rs = lax.rsqrt(jnp.mean(d * d, axis=-1, keepdims=True) + EPS)
                xst[0, h, pl.ds(r, 16), :] = jnp.broadcast_to(m, (16, LANES))
                xst[1, h, pl.ds(r, 16), :] = jnp.broadcast_to(rs, (16, LANES))

    def norm_apply(b, j):
        for r in range(0, H, 8):
            tok = yield
            mean = [_gate(xst[0, h, pl.ds(r, 8), :], tok) for h in range(2)]
            rstd = [xst[1, h, pl.ds(r, 8), :] for h in range(2)]
            for t in range(2):
                a = [(x_rows(b, j, q // 2, r, 8, pl.ds((q % 2) * DH + t * LANES, LANES)) - mean[q // 2])
                     * rstd[q // 2] for q in range(4)]
                for i, v in enumerate(_combos(_LHS, a)):
                    lnext[i, t, pl.ds(r, 8), :] = v

    def store_weights(m, top, bot, r=0):
        quads = [top[:, :DH], top[:, DH:], bot[:, :DH], bot[:, DH:]]
        for i, c in enumerate(_combos(_RHS, quads)):
            wr[m, i, pl.ds(r, top.shape[0]), :] = c.astype(BF16)

    for c in (wcopy[0], wcopy[1], wcopy[2], wcopy[3], dw_copy, xcopy(0, 0), wcopy[6], wup_copy):
        c.start()

    wcopy[0].wait()
    wcopy[1].wait()
    w = _mm_nt(wtmp[1], wtmp[0]) * (float(D) ** -0.5 * math.log2(math.e))
    store_weights(KEY, w[:DH], w[DH:])
    for ref in (kr, vr):
        pad = ref.shape[1] - T // 4
        ref[:, pl.ds(T // 4, pad), :] = jnp.zeros((49, pad, LANES), BF16)
    gs[:, pl.ds(0, HALO), :] = jnp.zeros((NT, HALO, LANES), F32)
    gs[:, pl.ds(HALO + T, HALO), :] = jnp.zeros((NT, HALO, LANES), F32)
    mrun[...] = jnp.full(mrun.shape, LOWEST, F32)
    lrun[...] = jnp.zeros(lrun.shape, F32)

    wcopy[2].wait()
    wcopy[3].wait()
    dw_copy.wait()
    wva = _dot(wtmp[2], wtmp[3]).astype(BF16)
    dwf = dwv[...].astype(F32)
    for t in range(NT):
        for i in range(KT):
            dwb[t, i] = jnp.broadcast_to(dwf[i:i + 1, t * LANES:(t + 1) * LANES], (8, LANES))
    acc[...] = jnp.zeros(acc.shape, F32)

    xcopy(0, 0).wait()
    wcopy[6].wait()
    xcopy(0, 1).start()
    w = _dot(wva, wtmp[6])
    side = _stream(_chain([norm_stats(0, 0), norm_apply(0, 0)]), H // 4, (1,) * 7 + (0,))
    hook = _spread([side], _never(pl.program_id(0)))
    for t in range(NT):
        for k in range(2):
            hook(2 * t + k, w[k * DH:(k + 1) * DH, t * LANES:(t + 1) * LANES])
    store_weights(VAL, w[:DH], w[DH:])

    wup_copy.wait()
    wcopy[4].start()
    wcopy[5].start()
    for f in range(2, B * NQ):
        xcopy(f // NQ, f % NQ).start()
    for r in range(0, DH, 32):
        top, bot = (wup[pl.ds(k * DH + r, 32), pl.ds(0, D)].astype(F32) for k in range(2))
        store_weights(UP, top, bot, r)
    for r in range(0, LANES, 8):
        tiles = [[wup[pl.ds((q // 2) * DH + (t // 2) * LANES + r, 8),
                      pl.ds(D + (q % 2) * DH + (t % 2) * LANES, LANES)].astype(F32) for q in range(4)]
                 for t in range(4)]
        outer = [_combos(_RHS, quads) for quads in tiles]
        for o in range(7):
            for i, c in enumerate(_combos(_RHS, [outer[t][o] for t in range(4)])):
                wg[7 * o + i, pl.ds(r, 8), :] = c.astype(BF16)

    def strassen2(left, mm, buf, hook):
        for n, o in enumerate((3, 0, 2, 1, 5, 4, 6)):
            def product(i):
                return mm(_combo(_LHS, i, lambda t: left[o, t % 2, pl.ds((t // 2) * Q, Q), :]), 7 * o + i)

            def emit(t, v):
                rows, cols = pl.ds((t // 2) * Q, Q), pl.ds((t % 2) * LANES, LANES)
                if n == 0:
                    to[t, 2] = v
                elif n == 1:
                    to[t, 0] = to[t, 2] + v
                elif n == 2:
                    to[t, 0] = to[t, 0] + v
                    to[t, 1] = v
                elif n == 3:
                    buf[2, rows, cols] = to[t, 2] + v
                elif n == 4:
                    buf[3, rows, cols] = (to[t, 0] - buf[2, rows, cols]) + v
                elif n == 5:
                    buf[1, rows, cols] = to[t, 1] + v
                else:
                    buf[0, rows, cols] = (to[t, 0] - buf[1, rows, cols]) + v
            m3, m5, m2, m4 = product(2), product(4), product(1), product(3)
            ti[0] = m4 - m5
            ti[1] = m3 - m2
            c12 = m3 + m5
            emit(1, c12)
            emit(2, m2 + m4)
            hook(2 * n, c12)
            m1, m6, m7 = product(0), product(5), product(6)
            c22 = (m1 + ti[1]) + m6
            emit(3, c22)
            emit(0, (m1 + ti[0]) + m7)
            hook(2 * n + 1, c22)

    def post_act(j, m):
        buf = ss.at[m]
        dst, off = (gs, HALO) if m == GATE else (us, 0)
        for h in (1, 0):
            for r in range(0, H, 8):
                tok = yield
                rr = pl.ds(r, 8)
                v = _gelu(_gate(jnp.concatenate([buf[2 * h, rr, :], buf[2 * h + 1, rr, :]], axis=1), tok))
                if m == GATE:
                    v = _layernorm(v)
                rows = pl.ds(_al(j * BQ + h * H + r + off, 8), 8)
                for t in range(NT):
                    dst[t, rows, :] = v[:, t * LANES:(t + 1) * LANES]

    def post_kv(j, m):
        buf = ss.at[m]
        dst = kr if m == KEY else vr
        perm = (0, 2, 1, 3) if m == KEY else (0, 1, 2, 3)
        for r in range(0, Q, 16):
            n = min(16, Q - r)
            pos = _al(j * QM + r, 16) if r < QM else _al(NQ * QM + j * (Q - QM) + r - QM, 8)
            for o in range(7):
                tok = yield

                def tile(t):
                    rows, cols = pl.ds((t // 2) * Q + r, n), pl.ds((t % 2) * LANES, LANES)
                    return _combo(_RHS, o, lambda q: buf[perm[q], rows, cols])
                tiles = [_gate(tile(0), tok), tile(perm[1]), tile(perm[2]), _gate(tile(3), tok)]
                for i, c in enumerate(_combos(_RHS, tiles)):
                    dst[7 * o + i, pl.ds(pos, n), :] = c.astype(BF16)

    def project(j, nb, nj):
        nkv = 7 * -(-Q // 16)
        gens = {"k": (post_kv(j, KEY), nkv), "v": (post_kv(j, VAL), nkv), "g": (post_act(j, GATE), H // 4),
                "s": (norm_stats(nb, nj), H // 8), "n": (norm_apply(nb, nj), H // 8)}
        streams = [_stream(*gens[name], (0,) * pos + w + (0,) * (35 - pos - len(w))) for name, pos, w in A_FILL]
        strassen2(lnext, lambda lhs, n: _mm(lhs, wg[n]), ss.at[GATE], _spread(streams, _never(j)))
        for pos, m in enumerate((KEY, VAL, UP)):
            buf = ss.at[m]

            def fin(q, v):
                buf[q] = v

            def product(i):
                if pos == 0:
                    v = [lnext[i, t] for t in range(2)]
                    for t in range(2):
                        ql[j, i, t] = v[t]
                else:
                    v = [ql[j, i, t] for t in range(2)]
                return _mm(jnp.concatenate(v, axis=1), wr[m, i])
            _strassen(product, buf, buf, fin, _spread(streams, _never(j), 14 + 7 * pos))
        _drain(post_act(j, UP))

    def valid_keys(c):
        return lax.broadcasted_iota(jnp.int32, (8, LANES), 1) < T // 4 - c * LANES

    def qk_unit(j, c, buf, hook):
        keys = pl.ds(_al(c * LANES, LANES), LANES)
        strassen2(ql.at[j], lambda lhs, n: _mm_nt(lhs, kr[n, keys, :]), buf, hook)

    def sumexp(c, buf, copy_to=None, halves=(1, 0)):
        valid = valid_keys(c)
        for h in halves:
            for r in range(0, H, 8):
                tok = yield
                rr = pl.ds(r, 8)
                old = _gate(mrun[h, rr, :], tok)
                v = []
                for q in (2 * h, 2 * h + 1):
                    for t in range(2):
                        v.append(buf[q, rr, pl.ds(t * LANES, LANES)])
                        if copy_to is not None:
                            copy_to[q, rr, pl.ds(t * LANES, LANES)] = v[-1]
                top = jnp.maximum(jnp.maximum(v[0], v[1]), jnp.maximum(v[2], v[3]))
                m = jnp.maximum(old, jnp.where(valid, top, LOWEST))
                e = [jnp.exp2(x - m) for x in v]
                l = lrun[h, rr, :] * jnp.exp2(old - m)
                lrun[h, rr, :] = l + jnp.where(valid, (e[0] + e[1]) + (e[2] + e[3]), 0.0)
                mrun[h, rr, :] = m

    def finish_stats(n):
        for h in range(2):
            for r in range(0, H, n):
                tok = yield
                rr = pl.ds(r, n)
                m = jnp.max(_gate(mrun[h, rr, :], tok), axis=-1, keepdims=True)
                mfin[h, rr, :] = jnp.broadcast_to(m, (n, LANES))
        for h in range(2):
            for r in range(0, H, n):
                tok = yield
                rr = pl.ds(r, n)
                e = jnp.exp2(_gate(mrun[h, rr, :], tok) - mfin[h, rr, :])
                l = jnp.sum(lrun[h, rr, :] * e, axis=-1, keepdims=True)
                linv[h, rr, :] = jnp.broadcast_to(1.0 / l, (n, LANES))
                mrun[h, rr, :] = jnp.full((n, LANES), LOWEST, F32)
                lrun[h, rr, :] = jnp.zeros((n, LANES), F32)

    def probs(c, buf, k, r0=0, r1=Q):
        valid = valid_keys(c)
        for r in range(r0, r1, 8):
            for t in range(4):
                tok = yield
                rr, cols = pl.ds((t // 2) * Q + r, 8), pl.ds((t % 2) * LANES, LANES)
                top = _gate(jnp.full((8, LANES), jnp.inf, F32), tok)
                m = [jnp.where(valid, mfin[h, rr, :], top) for h in range(2)]
                il = [linv[h, rr, :] for h in range(2)]
                p = [jnp.exp2(buf[q, rr, cols] - m[q // 2]) * il[q // 2] for q in range(4)]
                for o, v in enumerate(_combos(_LHS, p)):
                    pbuf[o, t, pl.ds(r, 8), pl.ds(k * LANES, LANES)] = v

    def pv_unit(u, hook, r0=0, r1=Q):
        rows = pl.ds(r0, r1 - r0)
        keys = pl.ds(_al(u * CU * LANES, LANES), CU * LANES)
        for n in range(49):
            lhs = _combo(_LHS, n % 7, lambda t: pbuf[n // 7, t, rows, :])
            v = _mm(lhs, vr[n, keys, :])
            acc[n, rows, :] = jnp.where(u > 0, acc[n, rows, :], 0.0) + v
            hook(n, v)

    def attn_rows():
        for r in range(0, Q, 8):
            tok = yield
            inner = []
            for o in range(7):
                m = [acc[7 * o + i, pl.ds(r, 8), :] for i in range(7)]
                m[2], m[3] = _gate(m[2], tok), _gate(m[3], tok)
                inner.append(_out_combos(m))
            for t in range(4):
                for q, v in enumerate(_out_combos([inner[o][t] for o in range(7)])):
                    sx[q, pl.ds((t // 2) * Q + r, 8), pl.ds((t % 2) * LANES, LANES)] = v

    def conv(j, t, h):
        r0 = j * BQ + h * H
        shift = HALO - KT // 2
        for a in range(0, H // 8, CV):
            o = None
            cnt = 0
            for r in range(8):
                taps = [i for i in range(KT) if (i + shift) % 8 == r]
                lo, hi = (taps[0] + shift) // 8, (taps[-1] + shift) // 8
                g = gs[t, pl.ds(r0 + 8 * (a + lo) + r, 8 * (CV + hi - lo)), :].reshape(CV + hi - lo, 8, LANES)
                for i in taps:
                    w = dwb[t, i]
                    if cnt % CG == 0:
                        tok = yield
                        w = _gate(w, tok)
                    cnt += 1
                    k = (i + shift) // 8 - lo
                    term = g[k:k + CV] * w[None]
                    o = term if o is None else o + term
            uc[t, pl.ds(h * H + 8 * a, 8 * CV), :] = (
                us[t, pl.ds(_al(r0 + 8 * a, 8), 8 * CV), :] * o.reshape(8 * CV, LANES))

    def conv_unit(j, u, weights):
        per = 2 * NT // NU
        steps = per * (H // 8 // CV) * -(-KT // CG)
        return _stream(_chain([conv(j, u * (per // 2) + k // 2, k % 2) for k in range(per)]), steps, weights)

    def first(c):
        p = jnp.maximum(c - 1, 0)
        se = [_stream(sumexp(jnp.where(c > 0, p, NC), ss.at[p], None, (0,)), H // 8, W_S0),
              _stream(sumexp(c, ss.at[c], None, (1,)), H // 8, (0,) * 9 + W_S1)]
        qk_unit(0, c, ss.at[c], _spread(se, _never(c)))

    def steady(j, u):
        never = _never(u)
        sv = ss.at[pl.ds(u * CU, CU)]
        nq = 14 * CU
        pc = _stream(_chain([probs(u * CU + k, sv.at[k], k) for k in list(range(1, CU)) + [0]]),
                     CU * Q // 2, W_PC * CU)
        for k in range(CU):
            qk_unit(j + 1, u * CU + k, sv.at[k] if k else sx, _spread([pc], never, 14 * k))
        se = _stream(_chain([sumexp(u * CU + k, sv.at[k] if k else sx, None if k else sv.at[0])
                             for k in range(CU)]), CU * H // 4, (1,) * W_SE + (0,) * (49 - W_SE))
        cv = conv_unit(j, u, (1,) * 49)
        pv_unit(u, _spread([cv, se], never))

    def last_probs(u, r0, r1):
        return _chain([probs(u * CU + k, ss.at[u * CU + k], k, r0, r1) for k in range(CU)])

    def last(u):
        never = _never(u)
        cv = conv_unit(NQ - 1, u, (1,) * 98)
        pc = _stream(last_probs(u, QS, Q), CU * (Q - QS) // 2, (1,) * 49)
        pv_unit(u, _spread([pc, cv], never), 0, QS)
        pc = _stream(last_probs(jnp.minimum(u + 1, NU - 1), 0, QS), CU * QS // 2, (0,) * 49 + (1,) * 49)
        pv_unit(u, _spread([pc, cv], never, 49), QS, Q)

    def finish_block(b, j, slot):
        def quad(q):
            return jnp.concatenate([uc[2 * (q % 2) + t, pl.ds((q // 2) * H, H), :] for t in range(2)], axis=1)

        def fin(q, v):
            cols = pl.ds((q % 2) * DH, DH)
            obuf[slot, pl.ds((q // 2) * H, H), cols] = (
                x_rows(b, j, q // 2, 0, H, cols) + (sx[q] + v)).astype(BF16)

        def product(i):
            return _mm(_combo(_LHS, i, quad), wr[DOWN, i])
        hook = _spread([_stream(attn_rows(), Q // 8, W_FIN), _stream(finish_stats(8), H // 2, W_FIN)], _never(j))
        v = product(0)
        tq[0] = v
        hook(0, v)
        v = tq[0] + product(6)
        tq[1] = v
        hook(1, v)
        v = tq[0] + product(5)
        tq[0] = v
        hook(2, v)
        v = product(2)
        tq[0] = tq[0] + v
        tq[2] = v
        hook(3, v)
        v = product(3)
        tq[1] = tq[1] + v
        tq[3] = v
        hook(4, v)
        v = product(1)
        fin(2, tq[3] + v)
        fin(3, tq[0] - v)
        ocopy(b, j, 1).start()
        hook(5, v)
        v = product(4)
        fin(1, tq[2] + v)
        fin(0, tq[1] - v)
        ocopy(b, j, 0).start()

    def batch(b):
        def project_block(j):
            f = b * NQ + j + 1
            nxt = jnp.minimum(f, B * NQ - 1)

            @pl.when(f < B * NQ)
            def _():
                xcopy(nxt // NQ, nxt % NQ).wait()
            project(j, nxt // NQ, nxt % NQ)
        _loop(NQ, project_block)
        _loop(NC, first, 2)

        def first_stats():
            _drain(sumexp(NC - 1, ss.at[NC - 1], None, (0,)))
            _drain(finish_stats(80))

        @pl.when(b == 0)
        def _():
            wcopy[4].wait()
            wcopy[5].wait()
            w = _dot(wtmp[4], wtmp[5])
            store_weights(DOWN, w[:DH], w[DH:])
            first_stats()

        @pl.when(b > 0)
        def _():
            first_stats()

        def query_block(j):
            @pl.when(j < NQ - 1)
            def _():
                _loop(NU, lambda u: steady(j, u))

            @pl.when(j == NQ - 1)
            def _():
                _drain(last_probs(0, 0, QS))
                _loop(NU, last)
            f = b * NQ + j

            @pl.when(f >= 2)
            def _():
                for h in range(2):
                    ocopy((f - 2) // NQ, (f - 2) % NQ, h).wait()
            finish_block(b, j, f % 2)
        _loop(NQ, query_block)
    _loop(B, batch)
    for j in (NQ - 2, NQ - 1):
        for h in range(2):
            ocopy(B - 1, j, h).wait()


@jax.jit
def pallas_standalone__conformer_family_branchformer__speech_kernel(
        x, w_q, w_k, w_v, w_ao, w_up, dw, w_dn, w_merge):
    B, T, D = x.shape
    KT = dw.shape[0]
    DH, NT, Q = D // 2, D // LANES, H // 2
    NQ = T // (2 * H)
    NC = -(-(T // 4) // LANES)
    assert D == 4 * LANES and T % (2 * H) == 0 and NQ >= 2 and NC % CU == 0 and NC >= 4
    assert KT % 2 == 1 and 8 <= KT <= 2 * HALO - 1
    scratch = [
        pltpu.VMEM((B, T, D), BF16),
        pltpu.VMEM((7, D, D), BF16),
        pltpu.VMEM((D, 2 * D), BF16),
        pltpu.VMEM((KT, D), BF16),
        pltpu.VMEM((4, 7, DH, DH), BF16),
        pltpu.VMEM((52, LANES, LANES), BF16),
        pltpu.VMEM((NT, 2 * HALO, 8, LANES), F32),
        pltpu.VMEM((NQ, 7, 2, H, LANES), F32),
        pltpu.VMEM((7, 2, H, LANES), F32),
        pltpu.VMEM((49, NC * LANES, LANES), BF16),
        pltpu.VMEM((49, NC * LANES, LANES), BF16),
        pltpu.VMEM((NT, T + 2 * HALO, LANES), F32),
        pltpu.VMEM((NT, T, LANES), F32),
        pltpu.VMEM((NT, 2 * H, LANES), F32),
        pltpu.VMEM((NC, 4, H, DH), F32),
        pltpu.VMEM((4, H, DH), F32),
        pltpu.VMEM((4, H, DH), F32),
        pltpu.VMEM((4, Q, LANES), F32),
        pltpu.VMEM((4, 3, Q, LANES), F32),
        pltpu.VMEM((7, 4, Q, CU * LANES), F32),
        pltpu.VMEM((52, Q, LANES), F32),
        pltpu.VMEM((2, H, LANES), F32),
        pltpu.VMEM((2, H, LANES), F32),
        pltpu.VMEM((2, H, LANES), F32),
        pltpu.VMEM((2, H, LANES), F32),
        pltpu.VMEM((2, 2, H, LANES), F32),
        pltpu.VMEM((2, 2 * H, D), BF16),
        pltpu.SemaphoreType.DMA((9,)),
        pltpu.SemaphoreType.DMA((B * NQ,)),
        pltpu.SemaphoreType.DMA((4,)),
    ]
    anyspec = pl.BlockSpec(memory_space=pl.ANY)
    return pl.pallas_call(
        _kernel,
        out_shape=jax.ShapeDtypeStruct(x.shape, x.dtype),
        grid=(1,),
        in_specs=[anyspec] * 9,
        out_specs=anyspec,
        scratch_shapes=scratch,
        compiler_params=pltpu.CompilerParams(vmem_limit_bytes=124 * 1024 * 1024),
    )(x, w_q, w_k, w_v, w_ao, w_up, dw, w_dn, w_merge)
```
